```python
import jax
import jax.numpy as jnp

def _softmax(x, axis=-1):
    return jax.nn.softmax(x, axis=axis)
def _gelu(x):
    return jax.nn.gelu(x, approximate=True)
def _silu(x):
    return jax.nn.silu(x)
def _sigmoid(x):
    return jax.nn.sigmoid(x)
def _layernorm(x, axis=-1, eps=1e-5):
    m = jnp.mean(x, axis=axis, keepdims=True)
    v = jnp.var(x, axis=axis, keepdims=True)
    return (x - m) / jnp.sqrt(v + eps)
def _scatter_add(tgt, idx, src, axis=0):
    return tgt.at[idx].add(src)
def _segment_sum(src, seg, n):
    return jax.ops.segment_sum(src, seg, n)
class _Rng:
    def __init__(self, key):
        self._k = key
    def _next(self):
        self._k, sub = jax.random.split(self._k)
        return sub
    def normal(self, shape):
        return jax.random.normal(self._next(), shape, dtype=jnp.bfloat16)
    def randint(self, lo, hi, shape):
        return jax.random.randint(self._next(), shape, lo, hi, dtype=jnp.int32)
    def uniform(self, shape, lo=0.0, hi=1.0):
        return jax.random.uniform(self._next(), shape, jnp.bfloat16, lo, hi)
    def permutation(self, n):
        return jax.random.permutation(self._next(), n)


kernel_name = 'interleave_layers__sliding_local_dilated__glu_gated_bilinear__prompt'

def setup_inputs():
    _rng = _Rng(jax.random.key(int.from_bytes(__import__("os").urandom(4), "little")))
    _w = (lambda a: (lambda t: t.astype(jnp.bfloat16) if jnp.issubdtype(t.dtype, jnp.floating) else t)(jnp.asarray(a)))
    def _A_setup():
        B, S, D = 1, 2048, 576
        return {
            "x": _w((lambda *s: _rng.normal(s) * 0.05)(B, S, D)),
            "wqkv": _w((lambda *s: _rng.normal(s) * 0.05)(D, 3 * D)),
            "wo": _w((lambda *s: _rng.normal(s) * 0.05)(D, D)),
        }
    _A_in = _A_setup()

    def _B_setup():
        B, S, D, F = 1, 2048, 576, 4608
        return {
            "x": _w((lambda *s: _rng.normal(s) * 0.05)(B, S, D)),
            "w_gate": _w((lambda *s: _rng.normal(s) * 0.05)(D, F) * (D ** -0.5)),
            "w_up": _w((lambda *s: _rng.normal(s) * 0.05)(D, F) * (D ** -0.5)),
            "w_down": _w((lambda *s: _rng.normal(s) * 0.05)(F, D) * (F ** -0.5)),
        }
    _B_in = _B_setup()

    return {
        "A_x": _A_in["x"],
        "A_wqkv": _A_in["wqkv"],
        "A_wo": _A_in["wo"],
        "B_x": _B_in["x"],
        "B_w_gate": _B_in["w_gate"],
        "B_w_up": _B_in["w_up"],
        "B_w_down": _B_in["w_down"],
    }

def reference(A_x, A_wqkv, A_wo, B_x, B_w_gate, B_w_up, B_w_down):
    def _A_ref(x, wqkv, wo):
        B, S, D = x.shape
        H = 32; Dh = D // H
        W, dil = 8, 2
        qkv = (lambda x, *d: x.transpose(*d))((x @ wqkv).reshape(B, S, 3, H, Dh), 2, 0, 3, 1, 4)
        q, k, v = qkv[0], qkv[1], qkv[2]
        scale = Dh ** -0.5
        pos = jnp.arange(S)
        off = jnp.arange(W) * dil
        idx = pos[:, None] - off[None, :]
        mask = idx >= 0
        idx_c = jnp.where(mask, idx, 0).reshape(-1)
        kg = k[:, :, idx_c, :].reshape(B, H, S, W, Dh)
        vg = v[:, :, idx_c, :].reshape(B, H, S, W, Dh)
        logits = jnp.einsum("bhsd,bhswd->bhsw", q, kg) * scale
        logits = jnp.where(mask[None, None, :, :], logits, -1e9)
        attn = _softmax(logits, axis=-1)
        o = jnp.einsum("bhsw,bhswd->bhsd", attn, vg)
        return (lambda x, *d: x.transpose(*d))(o, 0, 2, 1, 3).reshape(B, S, D) @ wo

    def _B_ref(x, w_gate, w_up, w_down):
        g = jnp.einsum("bsd,df->bsf", x, w_gate)
        u = jnp.einsum("bsd,df->bsf", x, w_up)
        h = g * u
        return jnp.einsum("bsf,fd->bsd", h, w_down)

    x = A_x
    x = x + _A_ref(_layernorm(x, axis=-1), A_wqkv, A_wo)
    x = x + _B_ref(_layernorm(x, axis=-1), B_w_gate, B_w_up, B_w_down)
    x = x + _A_ref(_layernorm(x, axis=-1), A_wqkv, A_wo)
    x = x + _B_ref(_layernorm(x, axis=-1), B_w_gate, B_w_up, B_w_down)
    return x
```

```python
import functools

import jax
import jax.numpy as jnp
import jax.experimental.pallas as pl
import jax.experimental.pallas.tpu as pltpu

S = 2048
D = 576
F = 4608
H = 32
DH = 18
W = 8
DIL = 2
EPS = 1e-5
LANES = 128

TM = 512
NT = S // TM
FC = 1152
NCH = F // FC
AR = TM // NCH
RB = 32
HALO = 16
NB = 14
DB = 5

Q_BLOCKS = (0, 1, 2, 3, 12)
K_BLOCKS = (4, 5, 6, 7, 13)
V_BLOCKS = (8, 9, 10, 11, 12)
KV_BLOCKS = (4, 5, 6, 7, 8, 9, 10, 11, 12, 13)

SCALE = DH ** -0.5
EXP2_SCALE = SCALE * 1.4426950408889634
MASKED_LOGIT = -1e9 / SCALE

NT_DIMS = (((1,), (1,)), ((), ()))
F32 = jnp.float32
BF16 = jnp.bfloat16


def _qkv_dest_row(part, d):
    if d < 16:
        return (part * 4 + d // 4) * LANES + (d % 4) * H
    base = (12 * LANES, 13 * LANES, 12 * LANES + 64)[part]
    return base + (d - 16) * H


def _o_dest_row(d):
    if d < 16:
        return d * H
    return 4 * LANES + 64 + (d - 16) * H


def _layernorm_t(x):
    m = jnp.mean(x, axis=0, keepdims=True)
    c = x - m
    v = jnp.mean(c * c, axis=0, keepdims=True)
    y = c * jax.lax.rsqrt(v + EPS)
    return y.astype(BF16).T


def _kernel(xT_hbm, wqkv_hbm, wo_hbm, wg_hbm, wu_hbm, wdT_hbm, out_hbm,
            xin, xres, xout, wqkv_raw, wo_raw, wg, wu, wd,
            wt_tmp, wq_p, wo_tmp, wo_p, wo_pt, qkv, o_s, xn2,
            sem_x, sem_w, sem_f, sem_o):

    def x_copy(t):
        return pltpu.make_async_copy(
            xT_hbm.at[:, pl.ds(t * TM, TM)], xin.at[t], sem_x.at[t])

    def f_copy(which, c):
        src = (wg_hbm, wu_hbm, wdT_hbm)[which]
        dst = (wg, wu, wd)[which]
        return pltpu.make_async_copy(
            src.at[:, pl.ds(c * FC, FC)], dst.at[c], sem_f.at[which * NCH + c])

    def out_copy(t):
        return pltpu.make_async_copy(
            xout.at[t], out_hbm.at[:, pl.ds(t * TM, TM)], sem_o.at[t])

    wqkv_copy = pltpu.make_async_copy(wqkv_hbm, wqkv_raw, sem_w.at[0])
    wo_copy = pltpu.make_async_copy(wo_hbm, wo_raw, sem_w.at[1])

    wqkv_copy.start()
    x_copy(0).start()
    wo_copy.start()
    for t in range(1, NT):
        x_copy(t).start()
    for c in range(NCH):
        for which in range(3):
            f_copy(which, c).start()

    def prep_wqkv():
        for j in range(DB):
            rows = min(LANES, D - j * LANES)
            blk = wqkv_raw[j * LANES:j * LANES + rows, :].astype(F32)
            wt_tmp[j, :, 0:rows] = blk.T
        for part in range(3):
            for d in range(DH):
                dst = _qkv_dest_row(part, d)
                for j in range(DB):
                    cols = min(LANES, D - j * LANES)
                    val = wt_tmp[j, pl.ds(part * D + d, H, stride=DH), :]
                    wq_p[dst:dst + H, j * LANES:j * LANES + cols] = (
                        val[:, 0:cols].astype(BF16))
        wq_p[13 * LANES + 64:14 * LANES, :] = jnp.zeros((64, D), BF16)

    def prep_wo():
        for j in range(DB):
            cols = min(LANES, D - j * LANES)
            wo_tmp[j, :, 0:cols] = (
                wo_raw[:, j * LANES:j * LANES + cols].astype(F32))
        for d in range(DH):
            dst = _o_dest_row(d)
            for j in range(DB):
                cols = min(LANES, D - j * LANES)
                val = wo_tmp[j, pl.ds(d, H, stride=DH), :]
                wo_p[dst:dst + H, j * LANES:j * LANES + cols] = val[:, 0:cols]
        wo_p[4 * LANES:4 * LANES + 64, :] = jnp.zeros((64, D), F32)
        wo_pt[...] = wo_p[...].astype(BF16).T

    def qkv_stage(t, first_tile):
        tails = None
        if first_tile is not True:
            tails = [qkv[j, TM:TM + HALO, :] for j in KV_BLOCKS]
        xn = _layernorm_t(xres[t])
        res = jax.lax.dot_general(xn, wq_p[...], NT_DIMS,
                                  preferred_element_type=F32)
        for j in range(NB):
            qkv[j, HALO:HALO + TM, :] = res[:, j * LANES:(j + 1) * LANES]
        for i, j in enumerate(KV_BLOCKS):
            row0 = jnp.broadcast_to(res[0:1, j * LANES:(j + 1) * LANES],
                                    (HALO, LANES))
            if first_tile is True:
                qkv[j, 0:HALO, :] = row0
            else:
                qkv[j, 0:HALO, :] = jnp.where(first_tile, row0, tails[i])

    def attn_unit(t, r0):
        def load(j, w):
            return qkv[j, pl.ds(HALO + r0 - DIL * w, RB), :]

        pos = t * TM + r0 + jax.lax.broadcasted_iota(jnp.int32, (RB, LANES), 0)
        q = [load(j, 0) for j in Q_BLOCKS]
        logits = []
        for w in range(W):
            p = q[0] * load(K_BLOCKS[0], w)
            for i in range(1, DB):
                p = p + q[i] * load(K_BLOCKS[i], w)
            p = p + pltpu.roll(p, 64, 1)
            p = p + pltpu.roll(p, 32, 1)
            if w > 0:
                p = jnp.where(pos >= DIL * w, p, MASKED_LOGIT)
            logits.append(p)
        m = logits[0]
        for w in range(1, W):
            m = jnp.maximum(m, logits[w])
        es = [jnp.exp2((l - m) * EXP2_SCALE) for l in logits]
        s = es[0]
        for w in range(1, W):
            s = s + es[w]
        r = 1.0 / s
        for i, j in enumerate(V_BLOCKS):
            o = es[0] * load(j, 0)
            for w in range(1, W):
                o = o + es[w] * load(j, w)
            o = o * r
            if i == DB - 1:
                lane = jax.lax.broadcasted_iota(jnp.int32, (RB, LANES), 1)
                o = jnp.where(lane >= 64, o, 0.0)
            o_s[pl.ds(r0, RB), i * LANES:(i + 1) * LANES] = o.astype(BF16)

    def wo_stage(t):
        upd = jax.lax.dot_general(wo_pt[...], o_s[...], NT_DIMS,
                                  preferred_element_type=F32)
        x = xres[t] + upd
        xres[t] = x
        xn2[...] = _layernorm_t(x)

    def ffn_chunk(t, c):
        xn = xn2[...]
        g = jnp.dot(xn, wg[c], preferred_element_type=F32)
        u = jnp.dot(xn, wu[c], preferred_element_type=F32)
        h = (g * u).astype(BF16)
        xres[t] += jax.lax.dot_general(wd[c], h, NT_DIMS,
                                       preferred_element_type=F32)

    wqkv_copy.wait()
    prep_wqkv()
    x_copy(0).wait()
    wo_copy.wait()
    for t in range(1, NT):
        x_copy(t).wait()
    for t in range(NT):
        xres[t] = xin[t].astype(F32)
    prep_wo()
    qkv_stage(0, True)

    def attn0(i, carry):
        attn_unit(0, pl.multiple_of(i * RB, RB))
        return carry
    jax.lax.fori_loop(0, TM // RB, attn0, 0)

    for c in range(NCH):
        for which in range(3):
            f_copy(which, c).wait()

    def step(n, carry):
        t = n % NT
        tn = (n + 1) % NT
        wo_stage(t)
        qkv_stage(tn, tn == 0)

        def chunk(c, carry2):
            ffn_chunk(t, c)
            for a in range(AR // RB):
                attn_unit(tn, pl.multiple_of(c * AR + a * RB, RB))
            return carry2
        jax.lax.fori_loop(0, NCH, chunk, 0)

        @pl.when(n >= NT)
        def _():
            xout[t] = xres[t].astype(BF16)
            out_copy(t).start()
        return carry
    jax.lax.fori_loop(0, 2 * NT - 1, step, 0)

    wo_stage(NT - 1)

    def last_chunk(c, carry):
        ffn_chunk(NT - 1, c)
        return carry
    jax.lax.fori_loop(0, NCH, last_chunk, 0)
    xout[NT - 1] = xres[NT - 1].astype(BF16)
    out_copy(NT - 1).start()
    for t in range(NT):
        out_copy(t).wait()


@jax.jit
def pallas_interleave_layers__sliding_local_dilated__glu_gated_bilinear__prompt_kernel(
    A_x: jax.Array,
    A_wqkv: jax.Array,
    A_wo: jax.Array,
    B_x: jax.Array,
    B_w_gate: jax.Array,
    B_w_up: jax.Array,
    B_w_down: jax.Array,
):
    del B_x
    xT = A_x.reshape(S, D).T
    wdT = B_w_down.T
    any_spec = pl.BlockSpec(memory_space=pl.ANY)
    outT = pl.pallas_call(
        _kernel,
        in_specs=[any_spec] * 6,
        out_specs=any_spec,
        out_shape=jax.ShapeDtypeStruct((D, S), BF16),
        scratch_shapes=[
            pltpu.VMEM((NT, D, TM), BF16),
            pltpu.VMEM((NT, D, TM), F32),
            pltpu.VMEM((NT, D, TM), BF16),
            pltpu.VMEM((D, 3 * D), BF16),
            pltpu.VMEM((D, D), BF16),
            pltpu.VMEM((NCH, D, FC), BF16),
            pltpu.VMEM((NCH, D, FC), BF16),
            pltpu.VMEM((NCH, D, FC), BF16),
            pltpu.VMEM((DB, 3 * D, LANES), F32),
            pltpu.VMEM((NB * LANES, D), BF16),
            pltpu.VMEM((DB, D, LANES), F32),
            pltpu.VMEM((DB * LANES, D), F32),
            pltpu.VMEM((D, DB * LANES), BF16),
            pltpu.VMEM((NB, HALO + TM, LANES), F32),
            pltpu.VMEM((TM, DB * LANES), BF16),
            pltpu.VMEM((TM, D), BF16),
            pltpu.SemaphoreType.DMA((NT,)),
            pltpu.SemaphoreType.DMA((2,)),
            pltpu.SemaphoreType.DMA((3 * NCH,)),
            pltpu.SemaphoreType.DMA((NT,)),
        ],
        compiler_params=pltpu.CompilerParams(
            vmem_limit_bytes=100 * 1024 * 1024),
    )(xT, A_wqkv, A_wo, B_w_gate, B_w_up, wdT)
    return outT.T.reshape(1, S, D)
```

```python
import functools

import jax
import jax.numpy as jnp
import jax.experimental.pallas as pl
import jax.experimental.pallas.tpu as pltpu

S = 2048
D = 576
F = 4608
H = 32
DH = 18
W = 8
DIL = 2
EPS = 1e-5
LANES = 128

TM = 512
NT = S // TM
FC = 1152
NCH = F // FC
AR = TM // NCH
RB = 32
HALO = 16
NB = 14
DB = 5

Q_BLOCKS = (0, 1, 2, 3, 12)
K_BLOCKS = (4, 5, 6, 7, 13)
V_BLOCKS = (8, 9, 10, 11, 12)
KV_BLOCKS = (4, 5, 6, 7, 8, 9, 10, 11, 12, 13)

SCALE = DH ** -0.5
EXP2_SCALE = SCALE * 1.4426950408889634
MASKED_LOGIT = -1e9 / SCALE

NT_DIMS = (((1,), (1,)), ((), ()))
F32 = jnp.float32
BF16 = jnp.bfloat16


def _qkv_dest_row(part, d):
    if d < 16:
        return (part * 4 + d // 4) * LANES + (d % 4) * H
    base = (12 * LANES, 13 * LANES, 12 * LANES + 64)[part]
    return base + (d - 16) * H


def _o_dest_row(d):
    if d < 16:
        return d * H
    return 4 * LANES + 64 + (d - 16) * H


def _layernorm_t(x):
    m = jnp.mean(x, axis=0, keepdims=True)
    c = x - m
    v = jnp.mean(c * c, axis=0, keepdims=True)
    y = c * jax.lax.rsqrt(v + EPS)
    return y.astype(BF16).T


def _kernel(xT_hbm, wqkv_hbm, wo_hbm, wg_hbm, wu_hbm, wdT_hbm, out_hbm,
            xin, xres, xout, wqkv_raw, wo_raw, wg, wu, wd,
            wt_tmp, wq_p, wo_tmp, wo_p, wo_pt, qkv, o_s, xn2,
            sem_x, sem_w, sem_f, sem_o):

    def x_copy(t):
        return pltpu.make_async_copy(
            xT_hbm.at[:, pl.ds(t * TM, TM)], xin.at[t], sem_x.at[t])

    def f_copy(which, c):
        src = (wg_hbm, wu_hbm, wdT_hbm)[which]
        dst = (wg, wu, wd)[which]
        return pltpu.make_async_copy(
            src.at[:, pl.ds(c * FC, FC)], dst.at[c], sem_f.at[which * NCH + c])

    def out_copy(t):
        return pltpu.make_async_copy(
            xout.at[t], out_hbm.at[:, pl.ds(t * TM, TM)], sem_o.at[t])

    wqkv_copy = pltpu.make_async_copy(wqkv_hbm, wqkv_raw, sem_w.at[0])
    wo_copy = pltpu.make_async_copy(wo_hbm, wo_raw, sem_w.at[1])

    wqkv_copy.start()
    x_copy(0).start()

    def prep_wqkv():
        for j in range(DB):
            rows = min(LANES, D - j * LANES)
            blk = wqkv_raw[j * LANES:j * LANES + rows, :].astype(F32)
            wt_tmp[j, :, 0:rows] = blk.T
        for part in range(3):
            for d in range(DH):
                dst = _qkv_dest_row(part, d)
                for j in range(DB):
                    cols = min(LANES, D - j * LANES)
                    val = wt_tmp[j, pl.ds(part * D + d, H, stride=DH), :]
                    wq_p[dst:dst + H, j * LANES:j * LANES + cols] = (
                        val[:, 0:cols].astype(BF16))
        wq_p[13 * LANES + 64:14 * LANES, :] = jnp.zeros((64, D), BF16)

    def prep_wo():
        for j in range(DB):
            cols = min(LANES, D - j * LANES)
            wo_tmp[j, :, 0:cols] = (
                wo_raw[:, j * LANES:j * LANES + cols].astype(F32))
        for d in range(DH):
            dst = _o_dest_row(d)
            for j in range(DB):
                cols = min(LANES, D - j * LANES)
                val = wo_tmp[j, pl.ds(d, H, stride=DH), :]
                wo_p[dst:dst + H, j * LANES:j * LANES + cols] = val[:, 0:cols]
        wo_p[4 * LANES:4 * LANES + 64, :] = jnp.zeros((64, D), F32)
        wo_pt[...] = wo_p[...].astype(BF16).T

    def qkv_stage(xn, first_tile):
        tails = None
        if first_tile is not True:
            tails = [qkv[j, TM:TM + HALO, :] for j in KV_BLOCKS]
        res = jax.lax.dot_general(xn, wq_p[...], NT_DIMS,
                                  preferred_element_type=F32)
        for j in range(NB):
            qkv[j, HALO:HALO + TM, :] = res[:, j * LANES:(j + 1) * LANES]
        for i, j in enumerate(KV_BLOCKS):
            row0 = jnp.broadcast_to(res[0:1, j * LANES:(j + 1) * LANES],
                                    (HALO, LANES))
            if first_tile is True:
                qkv[j, 0:HALO, :] = row0
            else:
                qkv[j, 0:HALO, :] = jnp.where(first_tile, row0, tails[i])

    def attn_unit(t, r0):
        def load(j, w):
            return qkv[j, pl.ds(HALO + r0 - DIL * w, RB), :]

        pos = t * TM + r0 + jax.lax.broadcasted_iota(jnp.int32, (RB, LANES), 0)
        q = [load(j, 0) for j in Q_BLOCKS]
        logits = []
        for w in range(W):
            p = q[0] * load(K_BLOCKS[0], w)
            for i in range(1, DB):
                p = p + q[i] * load(K_BLOCKS[i], w)
            p = p + pltpu.roll(p, 64, 1)
            p = p + pltpu.roll(p, 32, 1)
            if w > 0:
                p = jnp.where(pos >= DIL * w, p, MASKED_LOGIT)
            logits.append(p)
        m = logits[0]
        for w in range(1, W):
            m = jnp.maximum(m, logits[w])
        es = [jnp.exp2((l - m) * EXP2_SCALE) for l in logits]
        s = es[0]
        for w in range(1, W):
            s = s + es[w]
        r = 1.0 / s
        for i, j in enumerate(V_BLOCKS):
            o = es[0] * load(j, 0)
            for w in range(1, W):
                o = o + es[w] * load(j, w)
            o = o * r
            if i == DB - 1:
                lane = jax.lax.broadcasted_iota(jnp.int32, (RB, LANES), 1)
                o = jnp.where(lane >= 64, o, 0.0)
            o_s[pl.ds(r0, RB), i * LANES:(i + 1) * LANES] = o.astype(BF16)

    def wo_proj():
        return jax.lax.dot_general(wo_pt[...], o_s[...], NT_DIMS,
                                   preferred_element_type=F32)

    def wo_finish(t, upd):
        x = xres[t] + upd
        xres[t] = x
        xn2[...] = _layernorm_t(x)

    def ffn_chunk(t, c):
        xn = xn2[...]
        g = jnp.dot(xn, wg[c], preferred_element_type=F32)
        u = jnp.dot(xn, wu[c], preferred_element_type=F32)
        h = (g * u).astype(BF16)
        xres[t] += jax.lax.dot_general(wd[c], h, NT_DIMS,
                                       preferred_element_type=F32)

    with jax.named_scope("s_wait0"):
        wqkv_copy.wait()
        x_copy(0).wait()
        wo_copy.start()
        for t in range(1, NT):
            x_copy(t).start()
        for which in range(3):
            f_copy(which, 0).start()
    with jax.named_scope("s_prep"):
        prep_wqkv()
        xres[0] = xin[0].astype(F32)
        qkv_stage(_layernorm_t(xres[0]), True)
    with jax.named_scope("s_wait1"):
        wo_copy.wait()
        for t in range(1, NT):
            x_copy(t).wait()
        for c in range(1, NCH):
            for which in range(3):
                f_copy(which, c).start()
    with jax.named_scope("s_prep2"):
        for t in range(1, NT):
            xres[t] = xin[t].astype(F32)
        prep_wo()

    def attn0(i, carry):
        attn_unit(0, pl.multiple_of(i * RB, RB))
        return carry
    with jax.named_scope("s_attn0"):
        jax.lax.fori_loop(0, TM // RB, attn0, 0)

    def step(n, carry):
        t = n % NT
        tn = (n + 1) % NT
        with jax.named_scope("s_block1"):
            xn1 = _layernorm_t(xres[tn])
            upd = wo_proj()
            qkv_stage(xn1, tn == 0)
            wo_finish(t, upd)

        def chunk(c, carry2):
            @pl.when(n == 0)
            def _():
                for which in range(3):
                    f_copy(which, c).wait()
            ffn_chunk(t, c)
            for a in range(AR // RB):
                attn_unit(tn, pl.multiple_of(c * AR + a * RB, RB))
            return carry2
        with jax.named_scope("s_ffn"):
            jax.lax.fori_loop(0, NCH, chunk, 0)

        @pl.when(n >= NT)
        def _():
            xout[t] = xres[t].astype(BF16)
            out_copy(t).start()
        return carry
    jax.lax.fori_loop(0, 2 * NT - 1, step, 0)

    with jax.named_scope("s_wolast"):
        wo_finish(NT - 1, wo_proj())

    def last_chunk(c, carry):
        ffn_chunk(NT - 1, c)
        return carry
    with jax.named_scope("s_ffnlast"):
        jax.lax.fori_loop(0, NCH, last_chunk, 0)
    xout[NT - 1] = xres[NT - 1].astype(BF16)
    out_copy(NT - 1).start()
    for t in range(NT):
        out_copy(t).wait()


@jax.jit
def pallas_interleave_layers__sliding_local_dilated__glu_gated_bilinear__prompt_kernel(
    A_x: jax.Array,
    A_wqkv: jax.Array,
    A_wo: jax.Array,
    B_x: jax.Array,
    B_w_gate: jax.Array,
    B_w_up: jax.Array,
    B_w_down: jax.Array,
):
    del B_x
    xT = A_x.reshape(S, D).T
    wdT = B_w_down.T
    any_spec = pl.BlockSpec(memory_space=pl.ANY)
    outT = pl.pallas_call(
        _kernel,
        in_specs=[any_spec] * 6,
        out_specs=any_spec,
        out_shape=jax.ShapeDtypeStruct((D, S), BF16),
        scratch_shapes=[
            pltpu.VMEM((NT, D, TM), BF16),
            pltpu.VMEM((NT, D, TM), F32),
            pltpu.VMEM((NT, D, TM), BF16),
            pltpu.VMEM((D, 3 * D), BF16),
            pltpu.VMEM((D, D), BF16),
            pltpu.VMEM((NCH, D, FC), BF16),
            pltpu.VMEM((NCH, D, FC), BF16),
            pltpu.VMEM((NCH, D, FC), BF16),
            pltpu.VMEM((DB, 3 * D, LANES), F32),
            pltpu.VMEM((NB * LANES, D), BF16),
            pltpu.VMEM((DB, D, LANES), F32),
            pltpu.VMEM((DB * LANES, D), F32),
            pltpu.VMEM((D, DB * LANES), BF16),
            pltpu.VMEM((NB, HALO + TM, LANES), F32),
            pltpu.VMEM((TM, DB * LANES), BF16),
            pltpu.VMEM((TM, D), BF16),
            pltpu.SemaphoreType.DMA((NT,)),
            pltpu.SemaphoreType.DMA((2,)),
            pltpu.SemaphoreType.DMA((3 * NCH,)),
            pltpu.SemaphoreType.DMA((NT,)),
        ],
        compiler_params=pltpu.CompilerParams(
            vmem_limit_bytes=100 * 1024 * 1024),
    )(xT, A_wqkv, A_wo, B_w_gate, B_w_up, wdT)
    return outT.T.reshape(1, S, D)
```

```python
import jax
import jax.numpy as jnp
import jax.experimental.pallas as pl
import jax.experimental.pallas.tpu as pltpu

S = 2048
D = 576
F = 4608
H = 32
DH = 18
W = 8
DIL = 2
EPS = 1e-5
LANES = 128

TM = 512
NT = S // TM
FC = 1152
NCH = F // FC
SUB = TM // NCH
NS = S // SUB
RB = 8
RB0 = 32
HALO = 16
NB = 14
DB = 5

Q_BLOCKS = (0, 1, 2, 3, 12)
K_BLOCKS = (4, 5, 6, 7, 13)
V_BLOCKS = (8, 9, 10, 11, 12)
O_BLOCKS = (0, 1, 2, 3, 14)
KV_BLOCKS = (4, 5, 6, 7, 8, 9, 10, 11, 12, 13)

SCALE = DH ** -0.5
EXP2_SCALE = SCALE * 1.4426950408889634
MASKED_LOGIT = -1e9 / SCALE

NT_DIMS = (((1,), (1,)), ((), ()))
F32 = jnp.float32
BF16 = jnp.bfloat16


def _qkv_dest_row(part, d):
    if d < 16:
        return (part * 4 + d // 4) * LANES + (d % 4) * H
    base = (12 * LANES, 13 * LANES, 12 * LANES + 64)[part]
    return base + (d - 16) * H


def _o_dest_row(d):
    if d < 16:
        return d * H
    return 4 * LANES + 64 + (d - 16) * H


def _mod(a, n):
    assert n & (n - 1) == 0
    return jax.lax.bitwise_and(a, n - 1)


def _div(a, n):
    assert n & (n - 1) == 0
    return jax.lax.shift_right_logical(a, n.bit_length() - 1)


def _layernorm_t(x):
    m = jnp.mean(x, axis=0, keepdims=True)
    c = x - m
    v = jnp.mean(c * c, axis=0, keepdims=True)
    y = c * jax.lax.rsqrt(v + EPS)
    return y.astype(BF16).T


def _kernel(xT_hbm, wqkv_hbm, wo_hbm, wg_hbm, wu_hbm, wdT_hbm, out_hbm,
            xin, xres, xout, wqkv_raw, wo_raw, wg, wu, wd,
            wt_tmp, wq_p, wo_tmp, wo_p, wo_pt, xn1, xn2, row_s,
            sem_x, sem_w, sem_f, sem_o, *qkv_bufs):

    def x_copy(t):
        return pltpu.make_async_copy(
            xT_hbm.at[:, pl.ds(t * TM, TM)], xin.at[t], sem_x.at[t])

    def f_copy(which, c):
        src = (wg_hbm, wu_hbm, wdT_hbm)[which]
        dst = (wg, wu, wd)[which]
        start = c * FC
        if not isinstance(c, int):
            start = pl.multiple_of(start, LANES)
        return pltpu.make_async_copy(
            src.at[:, pl.ds(start, FC)], dst.at[c], sem_f.at[which * NCH + c])

    def out_copy(p):
        start = p * SUB
        if not isinstance(p, int):
            start = pl.multiple_of(start, LANES)
        return pltpu.make_async_copy(
            xout.at[p], out_hbm.at[:, pl.ds(start, SUB)], sem_o.at[p])

    def wqkv_copy(j):
        rows = pl.ds(j * LANES, min(LANES, D - j * LANES))
        return pltpu.make_async_copy(
            wqkv_hbm.at[rows], wqkv_raw.at[rows], sem_w.at[j])

    wo_copy = pltpu.make_async_copy(wo_hbm, wo_raw, sem_w.at[DB])

    def prep_wqkv(j):
        n = min(LANES, D - j * LANES)
        blk = wqkv_raw[j * LANES:j * LANES + n, :].astype(F32)
        wt_tmp[j, :, 0:n] = blk.T
        for part in range(3):
            for d in range(DH):
                dst = _qkv_dest_row(part, d)
                val = wt_tmp[j, pl.ds(part * D + d, H, stride=DH), :]
                wq_p[dst:dst + H, j * LANES:j * LANES + n] = (
                    val[:, 0:n].astype(BF16))

    def prep_wo():
        for j in range(DB):
            cols = min(LANES, D - j * LANES)
            wo_tmp[j, :, 0:cols] = (
                wo_raw[:, j * LANES:j * LANES + cols].astype(F32))
        for d in range(DH):
            dst = _o_dest_row(d)
            for j in range(DB):
                cols = min(LANES, D - j * LANES)
                val = wo_tmp[j, pl.ds(d, H, stride=DH), :]
                wo_p[dst:dst + H, j * LANES:j * LANES + cols] = val[:, 0:cols]
        wo_p[4 * LANES:4 * LANES + 64, :] = jnp.zeros((64, D), F32)
        wo_pt[...] = wo_p[...].astype(BF16).T

    def project(xn, qkv, prev, first):
        tails = None
        if first is not True:
            tails = [prev[j, SUB:SUB + HALO, :] for j in KV_BLOCKS]
        res = jax.lax.dot_general(xn, wq_p[...], NT_DIMS,
                                  preferred_element_type=F32)
        for j in range(NB):
            qkv[j, HALO:HALO + SUB, :] = res[:, j * LANES:(j + 1) * LANES]
        for i, j in enumerate(KV_BLOCKS):
            if first is False:
                qkv[j, 0:HALO, :] = tails[i]
                continue
            row0 = jnp.broadcast_to(res[0:1, j * LANES:(j + 1) * LANES],
                                    (HALO, LANES))
            if first is True:
                qkv[j, 0:HALO, :] = row0
            else:
                qkv[j, 0:HALO, :] = jnp.where(first, row0, tails[i])

    def attn_unit(qkv, p, r0, rb, masked):
        def load(j, w):
            return qkv[j, pl.ds(HALO + r0 - DIL * w, rb), :]

        q = [load(j, 0) for j in Q_BLOCKS]
        if masked:
            pos = (p * SUB + r0
                   + jax.lax.broadcasted_iota(jnp.int32, (rb, LANES), 0))
        logits = []
        for w in range(W):
            lg = q[0] * load(K_BLOCKS[0], w)
            for i in range(1, DB):
                lg = lg + q[i] * load(K_BLOCKS[i], w)
            lg = lg + pltpu.roll(lg, 64, 1)
            lg = lg + pltpu.roll(lg, 32, 1)
            if masked and w > 0:
                lg = jnp.where(pos >= DIL * w, lg, MASKED_LOGIT)
            logits.append(lg)
        m = logits[0]
        for w in range(1, W):
            m = jnp.maximum(m, logits[w])
        es = [jnp.exp2((lg - m) * EXP2_SCALE) for lg in logits]
        s = es[0]
        for w in range(1, W):
            s = s + es[w]
        r = 1.0 / s
        for i, j in enumerate(V_BLOCKS):
            o = es[0] * load(j, 0)
            for w in range(1, W):
                o = o + es[w] * load(j, w)
            o = o * r
            if i == DB - 1:
                lane = jax.lax.broadcasted_iota(jnp.int32, (rb, LANES), 1)
                o = jnp.where(lane >= 64, o, 0.0)
            qkv[O_BLOCKS[i], pl.ds(HALO + r0, rb), :] = o

    def attention(qkv, p, rb):
        for a in range(SUB // rb):
            masked = a * rb < (W - 1) * DIL and not (isinstance(p, int) and p > 0)
            r0 = pl.multiple_of(row_s[a * rb // 8], rb)
            attn_unit(qkv, p, r0, rb, masked)

    def out_proj(qkv, p, slot, row0):
        o = jnp.concatenate(
            [qkv[j, HALO:HALO + SUB, :].astype(BF16) for j in O_BLOCKS], axis=1)
        upd = jax.lax.dot_general(wo_pt[...], o, NT_DIMS,
                                  preferred_element_type=F32)
        x = xres[p] + upd
        xres[p] = x
        xn2[slot, pl.ds(row0, SUB), :] = _layernorm_t(x)

    def ffn_up(slot, c):
        xn = xn2[slot]
        g = jnp.dot(xn, wg[c], preferred_element_type=F32)
        u = jnp.dot(xn, wu[c], preferred_element_type=F32)
        return (g * u).astype(BF16)

    def ffn_down(h, t, c):
        res = jax.lax.dot_general(wd[c], h, NT_DIMS,
                                  preferred_element_type=F32)
        for i in range(NCH):
            xres[t * NCH + i] += res[:, i * SUB:(i + 1) * SUB]

    def load_x(t):
        for i in range(NCH):
            xres[t * NCH + i] = xin[t, :, i * SUB:(i + 1) * SUB].astype(F32)

    x_copy(0).start()
    for j in range(DB):
        wqkv_copy(j).start()
    wo_copy.start()
    for t in range(1, NT):
        x_copy(t).start()
    for c in range(NCH):
        for which in range(3):
            f_copy(which, c).start(priority=1)
    for a in range(SUB // 8):
        row_s[a] = a * 8
    wq_p[13 * LANES + 64:14 * LANES, :] = jnp.zeros((64, D), BF16)

    def ln1_pro(i):
        xn2[1, i * SUB:(i + 1) * SUB, :] = _layernorm_t(xres[i])

    def project_pro(i):
        project(xn2[1, i * SUB:(i + 1) * SUB, :], qkv_bufs[i],
                qkv_bufs[i - 1] if i else None, i == 0)

    with jax.named_scope("s_prep"):
        x_copy(0).wait()
        load_x(0)
        ln1_pro(0)
        for j in range(DB):
            wqkv_copy(j).wait()
            prep_wqkv(j)
        project_pro(0)
        for i in range(1, NCH):
            ln1_pro(i)
    barriers = ([wo_copy] + [x_copy(t) for t in range(1, NT)]
                + [f_copy(which, 0) for which in range(3)])
    with jax.named_scope("s_stage0"):
        for i in range(NCH + 1):
            barriers.pop(0).wait()
            if i > 0:
                out_proj(qkv_bufs[i - 1], i - 1, 0, (i - 1) * SUB)
            if i + 1 < NCH:
                project_pro(i + 1)
            if i < NCH:
                attention(qkv_bufs[i], i, RB0)
            if i == 0:
                prep_wo()
            elif i < NT:
                load_x(i)
            if i == NCH - 1:
                xn1[...] = _layernorm_t(xres[NCH])
        for cp in barriers:
            cp.wait()

    qkv = qkv_bufs[NCH - 1]
    n_main = 2 * NS - NCH

    def start_out(k):
        @pl.when(k > NS + NCH)
        def _():
            out_copy(k - NS - NCH - 1).start()

    def main(k, carry):
        n = _div(k, NCH)
        c = _mod(k, NCH)
        p = _mod(k + NCH, NS)
        start_out(k)

        project(xn1[...], qkv, qkv, p == 0)
        xn1[...] = _layernorm_t(xres[_mod(k + NCH + 1, NS)])
        pc = _mod(k + NS - NCH, NS)
        xout[pc] = xres[pc].astype(BF16)
        h = ffn_up(_mod(n, 2), c)
        attention(qkv, p, RB)
        out_proj(qkv, p, _mod(n + 1, 2), pl.multiple_of(c * SUB, SUB))
        ffn_down(h, _mod(n, NT), c)

        @pl.when(k + 1 < NCH)
        def _():
            for which in range(3):
                f_copy(which, k + 1).wait()
        return carry
    with jax.named_scope("s_main"):
        jax.lax.fori_loop(0, n_main, main, 0)

    def last(k, carry):
        c = _mod(k, NCH)
        start_out(k)
        pc = k - NS - NCH
        xout[pc] = xres[pc].astype(BF16)
        h = ffn_up((2 * NT - 1) % 2, c)
        ffn_down(h, NT - 1, c)
        return carry
    with jax.named_scope("s_last"):
        jax.lax.fori_loop(n_main, 2 * NS, last, 0)
    with jax.named_scope("s_tail"):
        out_copy(NS - NCH - 1).start()
        for p in range(NS - NCH, NS):
            xout[p] = xres[p].astype(BF16)
            out_copy(p).start()
        for p in range(NS):
            out_copy(p).wait()


@jax.jit
def pallas_interleave_layers__sliding_local_dilated__glu_gated_bilinear__prompt_kernel(
    A_x: jax.Array,
    A_wqkv: jax.Array,
    A_wo: jax.Array,
    B_x: jax.Array,
    B_w_gate: jax.Array,
    B_w_up: jax.Array,
    B_w_down: jax.Array,
):
    del B_x
    xT = A_x.reshape(S, D).T
    wdT = B_w_down.T
    any_spec = pl.BlockSpec(memory_space=pl.ANY)
    outT = pl.pallas_call(
        _kernel,
        in_specs=[any_spec] * 6,
        out_specs=any_spec,
        out_shape=jax.ShapeDtypeStruct((D, S), BF16),
        scratch_shapes=[
            pltpu.VMEM((NT, D, TM), BF16),
            pltpu.VMEM((NS, D, SUB), F32),
            pltpu.VMEM((NS, D, SUB), BF16),
            pltpu.VMEM((D, 3 * D), BF16),
            pltpu.VMEM((D, D), BF16),
            pltpu.VMEM((NCH, D, FC), BF16),
            pltpu.VMEM((NCH, D, FC), BF16),
            pltpu.VMEM((NCH, D, FC), BF16),
            pltpu.VMEM((DB, 3 * D, LANES), F32),
            pltpu.VMEM((NB * LANES, D), BF16),
            pltpu.VMEM((DB, D, LANES), F32),
            pltpu.VMEM((DB * LANES, D), F32),
            pltpu.VMEM((D, DB * LANES), BF16),
            pltpu.VMEM((SUB, D), BF16),
            pltpu.VMEM((2, TM, D), BF16),
            pltpu.SMEM((SUB // 8,), jnp.int32),
            pltpu.SemaphoreType.DMA((NT,)),
            pltpu.SemaphoreType.DMA((DB + 1,)),
            pltpu.SemaphoreType.DMA((3 * NCH,)),
            pltpu.SemaphoreType.DMA((NS,)),
        ] + [pltpu.VMEM((NB + 1, HALO + SUB, LANES), F32)] * NCH,
        compiler_params=pltpu.CompilerParams(
            vmem_limit_bytes=100 * 1024 * 1024),
    )(xT, A_wqkv, A_wo, B_w_gate, B_w_up, wdT)
    return outT.T.reshape(1, S, D)
```

```python
import jax
import jax.numpy as jnp
import jax.experimental.pallas as pl
import jax.experimental.pallas.tpu as pltpu

S = 2048
D = 576
F = 4608
H = 32
DH = 18
W = 8
DIL = 2
EPS = 1e-5
LANES = 128

TM = 512
NT = S // TM
FC = 1152
NCH = F // FC
SUB = TM // NCH
NS = S // SUB
RB = 8
RB0 = 16
HALO = 16
NB = 14
DB = 5

Q_BLOCKS = (0, 1, 2, 3, 12)
K_BLOCKS = (4, 5, 6, 7, 13)
V_BLOCKS = (8, 9, 10, 11, 12)
O_BLOCKS = (0, 1, 2, 3, 14)
KV_BLOCKS = (4, 5, 6, 7, 8, 9, 10, 11, 12, 13)

SCALE = DH ** -0.5
EXP2_SCALE = SCALE * 1.4426950408889634
MASKED_LOGIT = -1e9 / SCALE

NT_DIMS = (((1,), (1,)), ((), ()))
F32 = jnp.float32
BF16 = jnp.bfloat16


def _qkv_dest_row(part, d):
    if d < 16:
        return (part * 4 + d // 4) * LANES + (d % 4) * H
    base = (12 * LANES, 13 * LANES, 12 * LANES + 64)[part]
    return base + (d - 16) * H


def _o_dest_row(d):
    if d < 16:
        return d * H
    return 4 * LANES + 64 + (d - 16) * H


def _mod(a, n):
    assert n & (n - 1) == 0
    return jax.lax.bitwise_and(a, n - 1)


def _div(a, n):
    assert n & (n - 1) == 0
    return jax.lax.shift_right_logical(a, n.bit_length() - 1)


def _layernorm_t(x):
    m = jnp.mean(x, axis=0, keepdims=True)
    c = x - m
    v = jnp.mean(c * c, axis=0, keepdims=True)
    y = c * jax.lax.rsqrt(v + EPS)
    return y.astype(BF16).T


def _kernel(xT_hbm, wqkv_hbm, wo_hbm, wg_hbm, wu_hbm, wdT_hbm, out_hbm,
            xin, xres, xout, wqkv_raw, wo_raw, wg, wu, wd,
            wt_tmp, wq_p, wo_tmp, wo_p, wo_pt, ring, xn1, xn2, row_s,
            sem_x, sem_w, sem_f, sem_o, *qkv_bufs):

    def x_copy(t):
        return pltpu.make_async_copy(
            xT_hbm.at[:, pl.ds(t * TM, TM)], xin.at[t], sem_x.at[t])

    def f_copy(which, c):
        src = (wg_hbm, wu_hbm, wdT_hbm)[which]
        dst = (wg, wu, wd)[which]
        start = c * FC
        if not isinstance(c, int):
            start = pl.multiple_of(start, LANES)
        return pltpu.make_async_copy(
            src.at[:, pl.ds(start, FC)], dst.at[c], sem_f.at[which * NCH + c])

    def out_copy(p):
        start = p * SUB
        if not isinstance(p, int):
            start = pl.multiple_of(start, LANES)
        return pltpu.make_async_copy(
            xout.at[p], out_hbm.at[:, pl.ds(start, SUB)], sem_o.at[p])

    def wqkv_copy(j):
        rows = pl.ds(j * LANES, min(LANES, D - j * LANES))
        return pltpu.make_async_copy(
            wqkv_hbm.at[rows], wqkv_raw.at[rows], sem_w.at[j])

    wo_copy = pltpu.make_async_copy(wo_hbm, wo_raw, sem_w.at[DB])

    def prep_wqkv(j):
        n = min(LANES, D - j * LANES)
        blk = wqkv_raw[j * LANES:j * LANES + n, :].astype(F32)
        wt_tmp[j, :, 0:n] = blk.T
        for part in range(3):
            for d in range(DH):
                dst = _qkv_dest_row(part, d)
                val = wt_tmp[j, pl.ds(part * D + d, H, stride=DH), :]
                wq_p[dst:dst + H, j * LANES:j * LANES + n] = (
                    val[:, 0:n].astype(BF16))

    def prep_wo():
        for j in range(DB):
            cols = min(LANES, D - j * LANES)
            wo_tmp[j, :, 0:cols] = (
                wo_raw[:, j * LANES:j * LANES + cols].astype(F32))
        for d in range(DH):
            dst = _o_dest_row(d)
            for j in range(DB):
                cols = min(LANES, D - j * LANES)
                val = wo_tmp[j, pl.ds(d, H, stride=DH), :]
                wo_p[dst:dst + H, j * LANES:j * LANES + cols] = val[:, 0:cols]
        wo_p[4 * LANES:4 * LANES + 64, :] = jnp.zeros((64, D), F32)
        wo_pt[...] = wo_p[...].astype(BF16).T

    def project(xn, qkv, prev, first):
        tails = None
        if first is not True:
            tails = [prev[j, SUB:SUB + HALO, :] for j in KV_BLOCKS]
        res = jax.lax.dot_general(xn, wq_p[...], NT_DIMS,
                                  preferred_element_type=F32)
        for j in range(NB):
            qkv[j, HALO:HALO + SUB, :] = res[:, j * LANES:(j + 1) * LANES]
        for i, j in enumerate(KV_BLOCKS):
            if first is False:
                qkv[j, 0:HALO, :] = tails[i]
                continue
            row0 = jnp.broadcast_to(res[0:1, j * LANES:(j + 1) * LANES],
                                    (HALO, LANES))
            if first is True:
                qkv[j, 0:HALO, :] = row0
            else:
                qkv[j, 0:HALO, :] = jnp.where(first, row0, tails[i])

    def attn_unit(qkv, p, r0, rb, masked):
        def load(j, w):
            return qkv[j, pl.ds(HALO + r0 - DIL * w, rb), :]

        q = [load(j, 0) for j in Q_BLOCKS]
        if masked:
            pos = (p * SUB + r0
                   + jax.lax.broadcasted_iota(jnp.int32, (rb, LANES), 0))
        logits = []
        for w in range(W):
            lg = q[0] * load(K_BLOCKS[0], w)
            for i in range(1, DB):
                lg = lg + q[i] * load(K_BLOCKS[i], w)
            lg = lg + pltpu.roll(lg, 64, 1)
            lg = lg + pltpu.roll(lg, 32, 1)
            if masked and w > 0:
                lg = jnp.where(pos >= DIL * w, lg, MASKED_LOGIT)
            logits.append(lg)
        m = logits[0]
        for w in range(1, W):
            m = jnp.maximum(m, logits[w])
        es = [jnp.exp2((lg - m) * EXP2_SCALE) for lg in logits]
        s = es[0]
        for w in range(1, W):
            s = s + es[w]
        r = 1.0 / s
        for i, j in enumerate(V_BLOCKS):
            o = es[0] * load(j, 0)
            for w in range(1, W):
                o = o + es[w] * load(j, w)
            o = o * r
            if i == DB - 1:
                lane = jax.lax.broadcasted_iota(jnp.int32, (rb, LANES), 1)
                o = jnp.where(lane >= 64, o, 0.0)
            qkv[O_BLOCKS[i], pl.ds(HALO + r0, rb), :] = o

    def attention(qkv, p, rb):
        for a in range(SUB // rb):
            masked = a * rb < (W - 1) * DIL and not (isinstance(p, int) and p > 0)
            r0 = pl.multiple_of(row_s[a * rb // 8], rb)
            attn_unit(qkv, p, r0, rb, masked)

    def out_proj(qkv, p, slot, row0):
        o = jnp.concatenate(
            [qkv[j, HALO:HALO + SUB, :].astype(BF16) for j in O_BLOCKS], axis=1)
        upd = jax.lax.dot_general(wo_pt[...], o, NT_DIMS,
                                  preferred_element_type=F32)
        x = xres[p] + upd
        xres[p] = x
        xn2[slot, pl.ds(row0, SUB), :] = _layernorm_t(x)

    def ffn_up(slot, c):
        xn = xn2[slot]
        g = jnp.dot(xn, wg[c], preferred_element_type=F32)
        u = jnp.dot(xn, wu[c], preferred_element_type=F32)
        return (g * u).astype(BF16)

    def ffn_down(h, t, c):
        res = jax.lax.dot_general(wd[c], h, NT_DIMS,
                                  preferred_element_type=F32)
        for i in range(NCH):
            xres[t * NCH + i] += res[:, i * SUB:(i + 1) * SUB]

    def load_x(t):
        for i in range(NCH):
            xres[t * NCH + i] = xin[t, :, i * SUB:(i + 1) * SUB].astype(F32)

    x_copy(0).start()
    for j in range(DB):
        wqkv_copy(j).start()
    wo_copy.start()
    for t in range(1, NT):
        x_copy(t).start()
    for c in range(NCH):
        for which in range(3):
            f_copy(which, c).start(priority=1)
    for a in range(SUB // 8):
        row_s[a] = a * 8
    wq_p[13 * LANES + 64:14 * LANES, :] = jnp.zeros((64, D), BF16)

    def buf(j):
        return qkv_bufs[j] if j < NCH else ring.at[j - NCH]

    def ln1_pro(j):
        xn1[j] = _layernorm_t(xres[j])

    def project_pro(j):
        project(xn1[j], buf(j), buf(j - 1) if j else None, j == 0)

    with jax.named_scope("s_prep"):
        x_copy(0).wait()
        load_x(0)
        ln1_pro(0)
        for j in range(DB):
            wqkv_copy(j).wait()
            prep_wqkv(j)
        project_pro(0)
        for j in range(1, NCH):
            ln1_pro(j)
        project_pro(1)
    with jax.named_scope("s_stage0"):
        wo_copy.wait()
        for t in range(1, NT):
            x_copy(t).wait()
        project_pro(2)
        attention(buf(0), 0, RB0)
        load_x(1)
        prep_wo()
        project_pro(3)
        attention(buf(1), 1, RB0)
        for j in range(NCH, 2 * NCH):
            ln1_pro(j)
        project_pro(4)
        attention(buf(2), 2, RB0)
        out_proj(buf(0), 0, 0, 0)
        project_pro(5)
        attention(buf(3), 3, RB0)
        out_proj(buf(1), 1, 0, SUB)
        load_x(2)
        project_pro(6)
        out_proj(buf(2), 2, 0, 2 * SUB)
        out_proj(buf(3), 3, 0, 3 * SUB)
        load_x(3)
        project_pro(7)
        for which in range(3):
            f_copy(which, 0).wait()

    def start_out(k):
        @pl.when(k > NS + NCH)
        def _():
            out_copy(k - NS - NCH - 1).start()

    def body(k, do_attn, do_proj):
        n = _div(k, NCH)
        c = _mod(k, NCH)
        start_out(k)
        if do_proj:
            pj = _mod(k + 2 * NCH, NS)
            xn1[0] = _layernorm_t(xres[pj])
        pc = _mod(k + NS - NCH, NS)
        xout[pc] = xres[pc].astype(BF16)
        h = ffn_up(_mod(n, 2), c)
        if do_attn:
            p = _mod(k + NCH, NS)
            attention(ring.at[c], p, RB)
            out_proj(ring.at[c], p, _mod(n + 1, 2),
                     pl.multiple_of(c * SUB, SUB))
        if do_proj:
            project(xn1[0], ring.at[c], ring.at[_mod(c + NCH - 1, NCH)],
                    pj == 0)
        ffn_down(h, _mod(n, NT), c)
        if do_proj:
            @pl.when(k + 1 < NCH)
            def _():
                for which in range(3):
                    f_copy(which, k + 1).wait()

    def loop(lo, hi, do_attn, do_proj):
        def step(k, carry):
            body(k, do_attn, do_proj)
            return carry
        jax.lax.fori_loop(lo, hi, step, 0)

    with jax.named_scope("s_main"):
        loop(0, 2 * NS - 2 * NCH, True, True)
    with jax.named_scope("s_mid"):
        loop(2 * NS - 2 * NCH, 2 * NS - NCH, True, False)
    with jax.named_scope("s_last"):
        loop(2 * NS - NCH, 2 * NS, False, False)
    with jax.named_scope("s_tail"):
        out_copy(NS - NCH - 1).start()
        for p in range(NS - NCH, NS):
            xout[p] = xres[p].astype(BF16)
            out_copy(p).start()
        for p in range(NS):
            out_copy(p).wait()


@jax.jit
def pallas_interleave_layers__sliding_local_dilated__glu_gated_bilinear__prompt_kernel(
    A_x: jax.Array,
    A_wqkv: jax.Array,
    A_wo: jax.Array,
    B_x: jax.Array,
    B_w_gate: jax.Array,
    B_w_up: jax.Array,
    B_w_down: jax.Array,
):
    del B_x
    xT = A_x.reshape(S, D).T
    wdT = B_w_down.T
    any_spec = pl.BlockSpec(memory_space=pl.ANY)
    outT = pl.pallas_call(
        _kernel,
        in_specs=[any_spec] * 6,
        out_specs=any_spec,
        out_shape=jax.ShapeDtypeStruct((D, S), BF16),
        scratch_shapes=[
            pltpu.VMEM((NT, D, TM), BF16),
            pltpu.VMEM((NS, D, SUB), F32),
            pltpu.VMEM((NS, D, SUB), BF16),
            pltpu.VMEM((D, 3 * D), BF16),
            pltpu.VMEM((D, D), BF16),
            pltpu.VMEM((NCH, D, FC), BF16),
            pltpu.VMEM((NCH, D, FC), BF16),
            pltpu.VMEM((NCH, D, FC), BF16),
            pltpu.VMEM((DB, 3 * D, LANES), F32),
            pltpu.VMEM((NB * LANES, D), BF16),
            pltpu.VMEM((DB, D, LANES), F32),
            pltpu.VMEM((DB * LANES, D), F32),
            pltpu.VMEM((D, DB * LANES), BF16),
            pltpu.VMEM((NCH, NB + 1, HALO + SUB, LANES), F32),
            pltpu.VMEM((2 * NCH, SUB, D), BF16),
            pltpu.VMEM((2, TM, D), BF16),
            pltpu.SMEM((SUB // 8,), jnp.int32),
            pltpu.SemaphoreType.DMA((NT,)),
            pltpu.SemaphoreType.DMA((DB + 1,)),
            pltpu.SemaphoreType.DMA((3 * NCH,)),
            pltpu.SemaphoreType.DMA((NS,)),
        ] + [pltpu.VMEM((NB + 1, HALO + SUB, LANES), F32)] * NCH,
        compiler_params=pltpu.CompilerParams(
            vmem_limit_bytes=100 * 1024 * 1024),
    )(xT, A_wqkv, A_wo, B_w_gate, B_w_up, wdT)
    return outT.T.reshape(1, S, D)
```

```python
import jax
import jax.numpy as jnp
import jax.experimental.pallas as pl
import jax.experimental.pallas.tpu as pltpu

S = 2048
D = 576
F = 4608
H = 32
DH = 18
W = 8
DIL = 2
EPS = 1e-5
LANES = 128

TM = 512
NT = S // TM
FC = 1152
NCH = F // FC
SUB = TM // NCH
NS = S // SUB
RB = 8
RB0 = 16
HALO = 16
NB = 14
DB = 5

Q_BLOCKS = (0, 1, 2, 3, 12)
K_BLOCKS = (4, 5, 6, 7, 13)
V_BLOCKS = (8, 9, 10, 11, 12)
O_BLOCKS = (0, 1, 2, 3, 14)
KV_BLOCKS = (4, 5, 6, 7, 8, 9, 10, 11, 12, 13)

SCALE = DH ** -0.5
EXP2_SCALE = SCALE * 1.4426950408889634
MASKED_LOGIT = -1e9 / SCALE

NT_DIMS = (((1,), (1,)), ((), ()))
F32 = jnp.float32
BF16 = jnp.bfloat16


def _qkv_dest_row(part, d):
    if d < 16:
        return (part * 4 + d // 4) * LANES + (d % 4) * H
    base = (12 * LANES, 13 * LANES, 12 * LANES + 64)[part]
    return base + (d - 16) * H


def _o_dest_row(d):
    if d < 16:
        return d * H
    return 4 * LANES + 64 + (d - 16) * H


def _mod(a, n):
    assert n & (n - 1) == 0
    return jax.lax.bitwise_and(a, n - 1)


def _div(a, n):
    assert n & (n - 1) == 0
    return jax.lax.shift_right_logical(a, n.bit_length() - 1)


def _layernorm_t(x):
    m = jnp.mean(x, axis=0, keepdims=True)
    c = x - m
    v = jnp.mean(c * c, axis=0, keepdims=True)
    y = c * jax.lax.rsqrt(v + EPS)
    return y.astype(BF16).T


def _kernel(xT_hbm, wqkv_hbm, wo_hbm, wg_hbm, wu_hbm, wdT_hbm, out_hbm,
            xin, xres, xout, wqkv_raw, wo_raw, wg, wu, wd,
            wt_tmp, wq_p, wo_tmp, wo_p, wo_pt, ring, xn1, xn2, row_s,
            sem_in, sem_o, *qkv_bufs):

    def x_copy(t):
        return pltpu.make_async_copy(
            xT_hbm.at[:, pl.ds(t * TM, TM)], xin.at[t], sem_in.at[t])

    def f_copy(which, c):
        src = (wg_hbm, wu_hbm, wdT_hbm)[which]
        dst = (wg, wu, wd)[which]
        start = c * FC
        if not isinstance(c, int):
            start = pl.multiple_of(start, LANES)
        return pltpu.make_async_copy(
            src.at[:, pl.ds(start, FC)], dst.at[c],
            sem_in.at[NT + DB + 1 + which * NCH + c])

    def out_copy(p):
        start = p * SUB
        if not isinstance(p, int):
            start = pl.multiple_of(start, LANES)
        return pltpu.make_async_copy(
            xout.at[p], out_hbm.at[:, pl.ds(start, SUB)], sem_o.at[p])

    def wqkv_copy(j):
        rows = pl.ds(j * LANES, min(LANES, D - j * LANES))
        return pltpu.make_async_copy(
            wqkv_hbm.at[rows], wqkv_raw.at[rows], sem_in.at[NT + j])

    wo_copy = pltpu.make_async_copy(wo_hbm, wo_raw, sem_in.at[NT + DB])

    def prep_wqkv(j):
        n = min(LANES, D - j * LANES)
        blk = wqkv_raw[j * LANES:j * LANES + n, :].astype(F32)
        wt_tmp[j, :, 0:n] = blk.T
        for part in range(3):
            for d in range(DH):
                dst = _qkv_dest_row(part, d)
                val = wt_tmp[j, pl.ds(part * D + d, H, stride=DH), :]
                wq_p[dst:dst + H, j * LANES:j * LANES + n] = (
                    val[:, 0:n].astype(BF16))

    def prep_wo():
        for j in range(DB):
            cols = min(LANES, D - j * LANES)
            wo_tmp[j, :, 0:cols] = (
                wo_raw[:, j * LANES:j * LANES + cols].astype(F32))
        for d in range(DH):
            dst = _o_dest_row(d)
            for j in range(DB):
                cols = min(LANES, D - j * LANES)
                val = wo_tmp[j, pl.ds(d, H, stride=DH), :]
                wo_p[dst:dst + H, j * LANES:j * LANES + cols] = val[:, 0:cols]
        wo_p[4 * LANES:4 * LANES + 64, :] = jnp.zeros((64, D), F32)
        wo_pt[...] = wo_p[...].astype(BF16).T

    def project(xn, qkv, prev, first):
        tails = None
        if first is not True:
            tails = [prev[j, SUB:SUB + HALO, :] for j in KV_BLOCKS]
        res = jax.lax.dot_general(xn, wq_p[...], NT_DIMS,
                                  preferred_element_type=F32)
        for j in range(NB):
            qkv[j, HALO:HALO + SUB, :] = res[:, j * LANES:(j + 1) * LANES]
        for i, j in enumerate(KV_BLOCKS):
            if first is False:
                qkv[j, 0:HALO, :] = tails[i]
                continue
            row0 = jnp.broadcast_to(res[0:1, j * LANES:(j + 1) * LANES],
                                    (HALO, LANES))
            if first is True:
                qkv[j, 0:HALO, :] = row0
            else:
                qkv[j, 0:HALO, :] = jnp.where(first, row0, tails[i])

    def attn_unit(qkv, p, r0, rb, masked):
        def load(j, w):
            return qkv[j, pl.ds(HALO + r0 - DIL * w, rb), :]

        q = [load(j, 0) for j in Q_BLOCKS]
        if masked:
            pos = (p * SUB + r0
                   + jax.lax.broadcasted_iota(jnp.int32, (rb, LANES), 0))
        logits = []
        for w in range(W):
            lg = q[0] * load(K_BLOCKS[0], w)
            for i in range(1, DB):
                lg = lg + q[i] * load(K_BLOCKS[i], w)
            lg = lg + pltpu.roll(lg, 64, 1)
            lg = lg + pltpu.roll(lg, 32, 1)
            if masked and w > 0:
                lg = jnp.where(pos >= DIL * w, lg, MASKED_LOGIT)
            logits.append(lg)
        m = logits[0]
        for w in range(1, W):
            m = jnp.maximum(m, logits[w])
        es = [jnp.exp2((lg - m) * EXP2_SCALE) for lg in logits]
        s = es[0]
        for w in range(1, W):
            s = s + es[w]
        r = 1.0 / s
        for i, j in enumerate(V_BLOCKS):
            o = es[0] * load(j, 0)
            for w in range(1, W):
                o = o + es[w] * load(j, w)
            o = o * r
            if i == DB - 1:
                lane = jax.lax.broadcasted_iota(jnp.int32, (rb, LANES), 1)
                o = jnp.where(lane >= 64, o, 0.0)
            qkv[O_BLOCKS[i], pl.ds(HALO + r0, rb), :] = o

    def attention(qkv, p, rb):
        for a in range(SUB // rb):
            masked = a * rb < (W - 1) * DIL and not (isinstance(p, int) and p > 0)
            r0 = pl.multiple_of(row_s[a * rb // 8], rb)
            attn_unit(qkv, p, r0, rb, masked)

    def out_proj(qkv, p, slot, row0):
        o = jnp.concatenate(
            [qkv[j, HALO:HALO + SUB, :].astype(BF16) for j in O_BLOCKS], axis=1)
        upd = jax.lax.dot_general(wo_pt[...], o, NT_DIMS,
                                  preferred_element_type=F32)
        x = xres[p] + upd
        xres[p] = x
        xn2[slot, pl.ds(row0, SUB), :] = _layernorm_t(x)

    def ffn_up(slot, c):
        xn = xn2[slot]
        g = jnp.dot(xn, wg[c], preferred_element_type=F32)
        u = jnp.dot(xn, wu[c], preferred_element_type=F32)
        return (g * u).astype(BF16)

    def ffn_down(h, t, c):
        res = jax.lax.dot_general(wd[c], h, NT_DIMS,
                                  preferred_element_type=F32)
        for i in range(NCH):
            xres[t * NCH + i] += res[:, i * SUB:(i + 1) * SUB]

    def load_x(t):
        for i in range(NCH):
            xres[t * NCH + i] = xin[t, :, i * SUB:(i + 1) * SUB].astype(F32)

    x_copy(0).start()
    for j in range(DB):
        wqkv_copy(j).start()
    wo_copy.start()
    for t in range(1, NT):
        x_copy(t).start()
    for c in range(NCH):
        for which in range(3):
            f_copy(which, c).start()
    for a in range(SUB // 8):
        row_s[a] = a * 8
    wq_p[13 * LANES + 64:14 * LANES, :] = jnp.zeros((64, D), BF16)

    def buf(j):
        return qkv_bufs[j] if j < NCH else ring.at[j - NCH]

    def ln1_pro(j):
        xn1[j] = _layernorm_t(xres[j])

    def project_pro(j):
        project(xn1[j], buf(j), buf(j - 1) if j else None, j == 0)

    with jax.named_scope("s_prep"):
        x_copy(0).wait()
        load_x(0)
        ln1_pro(0)
        for j in range(DB):
            wqkv_copy(j).wait()
            prep_wqkv(j)
        project_pro(0)
        for j in range(1, NCH):
            ln1_pro(j)
        project_pro(1)
    with jax.named_scope("s_stage0"):
        wo_copy.wait()
        for t in range(1, NT):
            x_copy(t).wait()
        project_pro(2)
        attention(buf(0), 0, RB0)
        load_x(1)
        prep_wo()
        project_pro(3)
        attention(buf(1), 1, RB0)
        for j in range(NCH, 2 * NCH):
            ln1_pro(j)
        project_pro(4)
        attention(buf(2), 2, RB0)
        out_proj(buf(0), 0, 0, 0)
        project_pro(5)
        attention(buf(3), 3, RB0)
        out_proj(buf(1), 1, 0, SUB)
        load_x(2)
        project_pro(6)
        out_proj(buf(2), 2, 0, 2 * SUB)
        out_proj(buf(3), 3, 0, 3 * SUB)
        load_x(3)
        project_pro(7)
        for which in range(3):
            f_copy(which, 0).wait()

    def start_out(k):
        @pl.when(k > NS + NCH)
        def _():
            out_copy(k - NS - NCH - 1).start()

    def body(k, do_attn, do_proj):
        n = _div(k, NCH)
        c = _mod(k, NCH)
        start_out(k)
        if do_proj:
            pj = _mod(k + 2 * NCH, NS)
            xn1[0] = _layernorm_t(xres[pj])
        pc = _mod(k + NS - NCH, NS)
        xout[pc] = xres[pc].astype(BF16)
        h = ffn_up(_mod(n, 2), c)
        if do_attn:
            p = _mod(k + NCH, NS)
            attention(ring.at[c], p, RB)
            out_proj(ring.at[c], p, _mod(n + 1, 2),
                     pl.multiple_of(c * SUB, SUB))
        if do_proj:
            project(xn1[0], ring.at[c], ring.at[_mod(c + NCH - 1, NCH)],
                    pj == 0)
        ffn_down(h, _mod(n, NT), c)
        if do_proj:
            @pl.when(k + 1 < NCH)
            def _():
                for which in range(3):
                    f_copy(which, k + 1).wait()

    def loop(lo, hi, do_attn, do_proj):
        def step(k, carry):
            body(k, do_attn, do_proj)
            return carry
        jax.lax.fori_loop(lo, hi, step, 0)

    with jax.named_scope("s_main"):
        loop(0, 2 * NS - 2 * NCH, True, True)
    with jax.named_scope("s_mid"):
        loop(2 * NS - 2 * NCH, 2 * NS - NCH, True, False)
    with jax.named_scope("s_last"):
        loop(2 * NS - NCH, 2 * NS, False, False)
    with jax.named_scope("s_tail"):
        out_copy(NS - NCH - 1).start()
        for p in range(NS - NCH, NS):
            xout[p] = xres[p].astype(BF16)
            out_copy(p).start()
        for p in range(NS):
            out_copy(p).wait()


@jax.jit
def pallas_interleave_layers__sliding_local_dilated__glu_gated_bilinear__prompt_kernel(
    A_x: jax.Array,
    A_wqkv: jax.Array,
    A_wo: jax.Array,
    B_x: jax.Array,
    B_w_gate: jax.Array,
    B_w_up: jax.Array,
    B_w_down: jax.Array,
):
    del B_x
    xT = A_x.reshape(S, D).T
    wdT = B_w_down.T
    any_spec = pl.BlockSpec(memory_space=pl.ANY)
    outT = pl.pallas_call(
        _kernel,
        in_specs=[any_spec] * 6,
        out_specs=any_spec,
        out_shape=jax.ShapeDtypeStruct((D, S), BF16),
        scratch_shapes=[
            pltpu.VMEM((NT, D, TM), BF16),
            pltpu.VMEM((NS, D, SUB), F32),
            pltpu.VMEM((NS, D, SUB), BF16),
            pltpu.VMEM((D, 3 * D), BF16),
            pltpu.VMEM((D, D), BF16),
            pltpu.VMEM((NCH, D, FC), BF16),
            pltpu.VMEM((NCH, D, FC), BF16),
            pltpu.VMEM((NCH, D, FC), BF16),
            pltpu.VMEM((DB, 3 * D, LANES), F32),
            pltpu.VMEM((NB * LANES, D), BF16),
            pltpu.VMEM((DB, D, LANES), F32),
            pltpu.VMEM((DB * LANES, D), F32),
            pltpu.VMEM((D, DB * LANES), BF16),
            pltpu.VMEM((NCH, NB + 1, HALO + SUB, LANES), F32),
            pltpu.VMEM((2 * NCH, SUB, D), BF16),
            pltpu.VMEM((2, TM, D), BF16),
            pltpu.SMEM((SUB // 8,), jnp.int32),
            pltpu.SemaphoreType.DMA((NT + DB + 1 + 3 * NCH,)),
            pltpu.SemaphoreType.DMA((NS,)),
        ] + [pltpu.VMEM((NB + 1, HALO + SUB, LANES), F32)] * NCH,
        compiler_params=pltpu.CompilerParams(
            vmem_limit_bytes=100 * 1024 * 1024),
    )(xT, A_wqkv, A_wo, B_w_gate, B_w_up, wdT)
    return outT.T.reshape(1, S, D)
```

```python
import jax
import jax.numpy as jnp
import jax.experimental.pallas as pl
import jax.experimental.pallas.tpu as pltpu

S = 2048
D = 576
F = 4608
H = 32
DH = 18
W = 8
DIL = 2
EPS = 1e-5
LANES = 128

TM = 512
NT = S // TM
FC = 1152
NCH = F // FC
SUB = TM // NCH
NS = S // SUB
RB = 8
RB0 = 16
HALO = 16
NB = 14
DB = 5

Q_BLOCKS = (0, 1, 2, 3, 12)
K_BLOCKS = (4, 5, 6, 7, 13)
V_BLOCKS = (8, 9, 10, 11, 12)
O_BLOCKS = (0, 1, 2, 3, 14)
KV_BLOCKS = (4, 5, 6, 7, 8, 9, 10, 11, 12, 13)

SCALE = DH ** -0.5
EXP2_SCALE = SCALE * 1.4426950408889634
MASKED_LOGIT = -1e9 / SCALE

NT_DIMS = (((1,), (1,)), ((), ()))
F32 = jnp.float32
BF16 = jnp.bfloat16


def _qkv_dest_row(part, d):
    if d < 16:
        return (part * 4 + d // 4) * LANES + (d % 4) * H
    base = (12 * LANES, 13 * LANES, 12 * LANES + 64)[part]
    return base + (d - 16) * H


def _o_dest_row(d):
    if d < 16:
        return d * H
    return 4 * LANES + 64 + (d - 16) * H


def _mod(a, n):
    assert n & (n - 1) == 0
    return jax.lax.bitwise_and(a, n - 1)


def _div(a, n):
    assert n & (n - 1) == 0
    return jax.lax.shift_right_logical(a, n.bit_length() - 1)


def _layernorm_t(x):
    m = jnp.mean(x, axis=0, keepdims=True)
    c = x - m
    v = jnp.mean(c * c, axis=0, keepdims=True)
    y = c * jax.lax.rsqrt(v + EPS)
    return y.astype(BF16).T


def _kernel(xT_hbm, wqkv_hbm, wo_hbm, wg_hbm, wu_hbm, wdT_hbm, out_hbm,
            xin, xres, xout, wqkv_raw, wo_raw, wg, wu, wd,
            wt_tmp, wq_p, wo_tmp, wo_p, wo_pt, ring, xn1, xn2, row_s,
            sem_in, sem_o, *qkv_bufs):

    def x_copy(t):
        return pltpu.make_async_copy(
            xT_hbm.at[:, pl.ds(t * TM, TM)], xin.at[t], sem_in.at[t])

    def f_copy(which, c):
        src = (wg_hbm, wu_hbm, wdT_hbm)[which]
        dst = (wg, wu, wd)[which]
        start = c * FC
        if not isinstance(c, int):
            start = pl.multiple_of(start, LANES)
        return pltpu.make_async_copy(
            src.at[:, pl.ds(start, FC)], dst.at[c],
            sem_in.at[NT + DB + 1 + which * NCH + c])

    def out_copy(p):
        start = p * SUB
        if not isinstance(p, int):
            start = pl.multiple_of(start, LANES)
        return pltpu.make_async_copy(
            xout.at[p], out_hbm.at[:, pl.ds(start, SUB)], sem_o.at[p])

    def wqkv_copy(j):
        rows = pl.ds(j * LANES, min(LANES, D - j * LANES))
        return pltpu.make_async_copy(
            wqkv_hbm.at[rows], wqkv_raw.at[rows], sem_in.at[NT + j])

    wo_copy = pltpu.make_async_copy(wo_hbm, wo_raw, sem_in.at[NT + DB])

    def prep_wqkv(j):
        n = min(LANES, D - j * LANES)
        blk = wqkv_raw[j * LANES:j * LANES + n, :].astype(F32)
        wt_tmp[j, :, 0:n] = blk.T
        for part in range(3):
            for d in range(DH):
                dst = _qkv_dest_row(part, d)
                val = wt_tmp[j, pl.ds(part * D + d, H, stride=DH), :]
                wq_p[dst:dst + H, j * LANES:j * LANES + n] = (
                    val[:, 0:n].astype(BF16))

    def prep_wo():
        for j in range(DB):
            cols = min(LANES, D - j * LANES)
            wo_tmp[j, :, 0:cols] = (
                wo_raw[:, j * LANES:j * LANES + cols].astype(F32))
        for d in range(DH):
            dst = _o_dest_row(d)
            for j in range(DB):
                cols = min(LANES, D - j * LANES)
                val = wo_tmp[j, pl.ds(d, H, stride=DH), :]
                wo_p[dst:dst + H, j * LANES:j * LANES + cols] = val[:, 0:cols]
        wo_p[4 * LANES:4 * LANES + 64, :] = jnp.zeros((64, D), F32)
        wo_pt[...] = wo_p[...].astype(BF16).T

    def project(xn, qkv, prev, first):
        tails = None
        if first is not True:
            tails = [prev[j, SUB:SUB + HALO, :] for j in KV_BLOCKS]
        res = jax.lax.dot_general(xn, wq_p[...], NT_DIMS,
                                  preferred_element_type=F32)
        for j in range(NB):
            qkv[j, HALO:HALO + SUB, :] = res[:, j * LANES:(j + 1) * LANES]
        for i, j in enumerate(KV_BLOCKS):
            if first is False:
                qkv[j, 0:HALO, :] = tails[i]
                continue
            row0 = jnp.broadcast_to(res[0:1, j * LANES:(j + 1) * LANES],
                                    (HALO, LANES))
            if first is True:
                qkv[j, 0:HALO, :] = row0
            else:
                qkv[j, 0:HALO, :] = jnp.where(first, row0, tails[i])

    def attn_unit(qkv, p, r0, rb, masked):
        def load(j, w):
            return qkv[j, pl.ds(HALO + r0 - DIL * w, rb), :]

        q = [load(j, 0) for j in Q_BLOCKS]
        if masked:
            pos = (p * SUB + r0
                   + jax.lax.broadcasted_iota(jnp.int32, (rb, LANES), 0))
        logits = []
        for w in range(W):
            lg = q[0] * load(K_BLOCKS[0], w)
            for i in range(1, DB):
                lg = lg + q[i] * load(K_BLOCKS[i], w)
            lg = lg + pltpu.roll(lg, 64, 1)
            lg = lg + pltpu.roll(lg, 32, 1)
            if masked and w > 0:
                lg = jnp.where(pos >= DIL * w, lg, MASKED_LOGIT)
            logits.append(lg)
        m = logits[0]
        for w in range(1, W):
            m = jnp.maximum(m, logits[w])
        es = [jnp.exp2((lg - m) * EXP2_SCALE) for lg in logits]
        s = es[0]
        for w in range(1, W):
            s = s + es[w]
        r = 1.0 / s
        for i, j in enumerate(V_BLOCKS):
            o = es[0] * load(j, 0)
            for w in range(1, W):
                o = o + es[w] * load(j, w)
            o = o * r
            if i == DB - 1:
                lane = jax.lax.broadcasted_iota(jnp.int32, (rb, LANES), 1)
                o = jnp.where(lane >= 64, o, 0.0)
            qkv[O_BLOCKS[i], pl.ds(HALO + r0, rb), :] = o

    def attention(qkv, p, rb):
        for a in range(SUB // rb):
            masked = a * rb < (W - 1) * DIL and not (isinstance(p, int) and p > 0)
            r0 = pl.multiple_of(row_s[a * rb // 8], rb)
            attn_unit(qkv, p, r0, rb, masked)

    def out_proj(qkv, p, slot, row0):
        o = jnp.concatenate(
            [qkv[j, HALO:HALO + SUB, :].astype(BF16) for j in O_BLOCKS], axis=1)
        upd = jax.lax.dot_general(wo_pt[...], o, NT_DIMS,
                                  preferred_element_type=F32)
        x = xres[p] + upd
        xres[p] = x
        xn2[slot, pl.ds(row0, SUB), :] = _layernorm_t(x)

    def ffn_up(slot, c):
        xn = xn2[slot]
        g = jnp.dot(xn, wg[c], preferred_element_type=F32)
        u = jnp.dot(xn, wu[c], preferred_element_type=F32)
        return (g * u).astype(BF16)

    def ffn_down(h, t, c):
        res = jax.lax.dot_general(wd[c], h, NT_DIMS,
                                  preferred_element_type=F32)
        for i in range(NCH):
            x = xres[t * NCH + i] + res[:, i * SUB:(i + 1) * SUB]
            xres[t * NCH + i] = x
            xout[t * NCH + i] = x.astype(BF16)

    def load_x(t):
        for i in range(NCH):
            xres[t * NCH + i] = xin[t, :, i * SUB:(i + 1) * SUB].astype(F32)

    x_copy(0).start()
    for j in range(DB):
        wqkv_copy(j).start()
    wo_copy.start()
    for t in range(1, NT):
        x_copy(t).start()
    for c in range(NCH):
        for which in range(3):
            f_copy(which, c).start()
    for a in range(SUB // 8):
        row_s[a] = a * 8
    wq_p[13 * LANES + 64:14 * LANES, :] = jnp.zeros((64, D), BF16)

    def buf(j):
        return qkv_bufs[j] if j < NCH else ring.at[j - NCH]

    def ln1_pro(j):
        xn1[j] = _layernorm_t(xres[j])

    def project_pro(j):
        project(xn1[j], buf(j), buf(j - 1) if j else None, j == 0)

    with jax.named_scope("s_prep"):
        x_copy(0).wait()
        load_x(0)
        ln1_pro(0)
        for j in range(DB):
            wqkv_copy(j).wait()
            prep_wqkv(j)
        project_pro(0)
        for j in range(1, NCH):
            ln1_pro(j)
        project_pro(1)
    with jax.named_scope("s_stage0"):
        wo_copy.wait()
        for t in range(1, NT):
            x_copy(t).wait()
        project_pro(2)
        attention(buf(0), 0, RB0)
        load_x(1)
        prep_wo()
        project_pro(3)
        attention(buf(1), 1, RB0)
        for j in range(NCH, 2 * NCH):
            ln1_pro(j)
        project_pro(4)
        attention(buf(2), 2, RB0)
        out_proj(buf(0), 0, 0, 0)
        project_pro(5)
        attention(buf(3), 3, RB0)
        out_proj(buf(1), 1, 0, SUB)
        load_x(2)
        project_pro(6)
        out_proj(buf(2), 2, 0, 2 * SUB)
        out_proj(buf(3), 3, 0, 3 * SUB)
        load_x(3)
        project_pro(7)
        for which in range(3):
            f_copy(which, 0).wait()

    def start_out(k):
        @pl.when(k >= NS + NCH)
        def _():
            out_copy(k - NS - NCH).start()

    def body(k, do_attn, do_proj):
        n = _div(k, NCH)
        c = _mod(k, NCH)
        start_out(k)
        if do_proj:
            pj = _mod(k + 2 * NCH, NS)
            xn1[0] = _layernorm_t(xres[pj])
        h = ffn_up(_mod(n, 2), c)
        if do_attn:
            p = _mod(k + NCH, NS)
            attention(ring.at[c], p, RB)
            out_proj(ring.at[c], p, _mod(n + 1, 2),
                     pl.multiple_of(c * SUB, SUB))
        if do_proj:
            project(xn1[0], ring.at[c], ring.at[_mod(c + NCH - 1, NCH)],
                    pj == 0)
        ffn_down(h, _mod(n, NT), c)
        if do_proj:
            @pl.when(k + 1 < NCH)
            def _():
                for which in range(3):
                    f_copy(which, k + 1).wait()

    def loop(lo, hi, do_attn, do_proj):
        def step(k, carry):
            body(k, do_attn, do_proj)
            return carry
        jax.lax.fori_loop(lo, hi, step, 0)

    with jax.named_scope("s_main"):
        loop(0, 2 * NS - 2 * NCH, True, True)
    with jax.named_scope("s_mid"):
        loop(2 * NS - 2 * NCH, 2 * NS - NCH, True, False)
    with jax.named_scope("s_last"):
        loop(2 * NS - NCH, 2 * NS, False, False)
    with jax.named_scope("s_tail"):
        for p in range(NS - NCH, NS):
            out_copy(p).start()
        for p in range(NS):
            out_copy(p).wait()


@jax.jit
def pallas_interleave_layers__sliding_local_dilated__glu_gated_bilinear__prompt_kernel(
    A_x: jax.Array,
    A_wqkv: jax.Array,
    A_wo: jax.Array,
    B_x: jax.Array,
    B_w_gate: jax.Array,
    B_w_up: jax.Array,
    B_w_down: jax.Array,
):
    del B_x
    xT = A_x.reshape(S, D).T
    wdT = B_w_down.T
    any_spec = pl.BlockSpec(memory_space=pl.ANY)
    outT = pl.pallas_call(
        _kernel,
        in_specs=[any_spec] * 6,
        out_specs=any_spec,
        out_shape=jax.ShapeDtypeStruct((D, S), BF16),
        scratch_shapes=[
            pltpu.VMEM((NT, D, TM), BF16),
            pltpu.VMEM((NS, D, SUB), F32),
            pltpu.VMEM((NS, D, SUB), BF16),
            pltpu.VMEM((D, 3 * D), BF16),
            pltpu.VMEM((D, D), BF16),
            pltpu.VMEM((NCH, D, FC), BF16),
            pltpu.VMEM((NCH, D, FC), BF16),
            pltpu.VMEM((NCH, D, FC), BF16),
            pltpu.VMEM((DB, 3 * D, LANES), F32),
            pltpu.VMEM((NB * LANES, D), BF16),
            pltpu.VMEM((DB, D, LANES), F32),
            pltpu.VMEM((DB * LANES, D), F32),
            pltpu.VMEM((D, DB * LANES), BF16),
            pltpu.VMEM((NCH, NB + 1, HALO + SUB, LANES), F32),
            pltpu.VMEM((2 * NCH, SUB, D), BF16),
            pltpu.VMEM((2, TM, D), BF16),
            pltpu.SMEM((SUB // 8,), jnp.int32),
            pltpu.SemaphoreType.DMA((NT + DB + 1 + 3 * NCH,)),
            pltpu.SemaphoreType.DMA((NS,)),
        ] + [pltpu.VMEM((NB + 1, HALO + SUB, LANES), F32)] * NCH,
        compiler_params=pltpu.CompilerParams(
            vmem_limit_bytes=100 * 1024 * 1024),
    )(xT, A_wqkv, A_wo, B_w_gate, B_w_up, wdT)
    return outT.T.reshape(1, S, D)
```

```python
import jax
import jax.numpy as jnp
import jax.experimental.pallas as pl
import jax.experimental.pallas.tpu as pltpu

S = 2048
D = 576
F = 4608
H = 32
DH = 18
W = 8
DIL = 2
EPS = 1e-5
LANES = 128

TM = 512
NT = S // TM
FC = 1152
NCH = F // FC
SUB = TM // NCH
NS = S // SUB
RB = 8
RB0 = 16
PIPE = 0
PIPE0 = 0
UNROLL = (1, 1, 2)
RING = 4
HALO = 16
NB = 14
DB = 5

Q_BLOCKS = (0, 1, 2, 3, 12)
K_BLOCKS = (4, 5, 6, 7, 13)
V_BLOCKS = (8, 9, 10, 11, 12)
O_BLOCKS = (0, 1, 2, 3, 14)
KV_BLOCKS = (4, 5, 6, 7, 8, 9, 10, 11, 12, 13)

SCALE = DH ** -0.5
EXP2_SCALE = SCALE * 1.4426950408889634
MASKED_LOGIT = -1e9 / SCALE

NT_DIMS = (((1,), (1,)), ((), ()))
F32 = jnp.float32
BF16 = jnp.bfloat16


def _qkv_dest_row(part, d):
    if d < 16:
        return (part * 4 + d // 4) * LANES + (d % 4) * H
    base = (12 * LANES, 13 * LANES, 12 * LANES + 64)[part]
    return base + (d - 16) * H


def _o_dest_row(d):
    if d < 16:
        return d * H
    return 4 * LANES + 64 + (d - 16) * H


def _mod(a, n):
    assert n & (n - 1) == 0
    return jax.lax.bitwise_and(a, n - 1)


def _div(a, n):
    assert n & (n - 1) == 0
    return jax.lax.shift_right_logical(a, n.bit_length() - 1)


def _layernorm_t(x):
    m = jnp.mean(x, axis=0, keepdims=True)
    c = x - m
    v = jnp.mean(c * c, axis=0, keepdims=True)
    y = c * jax.lax.rsqrt(v + EPS)
    return y.astype(BF16).T


def _kernel(xT_hbm, wqkv_hbm, wo_hbm, wg_hbm, wu_hbm, wdT_hbm, out_hbm,
            xin, xres, xout, wqkv_raw, wo_raw, wg, wu, wd,
            wt_tmp, wq_p, wo_tmp, wo_p, wo_pt, ring, xn1, xn2, row_s,
            sem_in, sem_o, *qkv_bufs):

    def x_copy(t):
        return pltpu.make_async_copy(
            xT_hbm.at[:, pl.ds(t * TM, TM)], xin.at[t], sem_in.at[t])

    def f_copy(which, c):
        src = (wg_hbm, wu_hbm, wdT_hbm)[which]
        dst = (wg, wu, wd)[which]
        start = c * FC
        if not isinstance(c, int):
            start = pl.multiple_of(start, LANES)
        return pltpu.make_async_copy(
            src.at[:, pl.ds(start, FC)], dst.at[c],
            sem_in.at[NT + DB + 1 + which * NCH + c])

    def out_copy(p):
        start = p * SUB
        if not isinstance(p, int):
            start = pl.multiple_of(start, LANES)
        return pltpu.make_async_copy(
            xout.at[p], out_hbm.at[:, pl.ds(start, SUB)], sem_o.at[p])

    def wqkv_copy(j):
        rows = pl.ds(j * LANES, min(LANES, D - j * LANES))
        return pltpu.make_async_copy(
            wqkv_hbm.at[rows], wqkv_raw.at[rows], sem_in.at[NT + j])

    wo_copy = pltpu.make_async_copy(wo_hbm, wo_raw, sem_in.at[NT + DB])

    def prep_wqkv(j):
        n = min(LANES, D - j * LANES)
        blk = wqkv_raw[j * LANES:j * LANES + n, :].astype(F32)
        wt_tmp[j, :, 0:n] = blk.T
        for part in range(3):
            for d in range(DH):
                dst = _qkv_dest_row(part, d)
                val = wt_tmp[j, pl.ds(part * D + d, H, stride=DH), :]
                wq_p[dst:dst + H, j * LANES:j * LANES + n] = (
                    val[:, 0:n].astype(BF16))

    def prep_wo():
        for j in range(DB):
            cols = min(LANES, D - j * LANES)
            wo_tmp[j, :, 0:cols] = (
                wo_raw[:, j * LANES:j * LANES + cols].astype(F32))
        for d in range(DH):
            dst = _o_dest_row(d)
            for j in range(DB):
                cols = min(LANES, D - j * LANES)
                val = wo_tmp[j, pl.ds(d, H, stride=DH), :]
                wo_p[dst:dst + H, j * LANES:j * LANES + cols] = val[:, 0:cols]
        wo_p[4 * LANES:4 * LANES + 64, :] = jnp.zeros((64, D), F32)
        wo_pt[...] = wo_p[...].astype(BF16).T

    def project(xn, qkv, prev, first):
        tails = None
        if first is not True:
            tails = [prev[j, SUB:SUB + HALO, :] for j in KV_BLOCKS]
        res = jax.lax.dot_general(xn, wq_p[...], NT_DIMS,
                                  preferred_element_type=F32)
        for j in range(NB):
            qkv[j, HALO:HALO + SUB, :] = res[:, j * LANES:(j + 1) * LANES]
        for i, j in enumerate(KV_BLOCKS):
            if first is False:
                qkv[j, 0:HALO, :] = tails[i]
                continue
            row0 = jnp.broadcast_to(res[0:1, j * LANES:(j + 1) * LANES],
                                    (HALO, LANES))
            if first is True:
                qkv[j, 0:HALO, :] = row0
            else:
                qkv[j, 0:HALO, :] = jnp.where(first, row0, tails[i])

    def window(qkv, j, r0, rb, w):
        return qkv[j, pl.ds(HALO + r0 - DIL * w, rb), :]

    def attn_scores(qkv, p, r0, rb, masked):
        q = [window(qkv, j, r0, rb, 0) for j in Q_BLOCKS]
        if masked:
            pos = (p * SUB + r0
                   + jax.lax.broadcasted_iota(jnp.int32, (rb, LANES), 0))
        logits = []
        for w in range(W):
            lg = q[0] * window(qkv, K_BLOCKS[0], r0, rb, w)
            for i in range(1, DB):
                lg = lg + q[i] * window(qkv, K_BLOCKS[i], r0, rb, w)
            lg = lg + pltpu.roll(lg, 64, 1)
            lg = lg + pltpu.roll(lg, 32, 1)
            if masked and w > 0:
                lg = jnp.where(pos >= DIL * w, lg, MASKED_LOGIT)
            logits.append(lg)
        m = logits[0]
        for w in range(1, W):
            m = jnp.maximum(m, logits[w])
        es = [jnp.exp2((lg - m) * EXP2_SCALE) for lg in logits]
        s = es[0]
        for w in range(1, W):
            s = s + es[w]
        return es, 1.0 / s

    def attn_values(qkv, r0, rb, es, r):
        for i, j in enumerate(V_BLOCKS):
            o = es[0] * window(qkv, j, r0, rb, 0)
            for w in range(1, W):
                o = o + es[w] * window(qkv, j, r0, rb, w)
            o = o * r
            if i == DB - 1:
                lane = jax.lax.broadcasted_iota(jnp.int32, (rb, LANES), 1)
                o = jnp.where(lane >= 64, o, 0.0)
            qkv[O_BLOCKS[i], pl.ds(HALO + r0, rb), :] = o

    def attention(qkv, p, rb, pipe):
        pending = None
        for a in range(SUB // rb):
            masked = a * rb < (W - 1) * DIL and not (isinstance(p, int) and p > 0)
            r0 = pl.multiple_of(row_s[a * rb // 8], rb)
            cur = (qkv, r0, rb) + attn_scores(qkv, p, r0, rb, masked)
            if not pipe:
                attn_values(*cur)
                continue
            if pending is not None:
                attn_values(*pending)
            pending = cur
        if pending is not None:
            attn_values(*pending)

    def out_proj(qkv, p, slot, row0):
        o = jnp.concatenate(
            [qkv[j, HALO:HALO + SUB, :].astype(BF16) for j in O_BLOCKS], axis=1)
        upd = jax.lax.dot_general(wo_pt[...], o, NT_DIMS,
                                  preferred_element_type=F32)
        x = xres[p] + upd
        xres[p] = x
        xn2[slot, pl.ds(row0, SUB), :] = _layernorm_t(x)

    def ffn_up(slot, c):
        xn = xn2[slot]
        g = jnp.dot(xn, wg[c], preferred_element_type=F32)
        u = jnp.dot(xn, wu[c], preferred_element_type=F32)
        return (g * u).astype(BF16)

    def ffn_down(h, t, c):
        res = jax.lax.dot_general(wd[c], h, NT_DIMS,
                                  preferred_element_type=F32)
        for i in range(NCH):
            x = xres[t * NCH + i] + res[:, i * SUB:(i + 1) * SUB]
            xres[t * NCH + i] = x
            xout[t * NCH + i] = x.astype(BF16)

    def load_x(t):
        for i in range(NCH):
            xres[t * NCH + i] = xin[t, :, i * SUB:(i + 1) * SUB].astype(F32)

    x_copy(0).start()
    for j in range(DB):
        wqkv_copy(j).start()
    wo_copy.start()
    for t in range(1, NT):
        x_copy(t).start()
    for c in range(NCH):
        for which in range(3):
            f_copy(which, c).start()
    for a in range(SUB // 8):
        row_s[a] = a * 8
    wq_p[13 * LANES + 64:14 * LANES, :] = jnp.zeros((64, D), BF16)

    def buf(j):
        return qkv_bufs[j] if j < NCH else ring.at[(j - NCH) % RING]

    def ln1_pro(j):
        xn1[j] = _layernorm_t(xres[j])

    def project_pro(j):
        project(xn1[j], buf(j), buf(j - 1) if j else None, j == 0)

    n_pro = NCH + RING
    with jax.named_scope("s_prep"):
        x_copy(0).wait()
        load_x(0)
        ln1_pro(0)
        for j in range(DB):
            wqkv_copy(j).wait()
            prep_wqkv(j)
        project_pro(0)
        for j in range(1, NCH):
            ln1_pro(j)
        project_pro(1)
    with jax.named_scope("s_stage0"):
        wo_copy.wait()
        for t in range(1, NT):
            x_copy(t).wait()
        side = {}
        for i in range(NCH):
            side.setdefault(2 + i * RING // NCH, []).append(
                lambda i=i: attention(buf(i), i, RB0, PIPE0))
            side.setdefault(min(2 + (i + 2) * RING // NCH, n_pro - 2), []).append(
                lambda i=i: out_proj(buf(i), i, 0, i * SUB))
        side[2] += [lambda: load_x(1), prep_wo]
        for t in range(2, NT):
            side.setdefault(min(t * NCH - 2, n_pro - NT + t - 1), []).append(
                lambda t=t: load_x(t))
        for j in range(2, n_pro):
            if j >= NCH:
                ln1_pro(j)
            project_pro(j)
            for f in side.get(j, []):
                f()
        for c in range(UNROLL[0]):
            for which in range(3):
                f_copy(which, c).wait()

    def start_out(k):
        @pl.when(k >= NS + NCH)
        def _():
            out_copy(k - NS - NCH).start()

    def body(k, do_attn, do_proj):
        n = _div(k, NCH)
        c = _mod(k, NCH)
        sl = _mod(k, RING)
        if do_proj:
            pj = _mod(k + n_pro, NS)
            xn1[0] = _layernorm_t(xres[pj])
        h = ffn_up(_mod(n, 2), c)
        if do_attn:
            p = _mod(k + NCH, NS)
            attention(ring.at[sl], p, RB, PIPE)
            out_proj(ring.at[sl], p, _mod(n + 1, 2),
                     pl.multiple_of(c * SUB, SUB))
        if do_proj:
            project(xn1[0], ring.at[sl], ring.at[_mod(k + RING - 1, RING)],
                    pj == 0)
        ffn_down(h, _mod(n, NT), c)

    def loop(lo, hi, do_attn, do_proj, unroll):
        def step(m, carry):
            k0 = m * unroll
            for u in range(unroll):
                start_out(k0 + u)
            for u in range(unroll):
                body(k0 + u, do_attn, do_proj)
            if lo == 0:
                @pl.when(k0 + unroll < NCH)
                def _():
                    for u in range(unroll):
                        for which in range(3):
                            f_copy(which, k0 + unroll + u).wait()
            return carry
        assert lo % unroll == 0 and hi % unroll == 0 and NCH % unroll == 0
        jax.lax.fori_loop(lo // unroll, hi // unroll, step, 0)

    with jax.named_scope("s_main"):
        loop(0, 2 * NS - n_pro, True, True, UNROLL[0])
    with jax.named_scope("s_mid"):
        loop(2 * NS - n_pro, 2 * NS - NCH, True, False, UNROLL[1])
    with jax.named_scope("s_last"):
        loop(2 * NS - NCH, 2 * NS, False, False, UNROLL[2])
    with jax.named_scope("s_tail"):
        for p in range(NS - NCH, NS):
            out_copy(p).start()
        for p in range(NS):
            out_copy(p).wait()


@jax.jit
def pallas_interleave_layers__sliding_local_dilated__glu_gated_bilinear__prompt_kernel(
    A_x: jax.Array,
    A_wqkv: jax.Array,
    A_wo: jax.Array,
    B_x: jax.Array,
    B_w_gate: jax.Array,
    B_w_up: jax.Array,
    B_w_down: jax.Array,
):
    del B_x
    xT = A_x.reshape(S, D).T
    wdT = B_w_down.T
    any_spec = pl.BlockSpec(memory_space=pl.ANY)
    outT = pl.pallas_call(
        _kernel,
        in_specs=[any_spec] * 6,
        out_specs=any_spec,
        out_shape=jax.ShapeDtypeStruct((D, S), BF16),
        scratch_shapes=[
            pltpu.VMEM((NT, D, TM), BF16),
            pltpu.VMEM((NS, D, SUB), F32),
            pltpu.VMEM((NS, D, SUB), BF16),
            pltpu.VMEM((D, 3 * D), BF16),
            pltpu.VMEM((D, D), BF16),
            pltpu.VMEM((NCH, D, FC), BF16),
            pltpu.VMEM((NCH, D, FC), BF16),
            pltpu.VMEM((NCH, D, FC), BF16),
            pltpu.VMEM((DB, 3 * D, LANES), F32),
            pltpu.VMEM((NB * LANES, D), BF16),
            pltpu.VMEM((DB, D, LANES), F32),
            pltpu.VMEM((DB * LANES, D), F32),
            pltpu.VMEM((D, DB * LANES), BF16),
            pltpu.VMEM((RING, NB + 1, HALO + SUB, LANES), F32),
            pltpu.VMEM((NCH + RING, SUB, D), BF16),
            pltpu.VMEM((2, TM, D), BF16),
            pltpu.SMEM((SUB // 8,), jnp.int32),
            pltpu.SemaphoreType.DMA((NT + DB + 1 + 3 * NCH,)),
            pltpu.SemaphoreType.DMA((NS,)),
        ] + [pltpu.VMEM((NB + 1, HALO + SUB, LANES), F32)] * NCH,
        compiler_params=pltpu.CompilerParams(
            vmem_limit_bytes=100 * 1024 * 1024),
    )(xT, A_wqkv, A_wo, B_w_gate, B_w_up, wdT)
    return outT.T.reshape(1, S, D)
```

```python
import jax
import jax.numpy as jnp
import jax.experimental.pallas as pl
import jax.experimental.pallas.tpu as pltpu

S = 2048
D = 576
F = 4608
H = 32
DH = 18
W = 8
DIL = 2
EPS = 1e-5
LANES = 128

TM = 512
NT = S // TM
FC = 1152
NCH = F // FC
SUB = TM // NCH
NS = S // SUB
HG = 8
OPAQUE = 1
SB = 2
UNROLL = (1, 1, 2)
RING = 8
PIECES = (0, 256, 640, 1152, 1728)
LAG = 128
MC = 256
EARLY = 2
LASTP = 432
NP = len(PIECES) - 1

SCALE = DH ** -0.5
EXP2_SCALE = SCALE * 1.4426950408889634
MASKED_LOGIT = -1e9 / SCALE

NT_DIMS = (((1,), (1,)), ((), ()))
F32 = jnp.float32
BF16 = jnp.bfloat16


def _mod(a, n):
    assert n & (n - 1) == 0
    return jax.lax.bitwise_and(a, n - 1)


def _div(a, n):
    assert n & (n - 1) == 0
    return jax.lax.shift_right_logical(a, n.bit_length() - 1)


def _layernorm(x):
    m = jnp.mean(x, axis=0, keepdims=True)
    c = x - m
    v = jnp.mean(c * c, axis=0, keepdims=True)
    y = c * jax.lax.rsqrt(v + EPS)
    return y.astype(BF16)


def _kernel(xT_hbm, wqkv_hbm, wo_hbm, wg_hbm, wu_hbm, wdT_hbm, out_hbm,
            xin, xres, xout, wqkv_raw, wo_raw, wg, wu, wd,
            wqT, woT, ring, xn1, xn2, row_s, sem_in, sem_o):

    def x_copy(t):
        return pltpu.make_async_copy(
            xT_hbm.at[:, pl.ds(t * TM, TM)], xin.at[t], sem_in.at[t])

    def f_copy(which, c):
        src = (wg_hbm, wu_hbm, wdT_hbm)[which]
        dst = (wg, wu, wd)[which]
        start = c * FC
        if not isinstance(c, int):
            start = pl.multiple_of(start, LANES)
        return pltpu.make_async_copy(
            src.at[:, pl.ds(start, FC)], dst.at[c],
            sem_in.at[NT + NP + 1 + which * NCH + c])

    def out_copy(p):
        start = p * SUB
        if not isinstance(p, int):
            start = pl.multiple_of(start, LANES)
        return pltpu.make_async_copy(
            xout.at[p], out_hbm.at[:, pl.ds(start, SUB)], sem_o.at[p])

    def wqkv_copy(j):
        cols = pl.ds(PIECES[j], PIECES[j + 1] - PIECES[j])
        return pltpu.make_async_copy(
            wqkv_hbm.at[:, cols], wqkv_raw.at[:, cols], sem_in.at[NT + j])

    wo_copy = pltpu.make_async_copy(wo_hbm, wo_raw, sem_in.at[NT + NP])

    def transpose_cols(src, dst, lo, hi):
        for c0 in range(lo, hi, LANES):
            c1 = min(c0 + LANES, hi)
            dst[c0:c1, :] = src[:, c0:c1].T

    lane = jax.lax.broadcasted_iota(jnp.int32, (HG, LANES), 1)

    def shifted(cur, prev, w):
        if w == 0:
            return cur
        both = jnp.where(lane < LANES - DIL * w, cur, prev)
        return pltpu.roll(both, DIL * w, 1)

    def rows(base, part, d):
        return pl.ds(base + part * D + d, HG, stride=DH)

    def attn_scores(cur, prev, p, base):
        first = isinstance(p, int) and p == 0
        logits = [None] * W
        for d in range(DH):
            q = cur[rows(base, 0, d), :]
            kc = cur[rows(base, 1, d), :]
            kp = kc if first else prev[rows(base, 1, d), :]
            for w in range(W):
                t = q * shifted(kc, kp, w)
                logits[w] = t if d == 0 else logits[w] + t
        if first or not isinstance(p, int):
            pos = p * SUB + lane
            for w in range(1, W):
                logits[w] = jnp.where(pos >= DIL * w, logits[w], MASKED_LOGIT)
        m = logits[0]
        for w in range(1, W):
            m = jnp.maximum(m, logits[w])
        es = [jnp.exp2((lg - m) * EXP2_SCALE) for lg in logits]
        s = es[0]
        for w in range(1, W):
            s = s + es[w]
        r = 1.0 / s
        return [e * r for e in es]

    def attn_values(cur, prev, base, a, sb):
        done = []
        for d in range(DH):
            vc = cur[rows(base, 2, d), :]
            vp = prev[rows(base, 2, d), :]
            o = a[0] * vc
            for w in range(1, W):
                o = o + a[w] * shifted(vc, vp, w)
            done.append((d, o))
            if len(done) == sb or d == DH - 1:
                for dd, oo in done:
                    cur[rows(base, 0, dd), :] = oo
                done = []

    def attention(cur, prev, p):
        for g in range(H // HG):
            base = row_s[g] if OPAQUE else g * HG * DH
            attn_values(cur, prev, base, attn_scores(cur, prev, p, base), SB)

    def fill_clamped(dst, src):
        ring[dst, 2 * D:3 * D, :] = jnp.broadcast_to(
            ring[src, 2 * D:3 * D, 0:1], (D, LANES))

    def out_proj(qkv, p, slot, row0):
        upd = jnp.dot(woT[...], qkv[0:D, :].astype(BF16),
                      preferred_element_type=F32)
        x = xres[p] + upd
        xres[p] = x
        xn2[slot, pl.ds(row0, SUB), :] = _layernorm(x).T

    def ffn_up(slot, c):
        xn = xn2[slot]
        g = jnp.dot(xn, wg[c], preferred_element_type=F32)
        u = jnp.dot(xn, wu[c], preferred_element_type=F32)
        return (g * u).astype(BF16)

    def ffn_down(h, t, c):
        res = jax.lax.dot_general(wd[c], h, NT_DIMS,
                                  preferred_element_type=F32)
        for i in range(NCH):
            x = xres[t * NCH + i] + res[:, i * SUB:(i + 1) * SUB]
            xres[t * NCH + i] = x
            xout[t * NCH + i] = x.astype(BF16)

    def load_x(t):
        for i in range(NCH):
            xres[t * NCH + i] = xin[t, :, i * SUB:(i + 1) * SUB].astype(F32)

    def ln1_tile(t):
        for i in range(NCH):
            x = xin[t, :, i * SUB:(i + 1) * SUB].astype(F32)
            xres[t * NCH + i] = x
            xn1[t, :, i * SUB:(i + 1) * SUB] = _layernorm(x)

    def project_tile(t, lo, hi, mc=3 * D):
        for m0 in range(lo, hi, mc):
            m1 = min(m0 + mc, hi)
            res = jnp.dot(wqT[m0:m1, :], xn1[t], preferred_element_type=F32)
            for i in range(NCH):
                ring[t * NCH + i, m0:m1, :] = res[:, i * SUB:(i + 1) * SUB]

    x_copy(0).start()
    for j in range(NP):
        wqkv_copy(j).start()
    x_copy(1).start()
    wo_copy.start()
    for t in range(2, NT):
        x_copy(t).start()
    for c in range(NCH):
        for which in range(3):
            f_copy(which, c).start()
    for g in range(H // HG):
        row_s[g] = g * HG * DH

    def prev0(i):
        return ring.at[i - 1 if i else RING]

    def scores0(i):
        return [attn_scores(ring.at[i], prev0(i), i, g * HG * DH)
                for g in range(H // HG)]

    n_pro = 2 * NCH
    with jax.named_scope("s_prep"):
        x_copy(0).wait()
        ln1_tile(0)
        done = 0
        for j in range(NP):
            wqkv_copy(j).wait()
            if j == NP - 1:
                x_copy(1).wait()
            project_tile(0, done, PIECES[j], MC)
            transpose_cols(wqkv_raw, wqT, PIECES[j], PIECES[j + 1])
            done = PIECES[j + 1] - (LAG if j < NP - 1 else 0)
            if j == NP - 1:
                early = [scores0(i) for i in range(EARLY)]
                ln1_tile(1)
            project_tile(0, PIECES[j], done, MC if j else LANES)
    with jax.named_scope("s_stage0"):
        wo_copy.wait()
        for t in range(2, NT):
            x_copy(t).wait()
        fill_clamped(RING, 0)
        transpose_cols(wo_raw, woT, 0, D)
        cuts = [(3 * D - LASTP) * i // NCH // 16 * 16 for i in range(NCH)]
        cuts += [3 * D - LASTP]
        for i in range(NCH):
            sc = early[i] if i < EARLY else scores0(i)
            for g in range(H // HG):
                attn_values(ring.at[i], prev0(i), g * HG * DH, sc[g], 1)
            project_tile(1, cuts[i], cuts[i + 1])
            out_proj(ring.at[i], i, 0, i * SUB)
            if i >= 2:
                load_x(i)
        project_tile(1, cuts[NCH], 3 * D)
        for c in range(UNROLL[0]):
            for which in range(3):
                f_copy(which, c).wait()

    def start_out(k):
        @pl.when(k >= NS + NCH)
        def _():
            out_copy(k - NS - NCH).start()

    def body(k, do_attn, do_proj):
        n = _div(k, NCH)
        c = _mod(k, NCH)
        if do_proj:
            xn1[0, :, 0:SUB] = _layernorm(xres[_mod(k + n_pro, NS)])
        h = ffn_up(_mod(n, 2), c)
        if do_attn:
            p = _mod(k + NCH, NS)
            cur = ring.at[_mod(k + NCH, RING)]
            attention(cur, ring.at[_mod(k + NCH - 1, RING)], p)
            out_proj(cur, p, _mod(n + 1, 2), pl.multiple_of(c * SUB, SUB))
        if do_proj:
            ring[_mod(k + n_pro, RING)] = jnp.dot(
                wqT[...], xn1[0, :, 0:SUB], preferred_element_type=F32)
        ffn_down(h, _mod(n, NT), c)

    def loop(lo, hi, do_attn, do_proj, unroll):
        def step(m, carry):
            k0 = m * unroll
            for u in range(unroll):
                start_out(k0 + u)
            for u in range(unroll):
                body(k0 + u, do_attn, do_proj)
            if lo == 0:
                @pl.when(k0 + unroll < NCH)
                def _():
                    for u in range(unroll):
                        for which in range(3):
                            f_copy(which, k0 + unroll + u).wait()

                @pl.when(k0 + unroll == NS - NCH)
                def _():
                    fill_clamped((NS - 1) % RING, NS % RING)
            return carry
        assert lo % unroll == 0 and hi % unroll == 0 and NCH % unroll == 0
        jax.lax.fori_loop(lo // unroll, hi // unroll, step, 0)

    with jax.named_scope("s_main"):
        loop(0, 2 * NS - n_pro, True, True, UNROLL[0])
    with jax.named_scope("s_mid"):
        loop(2 * NS - n_pro, 2 * NS - NCH, True, False, UNROLL[1])
    with jax.named_scope("s_last"):
        loop(2 * NS - NCH, 2 * NS, False, False, UNROLL[2])
    with jax.named_scope("s_tail"):
        for p in range(NS - NCH, NS):
            out_copy(p).start()
        for p in range(NS):
            out_copy(p).wait()


@jax.jit
def pallas_interleave_layers__sliding_local_dilated__glu_gated_bilinear__prompt_kernel(
    A_x: jax.Array,
    A_wqkv: jax.Array,
    A_wo: jax.Array,
    B_x: jax.Array,
    B_w_gate: jax.Array,
    B_w_up: jax.Array,
    B_w_down: jax.Array,
):
    del B_x
    xT = A_x.reshape(S, D).T
    wdT = B_w_down.T
    any_spec = pl.BlockSpec(memory_space=pl.ANY)
    outT = pl.pallas_call(
        _kernel,
        in_specs=[any_spec] * 6,
        out_specs=any_spec,
        out_shape=jax.ShapeDtypeStruct((D, S), BF16),
        scratch_shapes=[
            pltpu.VMEM((NT, D, TM), BF16),
            pltpu.VMEM((NS, D, SUB), F32),
            pltpu.VMEM((NS, D, SUB), BF16),
            pltpu.VMEM((D, 3 * D), BF16),
            pltpu.VMEM((D, D), BF16),
            pltpu.VMEM((NCH, D, FC), BF16),
            pltpu.VMEM((NCH, D, FC), BF16),
            pltpu.VMEM((NCH, D, FC), BF16),
            pltpu.VMEM((3 * D, D), BF16),
            pltpu.VMEM((D, D), BF16),
            pltpu.VMEM((RING + 1, 3 * D, LANES), F32),
            pltpu.VMEM((2, D, TM), BF16),
            pltpu.VMEM((2, TM, D), BF16),
            pltpu.SMEM((H // HG,), jnp.int32),
            pltpu.SemaphoreType.DMA((NT + NP + 1 + 3 * NCH,)),
            pltpu.SemaphoreType.DMA((NS,)),
        ],
        compiler_params=pltpu.CompilerParams(
            vmem_limit_bytes=100 * 1024 * 1024),
    )(xT, A_wqkv, A_wo, B_w_gate, B_w_up, wdT)
    return outT.T.reshape(1, S, D)
```

```python
import jax
import jax.numpy as jnp
import jax.experimental.pallas as pl
import jax.experimental.pallas.tpu as pltpu

S = 2048
D = 576
F = 4608
H = 32
DH = 18
W = 8
DIL = 2
EPS = 1e-5
LANES = 128

TM = 512
NT = S // TM
FC = 1152
NCH = F // FC
SUB = TM // NCH
NS = S // SUB
HG = 8
OPAQUE = 1
SB = 2
UNROLL = (1, 1, 2)
RING = 16
PIECES = (0, 256, 640, 1152, 1728)
LAG = 128
MC = 256
AHEAD = 1
SB0 = 18
PT = 3
OW = 4
LN_SPLIT = 2
ACC0 = (4, 4)
ACCP = (1, 1)
ACC1 = (1, 1)
ACC2 = (1, 1)
RL1 = 0
RL2 = 1
RL0 = 0
XW = 1
LN2_AT = (2, 4, 6, 8)
X1_AT = 3
LASTP = 432
NP = len(PIECES) - 1

SCALE = DH ** -0.5
EXP2_SCALE = SCALE * 1.4426950408889634
MASKED_LOGIT = -1e9 / SCALE

NT_DIMS = (((1,), (1,)), ((), ()))
F32 = jnp.float32
BF16 = jnp.bfloat16


def _mod(a, n):
    assert n & (n - 1) == 0
    return jax.lax.bitwise_and(a, n - 1)


def _div(a, n):
    assert n & (n - 1) == 0
    return jax.lax.shift_right_logical(a, n.bit_length() - 1)


def _mean_rows(x, acc):
    part = jnp.sum(x.reshape(D // (8 * acc), 8 * acc, x.shape[1]), axis=0)
    return jnp.sum(part, axis=0, keepdims=True) * (1.0 / D)


def _layernorm(x, acc, reread=None):
    m = _mean_rows(x, acc[0])
    c = (x if reread is None else reread(0)) - m
    v = _mean_rows(c * c, acc[1])
    if reread is not None:
        c = reread(1) - m
    y = c * jax.lax.rsqrt(v + EPS)
    return y.astype(BF16)


def _kernel(xT_hbm, wqkv_hbm, wo_hbm, wg_hbm, wu_hbm, wdT_hbm, out_hbm,
            xres, xio, wqkv_raw, wo_raw, wg, wu, wd,
            wqT, woT, first, ring, xn1, xn2, row_s, zero_s, sem_in, sem_o):

    def x_copy(p):
        start = p * SUB
        if not isinstance(p, int):
            start = pl.multiple_of(start, LANES)
        return pltpu.make_async_copy(
            xT_hbm.at[:, pl.ds(start, SUB)], xio.at[p], sem_in.at[p])

    def f_copy(which, c):
        src = (wg_hbm, wu_hbm, wdT_hbm)[which]
        dst = (wg, wu, wd)[which]
        start = c * FC
        if not isinstance(c, int):
            start = pl.multiple_of(start, LANES)
        return pltpu.make_async_copy(
            src.at[:, pl.ds(start, FC)], dst.at[c],
            sem_in.at[NS + NP + 1 + which * NCH + c])

    def out_copy(p):
        start = p * SUB
        if not isinstance(p, int):
            start = pl.multiple_of(start, LANES)
        return pltpu.make_async_copy(
            xio.at[p], out_hbm.at[:, pl.ds(start, SUB)], sem_o.at[p])

    def wqkv_copy(j):
        cols = pl.ds(PIECES[j], PIECES[j + 1] - PIECES[j])
        return pltpu.make_async_copy(
            wqkv_hbm.at[:, cols], wqkv_raw.at[:, cols], sem_in.at[NS + j])

    wo_copy = pltpu.make_async_copy(wo_hbm, wo_raw, sem_in.at[NS + NP])

    def transpose_cols(src, dst, lo, hi):
        for c0 in range(lo, hi, LANES):
            c1 = min(c0 + LANES, hi)
            dst[c0:c1, :] = src[:, c0:c1].T

    lane = jax.lax.broadcasted_iota(jnp.int32, (HG, LANES), 1)

    def shifted(cur, prev, w):
        if w == 0:
            return cur
        both = jnp.where(lane < LANES - DIL * w, cur, prev)
        return pltpu.roll(both, DIL * w, 1)

    def rows(base, part, d):
        return pl.ds(base + part * D + d, HG, stride=DH)

    def attn_scores(cur, prev, p, base):
        first = isinstance(p, int) and p == 0
        logits = [None] * W
        for d in range(DH):
            q = cur[rows(base, 0, d), :]
            kc = cur[rows(base, 1, d), :]
            kp = kc if first else prev[rows(base, 1, d), :]
            for w in range(W):
                t = q * shifted(kc, kp, w)
                logits[w] = t if d == 0 else logits[w] + t
        if first or not isinstance(p, int):
            pos = p * SUB + lane
            for w in range(1, W):
                logits[w] = jnp.where(pos >= DIL * w, logits[w], MASKED_LOGIT)
        m = logits[0]
        for w in range(1, W):
            m = jnp.maximum(m, logits[w])
        es = [jnp.exp2((lg - m) * EXP2_SCALE) for lg in logits]
        s = es[0]
        for w in range(1, W):
            s = s + es[w]
        r = 1.0 / s
        return [e * r for e in es]

    def attn_values(cur, prev, base, a, sb):
        done = []
        for d in range(DH):
            vc = cur[rows(base, 2, d), :]
            vp = prev[rows(base, 2, d), :]
            o = a[0] * vc
            for w in range(1, W):
                o = o + a[w] * shifted(vc, vp, w)
            done.append((d, o))
            if len(done) == sb or d == DH - 1:
                for dd, oo in done:
                    cur[rows(base, 0, dd), :] = oo
                done = []

    def attention(cur, prev, p):
        for g in range(H // HG):
            base = row_s[g] if OPAQUE else g * HG * DH
            attn_values(cur, prev, base, attn_scores(cur, prev, p, base), SB)

    def fill_clamped(buf, dst, src):
        buf[dst, 2 * D:3 * D, :] = jnp.broadcast_to(
            buf[src, 2 * D:3 * D, 0:1], (D, LANES))

    def residual(p, from_input):
        if from_input is True:
            return xio[p].astype(F32)
        if from_input is False:
            return xres[p]
        return jnp.where(from_input, xio[p].astype(F32), xres[p])

    def out_proj(qkv, p, from_input, slot, row0):
        upd = jnp.dot(woT[...], qkv[0:D, :].astype(BF16),
                      preferred_element_type=F32)
        x = residual(p, from_input) + upd
        xres[p] = x
        again = (lambda i: xres[p + zero_s[i]]) if RL2 else None
        xn2[slot, pl.ds(row0, SUB), :] = _layernorm(x, ACC2, again).T

    def ln1(p, from_input, acc, reread):
        again = lambda i: residual(p + zero_s[i], from_input)
        return _layernorm(residual(p, from_input), acc,
                          again if reread else None)

    def ffn_up(slot, c):
        xn = xn2[slot]
        g = jnp.dot(xn, wg[c], preferred_element_type=F32)
        u = jnp.dot(xn, wu[c], preferred_element_type=F32)
        return (g * u).astype(BF16)

    def ffn_down(h, t, c):
        res = jax.lax.dot_general(wd[c], h, NT_DIMS,
                                  preferred_element_type=F32)
        for i in range(NCH):
            x = xres[t * NCH + i] + res[:, i * SUB:(i + 1) * SUB]
            xres[t * NCH + i] = x
            xio[t * NCH + i] = x.astype(BF16)

    def ln1_tile(t, lo=0, hi=NCH):
        for i in range(lo, hi):
            xn1[t, :, i * SUB:(i + 1) * SUB] = ln1(
                t * NCH + i, True, ACCP if t else ACC0, RL0 and t > 0)

    def project_tile(t, lo, hi, mc=3 * D):
        for m0 in range(lo, hi, mc):
            m1 = min(m0 + mc, hi)
            res = jnp.dot(wqT[m0:m1, :], xn1[t], preferred_element_type=F32)
            for i in range(NCH):
                part = res[:, i * SUB:(i + 1) * SUB]
                if t == 0:
                    first[i, m0:m1, :] = part
                if t > 0 or (i == NCH - 1 and m1 > D):
                    ring[t * NCH + i, m0:m1, :] = part

    def out_proj0(lo, hi):
        o = jnp.concatenate(
            [first[i, 0:D, :].astype(BF16) for i in range(lo, hi)], axis=1)
        upd = jnp.dot(woT[...], o, preferred_element_type=F32)
        for i in range(lo, hi):
            x = residual(i, True) + upd[:, (i - lo) * SUB:(i - lo + 1) * SUB]
            xres[i] = x
            again = (lambda j, i=i: xres[i + zero_s[j]]) if RL0 else None
            xn2[0, i * SUB:(i + 1) * SUB, :] = _layernorm(x, ACCP, again).T

    n_pro = PT * NCH
    for p in range(NCH):
        x_copy(p).start()
    for j in range(NP):
        wqkv_copy(j).start()
        if j == X1_AT:
            for p in range(NCH, 2 * NCH):
                x_copy(p).start()
    wo_copy.start()
    for p in range(2 * NCH, n_pro):
        x_copy(p).start()
    for c in range(NCH):
        for which in range(3):
            f_copy(which, c).start()
        if c == 0:
            for p in range(n_pro, NS):
                x_copy(p).start()
    for g in range(H // HG):
        row_s[g] = g * HG * DH
    zero_s[0] = 0
    zero_s[1] = 0

    def unit0(u):
        i, g = divmod(u, H // HG)
        return first.at[i], first.at[i - 1 if i else NCH], i, row_s[g]

    with jax.named_scope("s_ln"):
        for p0 in range(0, NCH, XW):
            for p in range(p0, p0 + XW):
                x_copy(p).wait()
            ln1_tile(0, p0, p0 + XW)
    done = 0
    for j in range(NP):
        with jax.named_scope(f"s_w{j}"):
            wqkv_copy(j).wait()
            if j == X1_AT:
                for p in range(NCH, 2 * NCH):
                    x_copy(p).wait()
        with jax.named_scope(f"s_b{j}"):
            project_tile(0, done, PIECES[j], MC)
            transpose_cols(wqkv_raw, wqT, PIECES[j], PIECES[j + 1])
            done = PIECES[j + 1] - (LAG if j < NP - 1 else 0)
            project_tile(0, PIECES[j], done, MC if j else LANES)
            if j == X1_AT:
                ln1_tile(1, 0, LN_SPLIT)
            if j == NP - 1:
                ln1_tile(1, LN_SPLIT, NCH)
    with jax.named_scope("s_wo"):
        wo_copy.wait()
        for p in range(2 * NCH, n_pro):
            x_copy(p).wait()
    with jax.named_scope("s_stage0"):
        fill_clamped(first, NCH, 0)
        project_tile(1, 0, 3 * D)
        n_units = NCH * H // HG
        sc = [attn_scores(*unit0(u)) for u in range(AHEAD)]
        for u in range(n_units):
            if u + AHEAD < n_units:
                sc.append(attn_scores(*unit0(u + AHEAD)))
            cur, prev, _, base = unit0(u)
            attn_values(cur, prev, base, sc[u], SB0)
            for i in range(NCH):
                if LN2_AT[i] == u:
                    y = ln1(2 * NCH + i, True, ACCP, RL0)
                    xn1[2, :, i * SUB:(i + 1) * SUB] = y
                    first[NCH, 0:16, :] = y[D - 16:D, :].astype(F32)
        project_tile(2, 0, 3 * D - LASTP)
        transpose_cols(wo_raw, woT, 0, D)
        out_proj0(0, NCH)
        project_tile(2, 3 * D - LASTP, 3 * D)
        for which in range(3):
            f_copy(which, 0).wait()
        for p in range(n_pro, NS):
            x_copy(p).wait()

    def start_out(k):
        @pl.when(k >= NS + NCH)
        def _():
            out_copy(k - NS - NCH).start()

    def body(k, do_attn, do_proj):
        n = _div(k, NCH)
        c = _mod(k, NCH)
        if do_proj:
            xn1[0, :, 0:SUB] = ln1(_mod(k + n_pro, NS), k + n_pro < NS,
                                   ACC1, RL1)
        h = ffn_up(_mod(n, 2), c)
        if do_attn:
            p = _mod(k + NCH, NS)
            cur = ring.at[_mod(k + NCH, RING)]
            attention(cur, ring.at[_mod(k + NCH - 1, RING)], p)
            out_proj(cur, p, do_proj and k + NCH < NS, _mod(n + 1, 2),
                     pl.multiple_of(c * SUB, SUB))
        if do_proj:
            ring[_mod(k + n_pro, RING)] = jnp.dot(
                wqT[...], xn1[0, :, 0:SUB], preferred_element_type=F32)
        ffn_down(h, _mod(n, NT), c)

    def loop(lo, hi, do_attn, do_proj, unroll):
        def step(m, carry):
            k0 = m * unroll
            for u in range(unroll):
                start_out(k0 + u)
            for u in range(unroll):
                body(k0 + u, do_attn, do_proj)
            if lo == 0:
                assert unroll == 1

                @pl.when(k0 + 1 < NCH)
                def _():
                    for which in range(3):
                        f_copy(which, k0 + 1).wait()


                @pl.when(k0 + unroll == NS - NCH)
                def _():
                    fill_clamped(ring, (NS - 1) % RING, NS % RING)
            return carry
        assert lo % unroll == 0 and hi % unroll == 0 and NCH % unroll == 0
        jax.lax.fori_loop(lo // unroll, hi // unroll, step, 0)

    with jax.named_scope("s_main"):
        loop(0, 2 * NS - n_pro, True, True, UNROLL[0])
    with jax.named_scope("s_mid"):
        loop(2 * NS - n_pro, 2 * NS - NCH, True, False, UNROLL[1])
    with jax.named_scope("s_last"):
        loop(2 * NS - NCH, 2 * NS, False, False, UNROLL[2])
    with jax.named_scope("s_tail"):
        for p in range(NS - NCH, NS):
            out_copy(p).start()
        for p in range(NS):
            out_copy(p).wait()


@jax.jit
def pallas_interleave_layers__sliding_local_dilated__glu_gated_bilinear__prompt_kernel(
    A_x: jax.Array,
    A_wqkv: jax.Array,
    A_wo: jax.Array,
    B_x: jax.Array,
    B_w_gate: jax.Array,
    B_w_up: jax.Array,
    B_w_down: jax.Array,
):
    del B_x
    xT = A_x.reshape(S, D).T
    wdT = B_w_down.T
    any_spec = pl.BlockSpec(memory_space=pl.ANY)
    outT = pl.pallas_call(
        _kernel,
        in_specs=[any_spec] * 6,
        out_specs=any_spec,
        out_shape=jax.ShapeDtypeStruct((D, S), BF16),
        scratch_shapes=[
            pltpu.VMEM((NS, D, SUB), F32),
            pltpu.VMEM((NS, D, SUB), BF16),
            pltpu.VMEM((D, 3 * D), BF16),
            pltpu.VMEM((D, D), BF16),
            pltpu.VMEM((NCH, D, FC), BF16),
            pltpu.VMEM((NCH, D, FC), BF16),
            pltpu.VMEM((NCH, D, FC), BF16),
            pltpu.VMEM((3 * D, D), BF16),
            pltpu.VMEM((D, D), BF16),
            pltpu.VMEM((NCH + 1, 3 * D, LANES), F32),
            pltpu.VMEM((RING, 3 * D, LANES), F32),
            pltpu.VMEM((PT, D, TM), BF16),
            pltpu.VMEM((2, TM, D), BF16),
            pltpu.SMEM((H // HG,), jnp.int32),
            pltpu.SMEM((2,), jnp.int32),
            pltpu.SemaphoreType.DMA((NS + NP + 1 + 3 * NCH,)),
            pltpu.SemaphoreType.DMA((NS,)),
        ],
        compiler_params=pltpu.CompilerParams(
            vmem_limit_bytes=100 * 1024 * 1024),
    )(xT, A_wqkv, A_wo, B_w_gate, B_w_up, wdT)
    return outT.T.reshape(1, S, D)
```

```python
import jax
import jax.numpy as jnp
import jax.experimental.pallas as pl
import jax.experimental.pallas.tpu as pltpu

S = 2048
D = 576
F = 4608
H = 32
DH = 18
W = 8
DIL = 2
EPS = 1e-5
LANES = 128

TM = 512
NT = S // TM
FC = 1152
NCH = F // FC
SUB = TM // NCH
NS = S // SUB
HG = 8
OPAQUE = 1
SB = 2
UNROLL = (1, 1, 2)
RING = 16
PIECES = (0, 256, 640, 1152, 1728)
LAG = 128
MC = 256
AHEAD = 1
SB0 = 18
PT = 3
OW = 4
LN_SPLIT = 2
ACC0 = (4, 4)
ACCP = (1, 1)
ACC1 = (1, 1)
ACC2 = (1, 1)
RL1 = 0
RL2 = 1
RL0 = 0
XW = 1
LN2_AT = (2, 4, 6, 8)
X1_AT = 3
LASTP = 432
NP = len(PIECES) - 1

SCALE = DH ** -0.5
EXP2_SCALE = SCALE * 1.4426950408889634
MASKED_LOGIT = -1e9 / SCALE

NT_DIMS = (((1,), (1,)), ((), ()))
F32 = jnp.float32
BF16 = jnp.bfloat16
U32 = jnp.uint32


def _mod(a, n):
    assert n & (n - 1) == 0
    return jax.lax.bitwise_and(a, n - 1)


def _div(a, n):
    assert n & (n - 1) == 0
    return jax.lax.shift_right_logical(a, n.bit_length() - 1)


def _pack(x):
    return pltpu.bitcast(x, U32)


def _unpack(x):
    return pltpu.bitcast(x, BF16)


def _mean_rows(x, acc):
    part = jnp.sum(x.reshape(D // (8 * acc), 8 * acc, x.shape[1]), axis=0)
    return jnp.sum(part, axis=0, keepdims=True) * (1.0 / D)


def _layernorm(x, acc, reread=None):
    m = _mean_rows(x, acc[0])
    c = (x if reread is None else reread(0)) - m
    v = _mean_rows(c * c, acc[1])
    if reread is not None:
        c = reread(1) - m
    y = c * jax.lax.rsqrt(v + EPS)
    return y.astype(BF16)


def _kernel(xT_hbm, wqkv_hbm, wo_hbm, wg_hbm, wu_hbm, wdT_hbm, out_hbm,
            xres, xio, wqkv_raw, wo_raw, wg, wu, wd,
            wqT, woT, first, ring, xn1, xn2, row_s, zero_s, sem_in, sem_o):

    def x_copy(p):
        start = p * SUB
        if not isinstance(p, int):
            start = pl.multiple_of(start, LANES)
        return pltpu.make_async_copy(
            xT_hbm.at[:, pl.ds(start, SUB)], xio.at[p], sem_in.at[p])

    def f_copy(which, c):
        src = (wg_hbm, wu_hbm, wdT_hbm)[which]
        dst = (wg, wu, wd)[which]
        start = c * FC
        if not isinstance(c, int):
            start = pl.multiple_of(start, LANES)
        return pltpu.make_async_copy(
            src.at[:, pl.ds(start, FC)], dst.at[c],
            sem_in.at[NS + NP + 1 + which * NCH + c])

    def out_copy(p):
        start = p * SUB
        if not isinstance(p, int):
            start = pl.multiple_of(start, LANES)
        return pltpu.make_async_copy(
            xio.at[p], out_hbm.at[:, pl.ds(start, SUB)], sem_o.at[p])

    def wqkv_copy(j):
        cols = pl.ds(PIECES[j], PIECES[j + 1] - PIECES[j])
        return pltpu.make_async_copy(
            wqkv_hbm.at[:, cols], wqkv_raw.at[:, cols], sem_in.at[NS + j])

    wo_copy = pltpu.make_async_copy(wo_hbm, wo_raw, sem_in.at[NS + NP])

    def transpose_cols(src, dst, lo, hi):
        for c0 in range(lo, hi, LANES):
            c1 = min(c0 + LANES, hi)
            dst[c0 // 2:c1 // 2, :] = _pack(src[:, c0:c1].T)

    lane = jax.lax.broadcasted_iota(jnp.int32, (HG, LANES), 1)

    def shifted(cur, prev, w):
        if w == 0:
            return cur
        both = jnp.where(lane < LANES - DIL * w, cur, prev)
        return pltpu.roll(both, DIL * w, 1)

    def rows(base, part, d):
        return pl.ds(base + part * D + d, HG, stride=DH)

    def attn_scores(cur, prev, p, base):
        first = isinstance(p, int) and p == 0
        logits = [None] * W
        for d in range(DH):
            q = cur[rows(base, 0, d), :]
            kc = cur[rows(base, 1, d), :]
            kp = kc if first else prev[rows(base, 1, d), :]
            for w in range(W):
                t = q * shifted(kc, kp, w)
                logits[w] = t if d == 0 else logits[w] + t
        if first or not isinstance(p, int):
            pos = p * SUB + lane
            for w in range(1, W):
                logits[w] = jnp.where(pos >= DIL * w, logits[w], MASKED_LOGIT)
        m = logits[0]
        for w in range(1, W):
            m = jnp.maximum(m, logits[w])
        es = [jnp.exp2((lg - m) * EXP2_SCALE) for lg in logits]
        s = es[0]
        for w in range(1, W):
            s = s + es[w]
        r = 1.0 / s
        return [e * r for e in es]

    def attn_values(cur, prev, base, a, sb):
        done = []
        for d in range(DH):
            vc = cur[rows(base, 2, d), :]
            vp = prev[rows(base, 2, d), :]
            o = a[0] * vc
            for w in range(1, W):
                o = o + a[w] * shifted(vc, vp, w)
            done.append((d, o))
            if len(done) == sb or d == DH - 1:
                for dd, oo in done:
                    cur[rows(base, 0, dd), :] = oo
                done = []

    def attention(cur, prev, p):
        for g in range(H // HG):
            base = row_s[g] if OPAQUE else g * HG * DH
            attn_values(cur, prev, base, attn_scores(cur, prev, p, base), SB)

    def fill_clamped(buf, dst, src):
        buf[dst, 2 * D:3 * D, :] = jnp.broadcast_to(
            buf[src, 2 * D:3 * D, 0:1], (D, LANES))

    def residual(p, from_input):
        if from_input is True:
            return xio[p].astype(F32)
        if from_input is False:
            return xres[p]
        return jnp.where(from_input, xio[p].astype(F32), xres[p])

    def out_proj(qkv, p, from_input, slot, row0):
        upd = jnp.dot(_unpack(woT[...]), qkv[0:D, :].astype(BF16),
                      preferred_element_type=F32)
        x = residual(p, from_input) + upd
        xres[p] = x
        again = (lambda i: xres[p + zero_s[i]]) if RL2 else None
        xn2[slot, pl.ds(row0, SUB // 2), :] = _pack(
            _layernorm(x, ACC2, again).T)

    def ln1(p, from_input, acc, reread):
        again = lambda i: residual(p + zero_s[i], from_input)
        return _layernorm(residual(p, from_input), acc,
                          again if reread else None)

    def ffn_up(slot, c):
        xn = _unpack(xn2[slot])
        g = jnp.dot(xn, wg[c], preferred_element_type=F32)
        u = jnp.dot(xn, wu[c], preferred_element_type=F32)
        return (g * u).astype(BF16)

    def ffn_down(h, t, c):
        res = jax.lax.dot_general(wd[c], h, NT_DIMS,
                                  preferred_element_type=F32)
        for i in range(NCH):
            x = xres[t * NCH + i] + res[:, i * SUB:(i + 1) * SUB]
            xres[t * NCH + i] = x
            xio[t * NCH + i] = x.astype(BF16)

    def ln1_tile(t, lo=0, hi=NCH):
        for i in range(lo, hi):
            xn1[t, :, i * SUB:(i + 1) * SUB] = _pack(ln1(
                t * NCH + i, True, ACCP if t else ACC0, RL0 and t > 0))

    def project_tile(t, lo, hi, mc=3 * D):
        for m0 in range(lo, hi, mc):
            m1 = min(m0 + mc, hi)
            res = jnp.dot(_unpack(wqT[m0 // 2:m1 // 2, :]), _unpack(xn1[t]),
                          preferred_element_type=F32)
            for i in range(NCH):
                part = res[:, i * SUB:(i + 1) * SUB]
                if t == 0:
                    first[i, m0:m1, :] = part
                if t > 0 or (i == NCH - 1 and m1 > D):
                    ring[t * NCH + i, m0:m1, :] = part

    def out_proj0(lo, hi):
        o = jnp.concatenate(
            [first[i, 0:D, :].astype(BF16) for i in range(lo, hi)], axis=1)
        upd = jnp.dot(_unpack(woT[...]), o, preferred_element_type=F32)
        for i in range(lo, hi):
            x = residual(i, True) + upd[:, (i - lo) * SUB:(i - lo + 1) * SUB]
            xres[i] = x
            again = (lambda j, i=i: xres[i + zero_s[j]]) if RL0 else None
            xn2[0, i * SUB // 2:(i + 1) * SUB // 2, :] = _pack(
                _layernorm(x, ACCP, again).T)

    n_pro = PT * NCH
    for p in range(NCH):
        x_copy(p).start()
    for j in range(NP):
        wqkv_copy(j).start()
        if j == X1_AT:
            for p in range(NCH, 2 * NCH):
                x_copy(p).start()
    wo_copy.start()
    for p in range(2 * NCH, n_pro):
        x_copy(p).start()
    for c in range(NCH):
        for which in range(3):
            f_copy(which, c).start()
        if c == 0:
            for p in range(n_pro, NS):
                x_copy(p).start()
    for g in range(H // HG):
        row_s[g] = g * HG * DH
    zero_s[0] = 0
    zero_s[1] = 0

    def unit0(u):
        i, g = divmod(u, H // HG)
        return first.at[i], first.at[i - 1 if i else NCH], i, row_s[g]

    with jax.named_scope("s_ln"):
        for p0 in range(0, NCH, XW):
            for p in range(p0, p0 + XW):
                x_copy(p).wait()
            ln1_tile(0, p0, p0 + XW)
    done = 0
    for j in range(NP):
        with jax.named_scope(f"s_w{j}"):
            wqkv_copy(j).wait()
            if j == X1_AT:
                for p in range(NCH, 2 * NCH):
                    x_copy(p).wait()
        with jax.named_scope(f"s_b{j}"):
            project_tile(0, done, PIECES[j], MC)
            transpose_cols(wqkv_raw, wqT, PIECES[j], PIECES[j + 1])
            done = PIECES[j + 1] - (LAG if j < NP - 1 else 0)
            project_tile(0, PIECES[j], done, MC if j else LANES)
            if j == X1_AT:
                ln1_tile(1, 0, LN_SPLIT)
            if j == NP - 1:
                ln1_tile(1, LN_SPLIT, NCH)
    with jax.named_scope("s_wo"):
        wo_copy.wait()
        for p in range(2 * NCH, n_pro):
            x_copy(p).wait()
    with jax.named_scope("s_stage0"):
        fill_clamped(first, NCH, 0)
        project_tile(1, 0, 3 * D)
        n_units = NCH * H // HG
        sc = [attn_scores(*unit0(u)) for u in range(AHEAD)]
        for u in range(n_units):
            if u + AHEAD < n_units:
                sc.append(attn_scores(*unit0(u + AHEAD)))
            cur, prev, _, base = unit0(u)
            attn_values(cur, prev, base, sc[u], SB0)
            for i in range(NCH):
                if LN2_AT[i] == u:
                    y = ln1(2 * NCH + i, True, ACCP, RL0)
                    xn1[2, :, i * SUB:(i + 1) * SUB] = _pack(y)
                    first[NCH, 0:16, :] = y[D - 16:D, :].astype(F32)
        project_tile(2, 0, 3 * D - LASTP)
        transpose_cols(wo_raw, woT, 0, D)
        out_proj0(0, NCH)
        project_tile(2, 3 * D - LASTP, 3 * D)
        for which in range(3):
            f_copy(which, 0).wait()
        for p in range(n_pro, NS):
            x_copy(p).wait()

    def start_out(k):
        @pl.when(k >= NS + NCH)
        def _():
            out_copy(k - NS - NCH).start()

    def body(k, do_attn, do_proj):
        n = _div(k, NCH)
        c = _mod(k, NCH)
        if do_proj:
            xn1[0, :, 0:SUB] = _pack(
                ln1(_mod(k + n_pro, NS), k + n_pro < NS, ACC1, RL1))
        h = ffn_up(_mod(n, 2), c)
        if do_attn:
            p = _mod(k + NCH, NS)
            cur = ring.at[_mod(k + NCH, RING)]
            attention(cur, ring.at[_mod(k + NCH - 1, RING)], p)
            out_proj(cur, p, do_proj and k + NCH < NS, _mod(n + 1, 2),
                     pl.multiple_of(c * (SUB // 2), SUB // 2))
        if do_proj:
            ring[_mod(k + n_pro, RING)] = jnp.dot(
                _unpack(wqT[...]), _unpack(xn1[0, :, 0:SUB]),
                preferred_element_type=F32)
        ffn_down(h, _mod(n, NT), c)

    def loop(lo, hi, do_attn, do_proj, unroll):
        def step(m, carry):
            k0 = m * unroll
            for u in range(unroll):
                start_out(k0 + u)
            for u in range(unroll):
                body(k0 + u, do_attn, do_proj)
            if lo == 0:
                assert unroll == 1

                @pl.when(k0 + 1 < NCH)
                def _():
                    for which in range(3):
                        f_copy(which, k0 + 1).wait()


                @pl.when(k0 + unroll == NS - NCH)
                def _():
                    fill_clamped(ring, (NS - 1) % RING, NS % RING)
            return carry
        assert lo % unroll == 0 and hi % unroll == 0 and NCH % unroll == 0
        jax.lax.fori_loop(lo // unroll, hi // unroll, step, 0)

    with jax.named_scope("s_main"):
        loop(0, 2 * NS - n_pro, True, True, UNROLL[0])
    with jax.named_scope("s_mid"):
        loop(2 * NS - n_pro, 2 * NS - NCH, True, False, UNROLL[1])
    with jax.named_scope("s_last"):
        loop(2 * NS - NCH, 2 * NS, False, False, UNROLL[2])
    with jax.named_scope("s_tail"):
        for p in range(NS - NCH, NS):
            out_copy(p).start()
        for p in range(NS):
            out_copy(p).wait()


@jax.jit
def pallas_interleave_layers__sliding_local_dilated__glu_gated_bilinear__prompt_kernel(
    A_x: jax.Array,
    A_wqkv: jax.Array,
    A_wo: jax.Array,
    B_x: jax.Array,
    B_w_gate: jax.Array,
    B_w_up: jax.Array,
    B_w_down: jax.Array,
):
    del B_x
    xT = A_x.reshape(S, D).T
    wdT = B_w_down.T
    any_spec = pl.BlockSpec(memory_space=pl.ANY)
    outT = pl.pallas_call(
        _kernel,
        in_specs=[any_spec] * 6,
        out_specs=any_spec,
        out_shape=jax.ShapeDtypeStruct((D, S), BF16),
        scratch_shapes=[
            pltpu.VMEM((NS, D, SUB), F32),
            pltpu.VMEM((NS, D, SUB), BF16),
            pltpu.VMEM((D, 3 * D), BF16),
            pltpu.VMEM((D, D), BF16),
            pltpu.VMEM((NCH, D, FC), BF16),
            pltpu.VMEM((NCH, D, FC), BF16),
            pltpu.VMEM((NCH, D, FC), BF16),
            pltpu.VMEM((3 * D // 2, D), U32),
            pltpu.VMEM((D // 2, D), U32),
            pltpu.VMEM((NCH + 1, 3 * D, LANES), F32),
            pltpu.VMEM((RING, 3 * D, LANES), F32),
            pltpu.VMEM((PT, D // 2, TM), U32),
            pltpu.VMEM((2, TM // 2, D), U32),
            pltpu.SMEM((H // HG,), jnp.int32),
            pltpu.SMEM((2,), jnp.int32),
            pltpu.SemaphoreType.DMA((NS + NP + 1 + 3 * NCH,)),
            pltpu.SemaphoreType.DMA((NS,)),
        ],
        compiler_params=pltpu.CompilerParams(
            vmem_limit_bytes=100 * 1024 * 1024),
    )(xT, A_wqkv, A_wo, B_w_gate, B_w_up, wdT)
    return outT.T.reshape(1, S, D)
```

```python
import jax
import jax.numpy as jnp
import jax.experimental.pallas as pl
import jax.experimental.pallas.tpu as pltpu

S = 2048
D = 576
F = 4608
H = 32
DH = 18
W = 8
DIL = 2
EPS = 1e-5
LANES = 128

TM = 512
NT = S // TM
FC = 1152
NCH = F // FC
SUB = TM // NCH
NS = S // SUB
HG = 8
OPAQUE = 1
SB = 5
UNROLL = (1, 1, 2)
RING = 16
PIECES = (0, 256, 640, 1152, 1728)
LAG = 128
MC = 256
AHEAD = 1
SB0 = 18
PT = 3
OW = 4
LN_SPLIT = 2
ACC0 = (4, 4)
ACCP = (1, 1)
ACC1 = (1, 1)
ACC2 = (1, 1)
RL1 = 0
RL2 = 1
RL0 = 0
LW = 2
XW = 1
LN2_AT = (2, 4, 6, 8)
X1_AT = 3
LASTP = 432
NP = len(PIECES) - 1

SCALE = DH ** -0.5
EXP2_SCALE = SCALE * 1.4426950408889634
MASKED_LOGIT = -1e9 / SCALE

NT_DIMS = (((1,), (1,)), ((), ()))
F32 = jnp.float32
BF16 = jnp.bfloat16
U32 = jnp.uint32


def _mod(a, n):
    assert n & (n - 1) == 0
    return jax.lax.bitwise_and(a, n - 1)


def _div(a, n):
    assert n & (n - 1) == 0
    return jax.lax.shift_right_logical(a, n.bit_length() - 1)


def _pack(x):
    return pltpu.bitcast(x, U32)


def _unpack(x):
    return pltpu.bitcast(x, BF16)


def _mean_rows(x, acc):
    part = jnp.sum(x.reshape(D // (8 * acc), 8 * acc, x.shape[1]), axis=0)
    return jnp.sum(part, axis=0, keepdims=True) * (1.0 / D)


def _layernorm(x, acc, reread=None):
    m = _mean_rows(x, acc[0])
    c = (x if reread is None else reread(0)) - m
    v = _mean_rows(c * c, acc[1])
    if reread is not None:
        c = reread(1) - m
    y = c * jax.lax.rsqrt(v + EPS)
    return y.astype(BF16)


def _kernel(xT_hbm, wqkv_hbm, wo_hbm, wg_hbm, wu_hbm, wdT_hbm, out_hbm,
            xres, xio, wqkv_raw, wo_raw, wg, wu, wd,
            wqT, woT, first, ring, xn1, xn2, row_s, zero_s, sem_in, sem_o):

    def x_copy(p):
        start = p * SUB
        if not isinstance(p, int):
            start = pl.multiple_of(start, LANES)
        return pltpu.make_async_copy(
            xT_hbm.at[:, pl.ds(start, SUB)], xio.at[p], sem_in.at[p])

    def f_copy(which, c):
        src = (wg_hbm, wu_hbm, wdT_hbm)[which]
        dst = (wg, wu, wd)[which]
        start = c * FC
        if not isinstance(c, int):
            start = pl.multiple_of(start, LANES)
        return pltpu.make_async_copy(
            src.at[:, pl.ds(start, FC)], dst.at[c],
            sem_in.at[NS + NP + 1 + which * NCH + c])

    def out_copy(p):
        start = p * SUB
        if not isinstance(p, int):
            start = pl.multiple_of(start, LANES)
        return pltpu.make_async_copy(
            xio.at[p], out_hbm.at[:, pl.ds(start, SUB)], sem_o.at[p])

    def wqkv_copy(j):
        cols = pl.ds(PIECES[j], PIECES[j + 1] - PIECES[j])
        return pltpu.make_async_copy(
            wqkv_hbm.at[:, cols], wqkv_raw.at[:, cols], sem_in.at[NS + j])

    wo_copy = pltpu.make_async_copy(wo_hbm, wo_raw, sem_in.at[NS + NP])

    def transpose_cols(src, dst, lo, hi):
        for c0 in range(lo, hi, LANES):
            c1 = min(c0 + LANES, hi)
            dst[c0 // 2:c1 // 2, :] = _pack(src[:, c0:c1].T)

    lane = jax.lax.broadcasted_iota(jnp.int32, (HG, LANES), 1)

    def shifted(cur, prev, w):
        if w == 0:
            return cur
        both = jnp.where(lane < LANES - DIL * w, cur, prev)
        return pltpu.roll(both, DIL * w, 1)

    def rows(base, part, d):
        return pl.ds(base + part * D + d, HG, stride=DH)

    def attn_scores(cur, prev, p, base):
        first = isinstance(p, int) and p == 0
        logits = [None] * W
        for d in range(DH):
            q = cur[rows(base, 0, d), :]
            kc = cur[rows(base, 1, d), :]
            kp = kc if first else prev[rows(base, 1, d), :]
            for w in range(W):
                t = q * shifted(kc, kp, w)
                logits[w] = t if d == 0 else logits[w] + t
        if first or not isinstance(p, int):
            pos = p * SUB + lane
            for w in range(1, W):
                logits[w] = jnp.where(pos >= DIL * w, logits[w], MASKED_LOGIT)
        m = logits[0]
        for w in range(1, W):
            m = jnp.maximum(m, logits[w])
        es = [jnp.exp2((lg - m) * EXP2_SCALE) for lg in logits]
        s = es[0]
        for w in range(1, W):
            s = s + es[w]
        r = 1.0 / s
        return [e * r for e in es]

    def attn_values(cur, prev, base, a, sb):
        done = []
        for d in range(DH):
            vc = cur[rows(base, 2, d), :]
            vp = prev[rows(base, 2, d), :]
            o = a[0] * vc
            for w in range(1, W):
                o = o + a[w] * shifted(vc, vp, w)
            done.append((d, o))
            if len(done) == sb or d == DH - 1:
                for dd, oo in done:
                    cur[rows(base, 0, dd), :] = oo
                done = []

    def attention(cur, prev, p):
        for g in range(H // HG):
            base = row_s[g] if OPAQUE else g * HG * DH
            attn_values(cur, prev, base, attn_scores(cur, prev, p, base), SB)

    def fill_clamped(buf, dst, src):
        buf[dst, 2 * D:3 * D, :] = jnp.broadcast_to(
            buf[src, 2 * D:3 * D, 0:1], (D, LANES))

    def residual(p, from_input):
        if from_input is True:
            return xio[p].astype(F32)
        if from_input is False:
            return xres[p]
        return jnp.where(from_input, xio[p].astype(F32), xres[p])

    def out_proj(qkv, p, from_input, slot, row0):
        upd = jnp.dot(_unpack(woT[...]), qkv[0:D, :].astype(BF16),
                      preferred_element_type=F32)
        x = residual(p, from_input) + upd
        xres[p] = x
        again = (lambda i: xres[p + zero_s[i]]) if RL2 else None
        xn2[slot, pl.ds(row0, SUB // 2), :] = _pack(
            _layernorm(x, ACC2, again).T)

    def ln1(p, from_input, acc, reread):
        again = lambda i: residual(p + zero_s[i], from_input)
        return _layernorm(residual(p, from_input), acc,
                          again if reread else None)

    def ffn_up(slot, c):
        xn = _unpack(xn2[slot])
        g = jnp.dot(xn, wg[c], preferred_element_type=F32)
        u = jnp.dot(xn, wu[c], preferred_element_type=F32)
        return (g * u).astype(BF16)

    def ffn_down(h, t, c):
        res = jax.lax.dot_general(wd[c], h, NT_DIMS,
                                  preferred_element_type=F32)
        for i in range(NCH):
            x = xres[t * NCH + i] + res[:, i * SUB:(i + 1) * SUB]
            xres[t * NCH + i] = x
            xio[t * NCH + i] = x.astype(BF16)

    def ln1_tile(t, lo=0, hi=NCH):
        for i in range(lo, hi):
            xn1[t, :, i * SUB:(i + 1) * SUB] = _pack(ln1(
                t * NCH + i, True, ACCP if t else ACC0, RL0 and t > 0))

    def project_tile(t, lo, hi, mc=3 * D):
        for m0 in range(lo, hi, mc):
            m1 = min(m0 + mc, hi)
            res = jnp.dot(_unpack(wqT[m0 // 2:m1 // 2, :]), _unpack(xn1[t]),
                          preferred_element_type=F32)
            for i in range(NCH):
                part = res[:, i * SUB:(i + 1) * SUB]
                if t == 0:
                    first[i, m0:m1, :] = part
                if t > 0 or (i == NCH - 1 and m1 > D):
                    ring[t * NCH + i, m0:m1, :] = part

    def out_proj0(lo, hi):
        o = jnp.concatenate(
            [first[i, 0:D, :].astype(BF16) for i in range(lo, hi)], axis=1)
        upd = jnp.dot(_unpack(woT[...]), o, preferred_element_type=F32)
        for i in range(lo, hi):
            x = residual(i, True) + upd[:, (i - lo) * SUB:(i - lo + 1) * SUB]
            xres[i] = x
            again = (lambda j, i=i: xres[i + zero_s[j]]) if RL0 else None
            xn2[0, i * SUB // 2:(i + 1) * SUB // 2, :] = _pack(
                _layernorm(x, ACCP, again).T)

    n_pro = PT * NCH
    for p in range(NCH):
        x_copy(p).start()
    for j in range(NP):
        wqkv_copy(j).start()
        if j == X1_AT:
            for p in range(NCH, 2 * NCH):
                x_copy(p).start()
    wo_copy.start()
    for p in range(2 * NCH, n_pro):
        x_copy(p).start()
    for c in range(NCH):
        for which in range(3):
            f_copy(which, c).start()
        if c == 0:
            for p in range(n_pro, NS):
                x_copy(p).start()
    for g in range(H // HG):
        row_s[g] = g * HG * DH
    zero_s[0] = 0
    zero_s[1] = 0

    def unit0(u):
        i, g = divmod(u, H // HG)
        return first.at[i], first.at[i - 1 if i else NCH], i, row_s[g]

    with jax.named_scope("s_ln"):
        for p0 in range(0, NCH, XW):
            for p in range(p0, p0 + XW):
                x_copy(p).wait()
            ln1_tile(0, p0, p0 + XW)
    done = 0
    for j in range(NP):
        with jax.named_scope(f"s_w{j}"):
            wqkv_copy(j).wait()
            if j == X1_AT:
                for p in range(NCH, 2 * NCH):
                    x_copy(p).wait()
        with jax.named_scope(f"s_b{j}"):
            project_tile(0, done, PIECES[j], MC)
            transpose_cols(wqkv_raw, wqT, PIECES[j], PIECES[j + 1])
            done = PIECES[j + 1] - (LAG if j < NP - 1 else 0)
            project_tile(0, PIECES[j], done, MC if j else LANES)
            if j == X1_AT:
                ln1_tile(1, 0, LN_SPLIT)
            if j == NP - 1:
                ln1_tile(1, LN_SPLIT, NCH)
    with jax.named_scope("s_wo"):
        wo_copy.wait()
        for p in range(2 * NCH, n_pro):
            x_copy(p).wait()
    with jax.named_scope("s_stage0"):
        fill_clamped(first, NCH, 0)
        project_tile(1, 0, 3 * D)
        n_units = NCH * H // HG
        sc = [attn_scores(*unit0(u)) for u in range(AHEAD)]
        for u in range(n_units):
            if u + AHEAD < n_units:
                sc.append(attn_scores(*unit0(u + AHEAD)))
            cur, prev, _, base = unit0(u)
            attn_values(cur, prev, base, sc[u], SB0)
            for i in range(NCH):
                if LN2_AT[i] == u:
                    y = ln1(2 * NCH + i, True, ACCP, RL0)
                    xn1[2, :, i * SUB:(i + 1) * SUB] = _pack(y)
                    first[NCH, 0:16, :] = y[D - 16:D, :].astype(F32)
        project_tile(2, 0, 3 * D - LASTP)
        transpose_cols(wo_raw, woT, 0, D)
        out_proj0(0, NCH)
        project_tile(2, 3 * D - LASTP, 3 * D)
        for which in range(3):
            f_copy(which, 0).wait()
        for p in range(n_pro, NS):
            x_copy(p).wait()

    def start_out(k):
        @pl.when(k >= NS + NCH)
        def _():
            out_copy(k - NS - NCH).start()

    def body(k, do_attn, do_proj):
        n = _div(k, NCH)
        c = _mod(k, NCH)
        if do_proj:
            xn1[0, :, 0:SUB] = _pack(
                ln1(_mod(k + n_pro, NS), k + n_pro < NS, ACC1, RL1))
        h = ffn_up(_mod(n, 2), c)
        if do_attn:
            p = _mod(k + NCH, NS)
            cur = ring.at[_mod(k + NCH, RING)]
            attention(cur, ring.at[_mod(k + NCH - 1, RING)], p)
            out_proj(cur, p, do_proj and k + NCH < NS, _mod(n + 1, 2),
                     pl.multiple_of(c * (SUB // 2), SUB // 2))
        if do_proj:
            ring[_mod(k + n_pro, RING)] = jnp.dot(
                _unpack(wqT[...]), _unpack(xn1[0, :, 0:SUB]),
                preferred_element_type=F32)
        ffn_down(h, _mod(n, NT), c)

    def loop(lo, hi, do_attn, do_proj, unroll):
        def step(m, carry):
            k0 = m * unroll
            for u in range(unroll):
                start_out(k0 + u)
            for u in range(unroll):
                body(k0 + u, do_attn, do_proj)
            if lo == 0:
                assert unroll == 1

                @pl.when(k0 + 1 < NCH)
                def _():
                    for which in range(3):
                        f_copy(which, k0 + 1).wait()


                @pl.when(k0 + unroll == NS - NCH)
                def _():
                    fill_clamped(ring, (NS - 1) % RING, NS % RING)
            return carry
        assert lo % unroll == 0 and hi % unroll == 0 and NCH % unroll == 0
        jax.lax.fori_loop(lo // unroll, hi // unroll, step, 0)

    with jax.named_scope("s_main"):
        loop(0, 2 * NS - n_pro, True, True, UNROLL[0])
    with jax.named_scope("s_mid"):
        loop(2 * NS - n_pro, 2 * NS - NCH, True, False, UNROLL[1])
    def last_step(m, carry):
        @pl.when(m == 0)
        def _():
            for p in range(NS - 2 * NCH, NS - NCH):
                out_copy(p).start()

        p0 = NS - NCH + m * LW

        @pl.when(m > 0)
        def _():
            for i in range(LW):
                out_copy(p0 - LW + i).start()

        half = LW * SUB // 2
        xn = _unpack(xn2[(2 * NT - 1) % 2,
                         pl.ds(pl.multiple_of(m * half, half), half), :])
        res = None
        for c in range(NCH):
            g = jnp.dot(xn, wg[c], preferred_element_type=F32)
            u = jnp.dot(xn, wu[c], preferred_element_type=F32)
            part = jax.lax.dot_general(wd[c], (g * u).astype(BF16), NT_DIMS,
                                       preferred_element_type=F32)
            res = part if res is None else res + part
        for i in range(LW):
            x = xres[p0 + i] + res[:, i * SUB:(i + 1) * SUB]
            xio[p0 + i] = x.astype(BF16)
        return carry

    with jax.named_scope("s_last"):
        jax.lax.fori_loop(0, NCH // LW, last_step, 0)
    with jax.named_scope("s_tail"):
        for p in range(NS - LW, NS):
            out_copy(p).start()
        for p in range(NS):
            out_copy(p).wait()


@jax.jit
def pallas_interleave_layers__sliding_local_dilated__glu_gated_bilinear__prompt_kernel(
    A_x: jax.Array,
    A_wqkv: jax.Array,
    A_wo: jax.Array,
    B_x: jax.Array,
    B_w_gate: jax.Array,
    B_w_up: jax.Array,
    B_w_down: jax.Array,
):
    del B_x
    xT = A_x.reshape(S, D).T
    wdT = B_w_down.T
    any_spec = pl.BlockSpec(memory_space=pl.ANY)
    outT = pl.pallas_call(
        _kernel,
        in_specs=[any_spec] * 6,
        out_specs=any_spec,
        out_shape=jax.ShapeDtypeStruct((D, S), BF16),
        scratch_shapes=[
            pltpu.VMEM((NS, D, SUB), F32),
            pltpu.VMEM((NS, D, SUB), BF16),
            pltpu.VMEM((D, 3 * D), BF16),
            pltpu.VMEM((D, D), BF16),
            pltpu.VMEM((NCH, D, FC), BF16),
            pltpu.VMEM((NCH, D, FC), BF16),
            pltpu.VMEM((NCH, D, FC), BF16),
            pltpu.VMEM((3 * D // 2, D), U32),
            pltpu.VMEM((D // 2, D), U32),
            pltpu.VMEM((NCH + 1, 3 * D, LANES), F32),
            pltpu.VMEM((RING, 3 * D, LANES), F32),
            pltpu.VMEM((PT, D // 2, TM), U32),
            pltpu.VMEM((2, TM // 2, D), U32),
            pltpu.SMEM((H // HG,), jnp.int32),
            pltpu.SMEM((2,), jnp.int32),
            pltpu.SemaphoreType.DMA((NS + NP + 1 + 3 * NCH,)),
            pltpu.SemaphoreType.DMA((NS,)),
        ],
        compiler_params=pltpu.CompilerParams(
            vmem_limit_bytes=100 * 1024 * 1024),
    )(xT, A_wqkv, A_wo, B_w_gate, B_w_up, wdT)
    return outT.T.reshape(1, S, D)
```

```python
import jax
import jax.numpy as jnp
import jax.experimental.pallas as pl
import jax.experimental.pallas.tpu as pltpu

S = 2048
D = 576
F = 4608
H = 32
DH = 18
W = 8
DIL = 2
EPS = 1e-5
LANES = 128

TM = 512
NT = S // TM
FC = 1152
NCH = F // FC
SUB = TM // NCH
NS = S // SUB
HG = 8
OPAQUE = 1
SB = 5
RING = 16
PIECES = (0, 256, 640, 1152, 1728)
LAG = 128
MC = 256
AHEAD = 1
PT = 3
ACC0 = (4, 4)
ACCP = (1, 1)
ACC1 = (1, 1)
ACC2 = (1, 1)
RL1 = 0
RL2 = 1
RL0 = 0
XE = 2
PLAN = {0: [("P", (4, 6, 0, 1728))], 1: [("L", 6)], 2: [("L", 7)], 3: [("L", 8)], 4: [("L", 9), ("P", (6, 10, 0, 1728))], 8: [("L", 10)], 10: [("L", 11)], 16: [("P", (10, 12, 0, 864)), ("T", 0), ("O", (0, 4)), ("P", (10, 12, 864, 1728))]}
MC2 = 288
RLO = 0
LW = 2
NP = len(PIECES) - 1

SCALE = DH ** -0.5
EXP2_SCALE = SCALE * 1.4426950408889634
MASKED_LOGIT = -1e9 / SCALE

NT_DIMS = (((1,), (1,)), ((), ()))
F32 = jnp.float32
BF16 = jnp.bfloat16
U32 = jnp.uint32


def _mod(a, n):
    assert n & (n - 1) == 0
    return jax.lax.bitwise_and(a, n - 1)


def _div(a, n):
    assert n & (n - 1) == 0
    return jax.lax.shift_right_logical(a, n.bit_length() - 1)


def _pack(x):
    return pltpu.bitcast(x, U32)


def _unpack(x):
    return pltpu.bitcast(x, BF16)


def _mean_rows(x, acc):
    part = jnp.sum(x.reshape(D // (8 * acc), 8 * acc, x.shape[1]), axis=0)
    return jnp.sum(part, axis=0, keepdims=True) * (1.0 / D)


def _layernorm(x, acc, reread=None):
    m = _mean_rows(x, acc[0])
    c = (x if reread is None else reread(0)) - m
    v = _mean_rows(c * c, acc[1])
    if reread is not None:
        c = reread(1) - m
    y = c * jax.lax.rsqrt(v + EPS)
    return y.astype(BF16)


def _kernel(xT_hbm, wqkv_hbm, wo_hbm, wg_hbm, wu_hbm, wdT_hbm, out_hbm,
            xres, xio, wqkv_raw, wo_raw, wg, wu, wd,
            wqT, woT, first, ring, xn1, xn2, row_s, zero_s, sem_in, sem_o):

    def x_copy(p):
        start = p * SUB
        if not isinstance(p, int):
            start = pl.multiple_of(start, LANES)
        return pltpu.make_async_copy(
            xT_hbm.at[:, pl.ds(start, SUB)], xio.at[p], sem_in.at[p])

    def f_copy(which, c):
        src = (wg_hbm, wu_hbm, wdT_hbm)[which]
        dst = (wg, wu, wd)[which]
        start = c * FC
        if not isinstance(c, int):
            start = pl.multiple_of(start, LANES)
        return pltpu.make_async_copy(
            src.at[:, pl.ds(start, FC)], dst.at[c],
            sem_in.at[NS + NP + 1 + which * NCH + c])

    def out_copy(p):
        start = p * SUB
        if not isinstance(p, int):
            start = pl.multiple_of(start, LANES)
        return pltpu.make_async_copy(
            xio.at[p], out_hbm.at[:, pl.ds(start, SUB)], sem_o.at[p])

    def wqkv_copy(j):
        cols = pl.ds(PIECES[j], PIECES[j + 1] - PIECES[j])
        return pltpu.make_async_copy(
            wqkv_hbm.at[:, cols], wqkv_raw.at[:, cols], sem_in.at[NS + j])

    wo_copy = pltpu.make_async_copy(wo_hbm, wo_raw, sem_in.at[NS + NP])

    def transpose_cols(src, dst, lo, hi):
        for c0 in range(lo, hi, LANES):
            c1 = min(c0 + LANES, hi)
            dst[c0 // 2:c1 // 2, :] = _pack(src[:, c0:c1].T)

    lane = jax.lax.broadcasted_iota(jnp.int32, (HG, LANES), 1)

    def shifted(cur, prev, w):
        if w == 0:
            return cur
        both = jnp.where(lane < LANES - DIL * w, cur, prev)
        return pltpu.roll(both, DIL * w, 1)

    def rows(base, part, d):
        return pl.ds(base + part * D + d, HG, stride=DH)

    def attn_scores(cur, prev, p, base):
        first = isinstance(p, int) and p == 0
        logits = [None] * W
        for d in range(DH):
            q = cur[rows(base, 0, d), :]
            kc = cur[rows(base, 1, d), :]
            kp = kc if first else prev[rows(base, 1, d), :]
            for w in range(W):
                t = q * shifted(kc, kp, w)
                logits[w] = t if d == 0 else logits[w] + t
        if first or not isinstance(p, int):
            pos = p * SUB + lane
            for w in range(1, W):
                logits[w] = jnp.where(pos >= DIL * w, logits[w], MASKED_LOGIT)
        m = logits[0]
        for w in range(1, W):
            m = jnp.maximum(m, logits[w])
        es = [jnp.exp2((lg - m) * EXP2_SCALE) for lg in logits]
        s = es[0]
        for w in range(1, W):
            s = s + es[w]
        r = 1.0 / s
        return [e * r for e in es]

    def attn_values(cur, prev, base, a, sb):
        done = []
        for d in range(DH):
            vc = cur[rows(base, 2, d), :]
            vp = prev[rows(base, 2, d), :]
            o = a[0] * vc
            for w in range(1, W):
                o = o + a[w] * shifted(vc, vp, w)
            done.append((d, o))
            if len(done) == sb or d == DH - 1:
                for dd, oo in done:
                    cur[rows(base, 0, dd), :] = oo
                done = []

    def attention(cur, prev, p):
        for g in range(H // HG):
            base = row_s[g] if OPAQUE else g * HG * DH
            attn_values(cur, prev, base, attn_scores(cur, prev, p, base), SB)

    def fill_clamped(buf, dst, src):
        buf[dst, 2 * D:3 * D, :] = jnp.broadcast_to(
            buf[src, 2 * D:3 * D, 0:1], (D, LANES))

    def residual(p, from_input):
        if from_input is True:
            return xio[p].astype(F32)
        if from_input is False:
            return xres[p]
        return jnp.where(from_input, xio[p].astype(F32), xres[p])

    def out_proj(qkv, p, from_input, slot, row0):
        upd = jnp.dot(_unpack(woT[...]), qkv[0:D, :].astype(BF16),
                      preferred_element_type=F32)
        x = residual(p, from_input) + upd
        xres[p] = x
        again = (lambda i: xres[p + zero_s[i]]) if RL2 else None
        xn2[slot, pl.ds(row0, SUB // 2), :] = _pack(
            _layernorm(x, ACC2, again).T)

    def ln1(p, from_input, acc, reread):
        again = lambda i: residual(p + zero_s[i], from_input)
        return _layernorm(residual(p, from_input), acc,
                          again if reread else None)

    def ffn_up(slot, c):
        xn = _unpack(xn2[slot])
        g = jnp.dot(xn, wg[c], preferred_element_type=F32)
        u = jnp.dot(xn, wu[c], preferred_element_type=F32)
        return (g * u).astype(BF16)

    def ffn_down(h, t, c):
        res = jax.lax.dot_general(wd[c], h, NT_DIMS,
                                  preferred_element_type=F32)
        for i in range(NCH):
            x = xres[t * NCH + i] + res[:, i * SUB:(i + 1) * SUB]
            xres[t * NCH + i] = x
            xio[t * NCH + i] = x.astype(BF16)

    def ln1_pro(p):
        y = ln1(p, True, ACCP if p >= NCH else ACC0, RL0 and p >= NCH)
        xn1[:, p * SUB:(p + 1) * SUB] = _pack(y)
        return y

    def project_pro(p0, p1, lo, hi, mc=3 * D):
        for m0 in range(lo, hi, mc):
            m1 = min(m0 + mc, hi)
            res = jnp.dot(_unpack(wqT[m0 // 2:m1 // 2, :]),
                          _unpack(xn1[:, p0 * SUB:p1 * SUB]),
                          preferred_element_type=F32)
            for p in range(p0, p1):
                part = res[:, (p - p0) * SUB:(p - p0 + 1) * SUB]
                if p < NCH:
                    first[p, m0:m1, :] = part
                if p >= NCH or (p == NCH - 1 and m1 > D):
                    ring[p, m0:m1, :] = part

    def out_proj0(lo, hi):
        o = jnp.concatenate(
            [first[i, 0:D, :].astype(BF16) for i in range(lo, hi)], axis=1)
        upd = jnp.dot(_unpack(woT[...]), o, preferred_element_type=F32)
        for i in range(lo, hi):
            x = residual(i, True) + upd[:, (i - lo) * SUB:(i - lo + 1) * SUB]
            xres[i] = x
            again = (lambda j, i=i: xres[i + zero_s[j]]) if RLO else None
            xn2[0, i * SUB // 2:(i + 1) * SUB // 2, :] = _pack(
                _layernorm(x, ACCP, again).T)

    n_pro = PT * NCH
    for p in range(NCH):
        x_copy(p).start()
    for j in range(NP):
        wqkv_copy(j).start()
    for p in range(NCH, NCH + XE):
        x_copy(p).start()
    wo_copy.start()
    for p in range(NCH + XE, n_pro):
        x_copy(p).start()
    for c in range(NCH):
        for which in range(3):
            f_copy(which, c).start()
        if c == 0:
            for p in range(n_pro, NS):
                x_copy(p).start()
    for g in range(H // HG):
        row_s[g] = g * HG * DH
    zero_s[0] = 0
    zero_s[1] = 0

    def unit0(u):
        i, g = divmod(u, H // HG)
        return first.at[i], first.at[i - 1 if i else NCH], i, row_s[g]

    with jax.named_scope("s_ln"):
        for p in range(NCH):
            x_copy(p).wait()
            ln1_pro(p)
    done = 0
    for j in range(NP):
        with jax.named_scope(f"s_w{j}"):
            wqkv_copy(j).wait()
            if j == NP - 1:
                for p in range(NCH, NCH + XE):
                    x_copy(p).wait()
        with jax.named_scope(f"s_b{j}"):
            project_pro(0, NCH, done, PIECES[j], MC)
            transpose_cols(wqkv_raw, wqT, PIECES[j], PIECES[j + 1])
            done = PIECES[j + 1] - (LAG if j < NP - 1 else 0)
            project_pro(0, NCH, PIECES[j], done, MC if j else LANES)
            if j == NP - 1:
                for p in range(NCH, NCH + XE):
                    ln1_pro(p)
    with jax.named_scope("s_wo"):
        wo_copy.wait()
        for p in range(NCH + XE, n_pro):
            x_copy(p).wait()
    with jax.named_scope("s_stage0"):
        fill_clamped(first, NCH, 0)
        n_units = NCH * H // HG
        sc = [attn_scores(*unit0(u)) for u in range(AHEAD)]
        for u in range(n_units + 1):
            for kind, arg in PLAN.get(u, ()):
                if kind == "P":
                    project_pro(*arg, MC2)
                elif kind == "O":
                    out_proj0(*arg)
                elif kind == "T":
                    transpose_cols(wo_raw, woT, 0, D)
                else:
                    y = ln1_pro(arg)
                    first[NCH, 0:16, :] = y[D - 16:D, :].astype(F32)
            if u == n_units:
                break
            if u + AHEAD < n_units:
                sc.append(attn_scores(*unit0(u + AHEAD)))
            cur, prev, _, base = unit0(u)
            attn_values(cur, prev, base, sc[u], DH)
        for which in range(3):
            f_copy(which, 0).wait()
        for p in range(n_pro, NS):
            x_copy(p).wait()

    def body(k, do_proj):
        n = _div(k, NCH)
        c = _mod(k, NCH)
        if do_proj:
            xn1[:, 0:SUB] = _pack(
                ln1(_mod(k + n_pro, NS), k + n_pro < NS, ACC1, RL1))
        h = ffn_up(_mod(n, 2), c)
        p = _mod(k + NCH, NS)
        cur = ring.at[_mod(k + NCH, RING)]
        attention(cur, ring.at[_mod(k + NCH - 1, RING)], p if do_proj else 1)
        out_proj(cur, p, do_proj and k + NCH < NS, _mod(n + 1, 2),
                 pl.multiple_of(c * (SUB // 2), SUB // 2))
        if do_proj:
            ring[_mod(k + n_pro, RING)] = jnp.dot(
                _unpack(wqT[...]), _unpack(xn1[:, 0:SUB]),
                preferred_element_type=F32)
        ffn_down(h, _mod(n, NT), c)

    n_main = 2 * NS - n_pro
    assert n_main == NS + NCH

    def main_step(k, carry):
        body(k, True)
        return carry

    def segment(i, lo):
        hi = jnp.where(i < NCH - 1, i + 1,
                       jnp.where(i == NCH - 1, NS - NCH, n_main))
        jax.lax.fori_loop(lo, hi, main_step, 0)

        @pl.when(i < NCH - 1)
        def _():
            for which in range(3):
                f_copy(which, i + 1).wait()

        @pl.when(i == NCH - 1)
        def _():
            fill_clamped(ring, (NS - 1) % RING, NS % RING)

        return hi

    def mid_step(k, carry):
        out_copy(k - n_main).start()
        body(k, False)
        return carry

    with jax.named_scope("s_main"):
        jax.lax.fori_loop(0, NCH + 1, segment, 0)
    with jax.named_scope("s_mid"):
        jax.lax.fori_loop(n_main, 2 * NS - NCH, mid_step, 0)

    def last_step(m, carry):
        @pl.when(m == 0)
        def _():
            for p in range(NS - 2 * NCH, NS - NCH):
                out_copy(p).start()

        p0 = NS - NCH + m * LW

        @pl.when(m > 0)
        def _():
            for i in range(LW):
                out_copy(p0 - LW + i).start()

        half = LW * SUB // 2
        xn = _unpack(xn2[(2 * NT - 1) % 2,
                         pl.ds(pl.multiple_of(m * half, half), half), :])
        res = None
        for c in range(NCH):
            g = jnp.dot(xn, wg[c], preferred_element_type=F32)
            u = jnp.dot(xn, wu[c], preferred_element_type=F32)
            part = jax.lax.dot_general(wd[c], (g * u).astype(BF16), NT_DIMS,
                                       preferred_element_type=F32)
            res = part if res is None else res + part
        for i in range(LW):
            x = xres[p0 + i] + res[:, i * SUB:(i + 1) * SUB]
            xio[p0 + i] = x.astype(BF16)
        return carry

    with jax.named_scope("s_last"):
        jax.lax.fori_loop(0, NCH // LW, last_step, 0)
    with jax.named_scope("s_tail"):
        for p in range(NS - LW, NS):
            out_copy(p).start()
        for p in range(NS):
            out_copy(p).wait()


@jax.jit
def pallas_interleave_layers__sliding_local_dilated__glu_gated_bilinear__prompt_kernel(
    A_x: jax.Array,
    A_wqkv: jax.Array,
    A_wo: jax.Array,
    B_x: jax.Array,
    B_w_gate: jax.Array,
    B_w_up: jax.Array,
    B_w_down: jax.Array,
):
    del B_x
    xT = A_x.reshape(S, D).T
    wdT = B_w_down.T
    any_spec = pl.BlockSpec(memory_space=pl.ANY)
    outT = pl.pallas_call(
        _kernel,
        in_specs=[any_spec] * 6,
        out_specs=any_spec,
        out_shape=jax.ShapeDtypeStruct((D, S), BF16),
        scratch_shapes=[
            pltpu.VMEM((NS, D, SUB), F32),
            pltpu.VMEM((NS, D, SUB), BF16),
            pltpu.VMEM((D, 3 * D), BF16),
            pltpu.VMEM((D, D), BF16),
            pltpu.VMEM((NCH, D, FC), BF16),
            pltpu.VMEM((NCH, D, FC), BF16),
            pltpu.VMEM((NCH, D, FC), BF16),
            pltpu.VMEM((3 * D // 2, D), U32),
            pltpu.VMEM((D // 2, D), U32),
            pltpu.VMEM((NCH + 1, 3 * D, LANES), F32),
            pltpu.VMEM((RING, 3 * D, LANES), F32),
            pltpu.VMEM((D // 2, PT * TM), U32),
            pltpu.VMEM((2, TM // 2, D), U32),
            pltpu.SMEM((H // HG,), jnp.int32),
            pltpu.SMEM((2,), jnp.int32),
            pltpu.SemaphoreType.DMA((NS + NP + 1 + 3 * NCH,)),
            pltpu.SemaphoreType.DMA((NS,)),
        ],
        compiler_params=pltpu.CompilerParams(
            vmem_limit_bytes=100 * 1024 * 1024),
    )(xT, A_wqkv, A_wo, B_w_gate, B_w_up, wdT)
    return outT.T.reshape(1, S, D)
```

```python
import jax
import jax.numpy as jnp
import jax.experimental.pallas as pl
import jax.experimental.pallas.tpu as pltpu

S = 2048
D = 576
F = 4608
H = 32
DH = 18
W = 8
DIL = 2
EPS = 1e-5
LANES = 128

TM = 512
NT = S // TM
FC = 1152
NCH = F // FC
SUB = TM // NCH
NS = S // SUB
HG = 8
OPAQUE = 1
SB = 5
RING = 16
PIECES = (0, 256, 640, 1152, 1728)
LAG = 128
MC = 256
AHEAD = 1
PT = 3
ACC0 = (4, 4)
ACCP = (1, 1)
ACCO = (1, 1)
ACC1 = (1, 1)
ACC2 = (1, 1)
RL1 = 0
RL2 = 1
RL0 = 0
XE = 2
PLANS = [
    {0: [("P", (4, 6, 0, 1728))], 1: [("L", 6)], 2: [("L", 7)], 3: [("L", 8)], 4: [("L", 9), ("P", (6, 10, 0, 1728))],
     16: [("N", 10), ("N", 11), ("P", (10, 12, 0, 864)), ("T", 0), ("O", (0, 4)), ("P", (10, 12, 864, 1728))]},
    {0: [("P", (4, 6, 0, 1728)), ("N", 6), ("N", 7), ("N", 8), ("N", 9), ("P", (6, 10, 0, 1728))],
     16: [("N", 10), ("N", 11), ("P", (10, 12, 0, 864)), ("T", 0), ("O", (0, 4)), ("P", (10, 12, 864, 1728))]},
    {0: [("P", (4, 6, 0, 1728)), ("N", 6), ("P", (6, 7, 0, 1728)), ("N", 7), ("P", (7, 8, 0, 1728)), ("N", 8), ("P", (8, 9, 0, 1728)),
         ("N", 9), ("P", (9, 10, 0, 1728)), ("N", 10), ("P", (10, 11, 0, 1728))],
     16: [("T", 0), ("O", (0, 4)), ("N", 11), ("P", (11, 12, 0, 1728))]},
    {0: [("P", (4, 6, 0, 1728))], 1: [("L", 6)], 2: [("L", 7)], 3: [("L", 8)], 4: [("L", 9), ("P", (6, 10, 0, 1728))],
     16: [("N", 10), ("N", 11), ("T", 0), ("O", (0, 1)), ("P", (10, 12, 0, 432)), ("O", (1, 2)), ("P", (10, 12, 432, 864)),
          ("O", (2, 3)), ("P", (10, 12, 864, 1296)), ("O", (3, 4)), ("P", (10, 12, 1296, 1728))]},
    {0: [("N", 6), ("N", 7), ("N", 8), ("N", 9), ("N", 10), ("N", 11), ("T", 0), ("P", (4, 6, 0, 1728)), ("P", (6, 10, 0, 1728)), ("P", (10, 12, 0, 864))],
     16: [("O", (0, 4)), ("P", (10, 12, 864, 1728))]},
    {0: [("N", 10), ("N", 11), ("P", (4, 6, 0, 1728))], 1: [("L", 6)], 2: [("L", 7)], 3: [("L", 8)], 4: [("L", 9), ("P", (6, 10, 0, 1728))],
     16: [("T", 0), ("O", (0, 1)), ("O", (1, 2)), ("P", (10, 12, 0, 576)),
          ("O", (2, 3)), ("P", (10, 12, 576, 1152)), ("O", (3, 4)), ("P", (10, 12, 1152, 1728))]},
    {0: [("P", (4, 6, 0, 1728))], 1: [("L", 6)], 2: [("L", 7)], 3: [("L", 8)], 4: [("L", 9), ("P", (6, 10, 0, 1728))], 5: [("L", 10)], 6: [("L", 11)],
     16: [("T", 0), ("O", (0, 1)), ("P", (10, 12, 0, 432)), ("O", (1, 2)), ("P", (10, 12, 432, 864)),
          ("O", (2, 3)), ("P", (10, 12, 864, 1296)), ("O", (3, 4)), ("P", (10, 12, 1296, 1728))]},
]
PI = 5
NOSEM = True
NOBND = False
PLAN = PLANS[PI]
MC2 = 288
RLO = 0
LW = 2
NP = len(PIECES) - 1

SCALE = DH ** -0.5
EXP2_SCALE = SCALE * 1.4426950408889634
MASKED_LOGIT = -1e9 / SCALE

NT_DIMS = (((1,), (1,)), ((), ()))
F32 = jnp.float32
BF16 = jnp.bfloat16
U32 = jnp.uint32


def _mod(a, n):
    assert n & (n - 1) == 0
    return jax.lax.bitwise_and(a, n - 1)


def _div(a, n):
    assert n & (n - 1) == 0
    return jax.lax.shift_right_logical(a, n.bit_length() - 1)


def _pack(x):
    return pltpu.bitcast(x, U32)


def _unpack(x):
    return pltpu.bitcast(x, BF16)


def _mean_rows(x, acc):
    part = jnp.sum(x.reshape(D // (8 * acc), 8 * acc, x.shape[1]), axis=0)
    return jnp.sum(part, axis=0, keepdims=True) * (1.0 / D)


def _layernorm(x, acc, reread=None):
    m = _mean_rows(x, acc[0])
    c = (x if reread is None else reread(0)) - m
    v = _mean_rows(c * c, acc[1])
    if reread is not None:
        c = reread(1) - m
    y = c * jax.lax.rsqrt(v + EPS)
    return y.astype(BF16)


def _kernel(xT_hbm, wqkv_hbm, wo_hbm, wg_hbm, wu_hbm, wdT_hbm, out_hbm,
            xres, xio, wqkv_raw, wo_raw, wg, wu, wd,
            wqT, woT, first, ring, xn1, xn2, row_s, zero_s, sem_in, sem_o):

    def x_copy(p):
        start = p * SUB
        if not isinstance(p, int):
            start = pl.multiple_of(start, LANES)
        return pltpu.make_async_copy(
            xT_hbm.at[:, pl.ds(start, SUB)], xio.at[p], sem_in.at[p])

    def f_copy(which, c):
        src = (wg_hbm, wu_hbm, wdT_hbm)[which]
        dst = (wg, wu, wd)[which]
        start = c * FC
        if not isinstance(c, int):
            start = pl.multiple_of(start, LANES)
        return pltpu.make_async_copy(
            src.at[:, pl.ds(start, FC)], dst.at[c],
            sem_in.at[NS + NP + 1 + which * NCH + c])

    def out_copy(p):
        start = p * SUB
        if not isinstance(p, int):
            start = pl.multiple_of(start, LANES)
        return pltpu.make_async_copy(
            xio.at[p], out_hbm.at[:, pl.ds(start, SUB)], sem_o.at[p])

    def wqkv_copy(j):
        cols = pl.ds(PIECES[j], PIECES[j + 1] - PIECES[j])
        return pltpu.make_async_copy(
            wqkv_hbm.at[:, cols], wqkv_raw.at[:, cols], sem_in.at[NS + j])

    wo_copy = pltpu.make_async_copy(wo_hbm, wo_raw, sem_in.at[NS + NP])

    def transpose_cols(src, dst, lo, hi):
        for c0 in range(lo, hi, LANES):
            c1 = min(c0 + LANES, hi)
            dst[c0 // 2:c1 // 2, :] = _pack(src[:, c0:c1].T)

    lane = jax.lax.broadcasted_iota(jnp.int32, (HG, LANES), 1)

    def shifted(cur, prev, w):
        if w == 0:
            return cur
        both = jnp.where(lane < LANES - DIL * w, cur, prev)
        return pltpu.roll(both, DIL * w, 1)

    def rows(base, part, d):
        return pl.ds(base + part * D + d, HG, stride=DH)

    def attn_scores(cur, prev, p, base):
        first = isinstance(p, int) and p == 0
        logits = [None] * W
        for d in range(DH):
            q = cur[rows(base, 0, d), :]
            kc = cur[rows(base, 1, d), :]
            kp = kc if first else prev[rows(base, 1, d), :]
            for w in range(W):
                t = q * shifted(kc, kp, w)
                logits[w] = t if d == 0 else logits[w] + t
        if first or not isinstance(p, int):
            pos = p * SUB + lane
            for w in range(1, W):
                logits[w] = jnp.where(pos >= DIL * w, logits[w], MASKED_LOGIT)
        m = logits[0]
        for w in range(1, W):
            m = jnp.maximum(m, logits[w])
        es = [jnp.exp2((lg - m) * EXP2_SCALE) for lg in logits]
        s = es[0]
        for w in range(1, W):
            s = s + es[w]
        r = 1.0 / s
        return [e * r for e in es]

    def attn_values(cur, prev, base, a, sb):
        done = []
        for d in range(DH):
            vc = cur[rows(base, 2, d), :]
            vp = prev[rows(base, 2, d), :]
            o = a[0] * vc
            for w in range(1, W):
                o = o + a[w] * shifted(vc, vp, w)
            done.append((d, o))
            if len(done) == sb or d == DH - 1:
                for dd, oo in done:
                    cur[rows(base, 0, dd), :] = oo
                done = []

    def attention(cur, prev, p):
        for g in range(H // HG):
            base = row_s[g] if OPAQUE else g * HG * DH
            attn_values(cur, prev, base, attn_scores(cur, prev, p, base), SB)

    def fill_clamped(buf, dst, src):
        buf[dst, 2 * D:3 * D, :] = jnp.broadcast_to(
            buf[src, 2 * D:3 * D, 0:1], (D, LANES))

    def residual(p, from_input):
        if from_input is True:
            return xio[p].astype(F32)
        if from_input is False:
            return xres[p]
        return jnp.where(from_input, xio[p].astype(F32), xres[p])

    def out_proj(qkv, p, from_input, slot, row0):
        upd = jnp.dot(_unpack(woT[...]), qkv[0:D, :].astype(BF16),
                      preferred_element_type=F32)
        x = residual(p, from_input) + upd
        xres[p] = x
        again = (lambda i: xres[p + zero_s[i]]) if RL2 else None
        xn2[slot, pl.ds(row0, SUB // 2), :] = _pack(
            _layernorm(x, ACC2, again).T)

    def ln1(p, from_input, acc, reread):
        x = residual(p, from_input)
        again = lambda i: (x if i + 1 < reread else
                           residual(p + zero_s[i], from_input))
        return _layernorm(x, acc, again if reread else None)

    def ffn_up(slot, c):
        xn = _unpack(xn2[slot])
        g = jnp.dot(xn, wg[c], preferred_element_type=F32)
        u = jnp.dot(xn, wu[c], preferred_element_type=F32)
        return (g * u).astype(BF16)

    def ffn_down(h, t, c):
        res = jax.lax.dot_general(wd[c], h, NT_DIMS,
                                  preferred_element_type=F32)
        for i in range(NCH):
            x = xres[t * NCH + i] + res[:, i * SUB:(i + 1) * SUB]
            xres[t * NCH + i] = x
            xio[t * NCH + i] = x.astype(BF16)

    def ln1_pro(p):
        y = ln1(p, True, ACCP if p >= NCH else ACC0, RL0 if p >= NCH else 0)
        xn1[:, p * SUB:(p + 1) * SUB] = _pack(y)
        return y

    def project_pro(p0, p1, lo, hi, mc=3 * D):
        for m0 in range(lo, hi, mc):
            m1 = min(m0 + mc, hi)
            res = jnp.dot(_unpack(wqT[m0 // 2:m1 // 2, :]),
                          _unpack(xn1[:, p0 * SUB:p1 * SUB]),
                          preferred_element_type=F32)
            for p in range(p0, p1):
                part = res[:, (p - p0) * SUB:(p - p0 + 1) * SUB]
                if p < NCH:
                    first[p, m0:m1, :] = part
                if p >= NCH or (p == NCH - 1 and m1 > D):
                    ring[p, m0:m1, :] = part

    def out_proj0(lo, hi):
        o = jnp.concatenate(
            [first[i, 0:D, :].astype(BF16) for i in range(lo, hi)], axis=1)
        upd = jnp.dot(_unpack(woT[...]), o, preferred_element_type=F32)
        for i in range(lo, hi):
            x = residual(i, True) + upd[:, (i - lo) * SUB:(i - lo + 1) * SUB]
            xres[i] = x
            again = (lambda j, i=i: xres[i + zero_s[j]]) if RLO else None
            xn2[0, i * SUB // 2:(i + 1) * SUB // 2, :] = _pack(
                _layernorm(x, ACCO, again).T)

    n_pro = PT * NCH
    for p in range(NCH):
        x_copy(p).start()
    for j in range(NP):
        wqkv_copy(j).start()
    for p in range(NCH, NCH + XE):
        x_copy(p).start()
    wo_copy.start()
    for p in range(NCH + XE, n_pro):
        x_copy(p).start()
    for c in range(NCH):
        for which in range(3):
            f_copy(which, c).start()
        if c == 0:
            for p in range(n_pro, NS):
                x_copy(p).start()
    for g in range(H // HG):
        row_s[g] = g * HG * DH
    zero_s[0] = 0
    zero_s[1] = 0

    def unit0(u):
        i, g = divmod(u, H // HG)
        return first.at[i], first.at[i - 1 if i else NCH], i, row_s[g]

    with jax.named_scope("s_ln"):
        for p in range(NCH):
            x_copy(p).wait()
            ln1_pro(p)
    done = 0
    for j in range(NP):
        with jax.named_scope(f"s_w{j}"):
            wqkv_copy(j).wait()
            if j == NP - 1:
                for p in range(NCH, NCH + XE):
                    x_copy(p).wait()
        with jax.named_scope(f"s_b{j}"):
            project_pro(0, NCH, done, PIECES[j], MC)
            transpose_cols(wqkv_raw, wqT, PIECES[j], PIECES[j + 1])
            done = PIECES[j + 1] - (LAG if j < NP - 1 else 0)
            project_pro(0, NCH, PIECES[j], done, MC if j else LANES)
            if j == NP - 1:
                for p in range(NCH, NCH + XE):
                    ln1_pro(p)
    with jax.named_scope("s_wo"):
        wo_copy.wait()
        for p in range(NCH + XE, n_pro):
            x_copy(p).wait()
    with jax.named_scope("s_stage0"):
        fill_clamped(first, NCH, 0)
        n_units = NCH * H // HG
        sc = [attn_scores(*unit0(u)) for u in range(AHEAD)]
        for u in range(n_units + 1):
            for kind, arg in PLAN.get(u, ()):
                if kind == "P":
                    project_pro(*arg, MC2)
                elif kind == "O":
                    out_proj0(*arg)
                elif kind == "N":
                    ln1_pro(arg)
                elif kind == "T":
                    transpose_cols(wo_raw, woT, 0, D)
                else:
                    y = ln1_pro(arg)
                    first[NCH, 0:16, :] = y[D - 16:D, :].astype(F32)
            if u == n_units:
                break
            if u + AHEAD < n_units:
                sc.append(attn_scores(*unit0(u + AHEAD)))
            cur, prev, _, base = unit0(u)
            attn_values(cur, prev, base, sc[u], DH)
        for which in range(3):
            f_copy(which, 0).wait()
        for p in range(n_pro, NS):
            x_copy(p).wait()

    def body(k, do_proj):
        n = _div(k, NCH)
        c = _mod(k, NCH)
        if do_proj:
            xn1[:, 0:SUB] = _pack(
                ln1(_mod(k + n_pro, NS), k + n_pro < NS, ACC1, RL1))
        h = ffn_up(_mod(n, 2), c)
        p = _mod(k + NCH, NS)
        cur = ring.at[_mod(k + NCH, RING)]
        attention(cur, ring.at[_mod(k + NCH - 1, RING)], p if do_proj else 1)
        out_proj(cur, p, do_proj and k + NCH < NS, _mod(n + 1, 2),
                 pl.multiple_of(c * (SUB // 2), SUB // 2))
        if do_proj:
            ring[_mod(k + n_pro, RING)] = jnp.dot(
                _unpack(wqT[...]), _unpack(xn1[:, 0:SUB]),
                preferred_element_type=F32)
        ffn_down(h, _mod(n, NT), c)

    n_main = 2 * NS - n_pro
    assert n_main == NS + NCH

    def main_step(k, carry):
        body(k, True)
        return carry

    def segment(i, lo):
        hi = jnp.where(i < NCH - 1, i + 1,
                       jnp.where(i == NCH - 1, NS - NCH, n_main))
        jax.lax.fori_loop(lo, hi, main_step, 0)

        @pl.when(i < NCH - 1)
        def _():
            for which in range(3):
                f_copy(which, i + 1).wait()

        @pl.when(i == NCH - 1)
        def _():
            fill_clamped(ring, (NS - 1) % RING, NS % RING)

        return hi

    def mid_step(k, carry):
        out_copy(k - n_main).start()
        body(k, False)
        return carry

    with jax.named_scope("s_main"):
        jax.lax.fori_loop(0, NCH + 1, segment, 0)
    with jax.named_scope("s_mid"):
        jax.lax.fori_loop(n_main, 2 * NS - NCH, mid_step, 0)

    def last_step(m, carry):
        @pl.when(m == 0)
        def _():
            for p in range(NS - 2 * NCH, NS - NCH):
                out_copy(p).start()

        p0 = NS - NCH + m * LW

        @pl.when(m > 0)
        def _():
            for i in range(LW):
                out_copy(p0 - LW + i).start()

        half = LW * SUB // 2
        xn = _unpack(xn2[(2 * NT - 1) % 2,
                         pl.ds(pl.multiple_of(m * half, half), half), :])
        res = None
        for c in range(NCH):
            g = jnp.dot(xn, wg[c], preferred_element_type=F32)
            u = jnp.dot(xn, wu[c], preferred_element_type=F32)
            part = jax.lax.dot_general(wd[c], (g * u).astype(BF16), NT_DIMS,
                                       preferred_element_type=F32)
            res = part if res is None else res + part
        for i in range(LW):
            x = xres[p0 + i] + res[:, i * SUB:(i + 1) * SUB]
            xio[p0 + i] = x.astype(BF16)
        return carry

    with jax.named_scope("s_last"):
        jax.lax.fori_loop(0, NCH // LW, last_step, 0)
    with jax.named_scope("s_tail"):
        for p in range(NS - LW, NS):
            out_copy(p).start()
        for p in range(NS):
            out_copy(p).wait()


@jax.jit
def pallas_interleave_layers__sliding_local_dilated__glu_gated_bilinear__prompt_kernel(
    A_x: jax.Array,
    A_wqkv: jax.Array,
    A_wo: jax.Array,
    B_x: jax.Array,
    B_w_gate: jax.Array,
    B_w_up: jax.Array,
    B_w_down: jax.Array,
):
    del B_x
    xT = A_x.reshape(S, D).T
    wdT = B_w_down.T
    any_spec = pl.BlockSpec(memory_space=pl.ANY)
    outT = pl.pallas_call(
        _kernel,
        in_specs=[any_spec] * 6,
        out_specs=any_spec,
        out_shape=jax.ShapeDtypeStruct((D, S), BF16),
        scratch_shapes=[
            pltpu.VMEM((NS, D, SUB), F32),
            pltpu.VMEM((NS, D, SUB), BF16),
            pltpu.VMEM((D, 3 * D), BF16),
            pltpu.VMEM((D, D), BF16),
            pltpu.VMEM((NCH, D, FC), BF16),
            pltpu.VMEM((NCH, D, FC), BF16),
            pltpu.VMEM((NCH, D, FC), BF16),
            pltpu.VMEM((3 * D // 2, D), U32),
            pltpu.VMEM((D // 2, D), U32),
            pltpu.VMEM((NCH + 1, 3 * D, LANES), F32),
            pltpu.VMEM((RING, 3 * D, LANES), F32),
            pltpu.VMEM((D // 2, PT * TM), U32),
            pltpu.VMEM((2, TM // 2, D), U32),
            pltpu.SMEM((H // HG,), jnp.int32),
            pltpu.SMEM((2,), jnp.int32),
            pltpu.SemaphoreType.DMA((NS + NP + 1 + 3 * NCH,)),
            pltpu.SemaphoreType.DMA((NS,)),
        ],
        compiler_params=pltpu.CompilerParams(
            vmem_limit_bytes=100 * 1024 * 1024,
            disable_semaphore_checks=NOSEM,
            disable_bounds_checks=NOBND),
    )(xT, A_wqkv, A_wo, B_w_gate, B_w_up, wdT)
    return outT.T.reshape(1, S, D)
```

```python
import jax
import jax.numpy as jnp
import jax.experimental.pallas as pl
import jax.experimental.pallas.tpu as pltpu

S = 2048
D = 576
F = 4608
H = 32
DH = 18
W = 8
DIL = 2
EPS = 1e-5
LANES = 128

TM = 512
NT = S // TM
FC = 1152
NCH = F // FC
SUB = TM // NCH
NS = S // SUB
HG = 8
NG = H // HG
SB = 5
RING = 16
PIECES = (0, 256, 640, 1152, 1728)
NP = len(PIECES) - 1
LAG = 128
MC = 256
MC2 = 288
NPRO = 12
XE = 2
LW = 2

PLAN = {
    0: [("N", 10), ("N", 11), ("P", (4, 6, 0, 1728))],
    1: [("L", 6)],
    2: [("L", 7)],
    3: [("L", 8)],
    4: [("L", 9), ("P", (6, 10, 0, 1728))],
    16: [("T", 0), ("O", 0), ("O", 1), ("P", (10, 12, 0, 576)),
         ("O", 2), ("P", (10, 12, 576, 1152)),
         ("O", 3), ("P", (10, 12, 1152, 1728))],
}

SCALE = DH ** -0.5
EXP2_SCALE = SCALE * 1.4426950408889634
MASKED_LOGIT = -1e9 / SCALE

NT_DIMS = (((1,), (1,)), ((), ()))
F32 = jnp.float32
BF16 = jnp.bfloat16
U32 = jnp.uint32


def _mod(a, n):
    assert n & (n - 1) == 0
    return jax.lax.bitwise_and(a, n - 1)


def _div(a, n):
    assert n & (n - 1) == 0
    return jax.lax.shift_right_logical(a, n.bit_length() - 1)


def _pack(x):
    return pltpu.bitcast(x, U32)


def _unpack(x):
    return pltpu.bitcast(x, BF16)


def _mean_rows(x, chains):
    part = jnp.sum(x.reshape(D // (8 * chains), 8 * chains, x.shape[1]), axis=0)
    return jnp.sum(part, axis=0, keepdims=True) * (1.0 / D)


def _layernorm(x, chains=1, reread=None):
    m = _mean_rows(x, chains)
    c = (x if reread is None else reread(0)) - m
    v = _mean_rows(c * c, chains)
    if reread is not None:
        c = reread(1) - m
    y = c * jax.lax.rsqrt(v + EPS)
    return y.astype(BF16)


def _kernel(xT_hbm, wqkv_hbm, wo_hbm, wg_hbm, wu_hbm, wdT_hbm, out_hbm,
            xres, xio, wqkv_raw, wo_raw, wg, wu, wd,
            wqT, woT, first, ring, xn1, xn2, row_s, zero_s, sem_in, sem_o):

    def x_copy(p):
        return pltpu.make_async_copy(
            xT_hbm.at[:, pl.ds(p * SUB, SUB)], xio.at[p], sem_in.at[p])

    def f_copy(which, c):
        src = (wg_hbm, wu_hbm, wdT_hbm)[which]
        dst = (wg, wu, wd)[which]
        start = c * FC
        if not isinstance(c, int):
            start = pl.multiple_of(start, LANES)
        return pltpu.make_async_copy(
            src.at[:, pl.ds(start, FC)], dst.at[c],
            sem_in.at[NS + NP + 1 + which * NCH + c])

    def out_copy(p):
        start = p * SUB
        if not isinstance(p, int):
            start = pl.multiple_of(start, LANES)
        return pltpu.make_async_copy(
            xio.at[p], out_hbm.at[:, pl.ds(start, SUB)], sem_o.at[p])

    def wqkv_copy(j):
        cols = pl.ds(PIECES[j], PIECES[j + 1] - PIECES[j])
        return pltpu.make_async_copy(
            wqkv_hbm.at[:, cols], wqkv_raw.at[:, cols], sem_in.at[NS + j])

    wo_copy = pltpu.make_async_copy(wo_hbm, wo_raw, sem_in.at[NS + NP])

    def transpose_cols(src, dst, lo, hi):
        for c0 in range(lo, hi, LANES):
            c1 = min(c0 + LANES, hi)
            dst[c0 // 2:c1 // 2, :] = _pack(src[:, c0:c1].T)

    lane = jax.lax.broadcasted_iota(jnp.int32, (HG, LANES), 1)

    def shifted(cur, prev, w):
        if w == 0:
            return cur
        both = jnp.where(lane < LANES - DIL * w, cur, prev)
        return pltpu.roll(both, DIL * w, 1)

    def rows(base, part, d):
        return pl.ds(base + part * D + d, HG, stride=DH)

    def attn_scores(cur, prev, p, base):
        at_start = isinstance(p, int) and p == 0
        logits = [None] * W
        for d in range(DH):
            q = cur[rows(base, 0, d), :]
            kc = cur[rows(base, 1, d), :]
            kp = kc if at_start else prev[rows(base, 1, d), :]
            for w in range(W):
                t = q * shifted(kc, kp, w)
                logits[w] = t if d == 0 else logits[w] + t
        if p is not None:
            pos = p * SUB + lane
            for w in range(1, W):
                logits[w] = jnp.where(pos >= DIL * w, logits[w], MASKED_LOGIT)
        m = logits[0]
        for w in range(1, W):
            m = jnp.maximum(m, logits[w])
        es = [jnp.exp2((lg - m) * EXP2_SCALE) for lg in logits]
        s = es[0]
        for w in range(1, W):
            s = s + es[w]
        r = 1.0 / s
        return [e * r for e in es]

    def attn_values(cur, prev, base, a, sb):
        done = []
        for d in range(DH):
            vc = cur[rows(base, 2, d), :]
            vp = prev[rows(base, 2, d), :]
            o = a[0] * vc
            for w in range(1, W):
                o = o + a[w] * shifted(vc, vp, w)
            done.append((d, o))
            if len(done) == sb or d == DH - 1:
                for dd, oo in done:
                    cur[rows(base, 0, dd), :] = oo
                done = []

    def fill_clamped(buf, dst, src):
        buf[dst, 2 * D:3 * D, :] = jnp.broadcast_to(
            buf[src, 2 * D:3 * D, 0:1], (D, LANES))

    def residual(p, from_input):
        if from_input is True:
            return xio[p].astype(F32)
        if from_input is False:
            return xres[p]
        return jnp.where(from_input, xio[p].astype(F32), xres[p])

    def out_proj(qkv, p, from_input, slot, row0, reread):
        upd = jnp.dot(_unpack(woT[...]), qkv[0:D, :].astype(BF16),
                      preferred_element_type=F32)
        x = residual(p, from_input) + upd
        xres[p] = x
        again = (lambda i: xres[p + zero_s[i]]) if reread else None
        xn2[slot, pl.ds(row0, SUB // 2), :] = _pack(
            _layernorm(x, reread=again).T)

    def ffn_up(xn, c):
        g = jnp.dot(xn, wg[c], preferred_element_type=F32)
        u = jnp.dot(xn, wu[c], preferred_element_type=F32)
        return (g * u).astype(BF16)

    def ffn_down(h, c):
        return jax.lax.dot_general(wd[c], h, NT_DIMS,
                                   preferred_element_type=F32)

    def ln1_pro(p):
        y = _layernorm(residual(p, True), chains=4 if p < NCH else 1)
        xn1[:, p * SUB:(p + 1) * SUB] = _pack(y)
        return y

    def project_pro(p0, p1, lo, hi, mc):
        for m0 in range(lo, hi, mc):
            m1 = min(m0 + mc, hi)
            res = jnp.dot(_unpack(wqT[m0 // 2:m1 // 2, :]),
                          _unpack(xn1[:, p0 * SUB:p1 * SUB]),
                          preferred_element_type=F32)
            for p in range(p0, p1):
                part = res[:, (p - p0) * SUB:(p - p0 + 1) * SUB]
                if p < NCH:
                    first[p, m0:m1, :] = part
                if p >= NCH or (p == NCH - 1 and m1 > D):
                    ring[p, m0:m1, :] = part

    for p in range(NCH):
        x_copy(p).start()
    for j in range(NP):
        wqkv_copy(j).start()
    for p in range(NCH, NCH + XE):
        x_copy(p).start()
    wo_copy.start()
    for p in range(NCH + XE, NPRO):
        x_copy(p).start()
    for c in range(NCH):
        for which in range(3):
            f_copy(which, c).start()
        if c == 0:
            for p in range(NPRO, NS):
                x_copy(p).start()
    for g in range(NG):
        row_s[g] = g * HG * DH
    zero_s[0] = 0
    zero_s[1] = 0

    for p in range(NCH):
        x_copy(p).wait()
        ln1_pro(p)
    done = 0
    for j in range(NP):
        last = j == NP - 1
        wqkv_copy(j).wait()
        if last:
            for p in range(NCH, NCH + XE):
                x_copy(p).wait()
        project_pro(0, NCH, done, PIECES[j], MC)
        transpose_cols(wqkv_raw, wqT, PIECES[j], PIECES[j + 1])
        done = PIECES[j + 1] - (0 if last else LAG)
        project_pro(0, NCH, PIECES[j], done, MC)
        if last:
            for p in range(NCH, NCH + XE):
                ln1_pro(p)
    wo_copy.wait()
    for p in range(NCH + XE, NPRO):
        x_copy(p).wait()

    def unit(u):
        i, g = divmod(u, NG)
        return first.at[i], first.at[i - 1 if i else NCH], row_s[g]

    def unit_scores(u):
        cur, prev, base = unit(u)
        return attn_scores(cur, prev, 0 if u < NG else None, base)

    fill_clamped(first, NCH, 0)
    n_units = NCH * NG
    scores = [unit_scores(0)]
    for u in range(n_units + 1):
        for kind, arg in PLAN.get(u, ()):
            if kind == "P":
                project_pro(*arg, MC2)
            elif kind == "O":
                out_proj(first.at[arg], arg, True, 0, arg * SUB // 2, False)
            elif kind == "T":
                transpose_cols(wo_raw, woT, 0, D)
            else:
                y = ln1_pro(arg)
                if kind == "L":
                    first[NCH, 0:16, :] = y[D - 16:D, :].astype(F32)
        if u + 1 < n_units:
            scores.append(unit_scores(u + 1))
        if u < n_units:
            attn_values(*unit(u), scores[u], DH)
    for which in range(3):
        f_copy(which, 0).wait()
    for p in range(NPRO, NS):
        x_copy(p).wait()

    def body(k, do_proj):
        n = _div(k, NCH)
        c = _mod(k, NCH)
        if do_proj:
            xn1[:, 0:SUB] = _pack(_layernorm(
                residual(_mod(k + NPRO, NS), k + NPRO < NS)))
        h = ffn_up(_unpack(xn2[_mod(n, 2)]), c)
        p = _mod(k + NCH, NS)
        cur = ring.at[_mod(k + NCH, RING)]
        prev = ring.at[_mod(k + NCH - 1, RING)]
        for g in range(NG):
            a = attn_scores(cur, prev, p if do_proj else None, row_s[g])
            attn_values(cur, prev, row_s[g], a, SB)
        out_proj(cur, p, do_proj and k + NCH < NS, _mod(n + 1, 2),
                 pl.multiple_of(c * (SUB // 2), SUB // 2), True)
        if do_proj:
            ring[_mod(k + NPRO, RING)] = jnp.dot(
                _unpack(wqT[...]), _unpack(xn1[:, 0:SUB]),
                preferred_element_type=F32)
        res = ffn_down(h, c)
        p0 = _mod(n, NT) * NCH
        for i in range(NCH):
            x = xres[p0 + i] + res[:, i * SUB:(i + 1) * SUB]
            xres[p0 + i] = x
            xio[p0 + i] = x.astype(BF16)

    n_main = 2 * NS - NPRO
    n_mid = 2 * NS - NCH
    assert n_main >= NS + NCH

    def main_step(k, carry):
        body(k, True)
        return carry

    def segment(i, lo):
        hi = jnp.where(i < NCH - 1, i + 1,
                       jnp.where(i == NCH - 1, NS - NCH, n_main))
        jax.lax.fori_loop(lo, hi, main_step, 0)

        @pl.when(i < NCH - 1)
        def _():
            for which in range(3):
                f_copy(which, i + 1).wait()

        @pl.when(i == NCH - 1)
        def _():
            fill_clamped(ring, (NS - 1) % RING, NS % RING)

        return hi

    def mid_step(k, carry):
        out_copy(k - n_main).start()
        body(k, False)
        return carry

    def last_step(m, carry):
        @pl.when(m == 0)
        def _():
            for p in range(n_mid - n_main, NS - NCH):
                out_copy(p).start()

        p0 = NS - NCH + m * LW

        @pl.when(m > 0)
        def _():
            for i in range(LW):
                out_copy(p0 - LW + i).start()

        half = LW * SUB // 2
        xn = _unpack(xn2[(2 * NT - 1) % 2,
                         pl.ds(pl.multiple_of(m * half, half), half), :])
        res = None
        for c in range(NCH):
            part = ffn_down(ffn_up(xn, c), c)
            res = part if res is None else res + part
        for i in range(LW):
            x = xres[p0 + i] + res[:, i * SUB:(i + 1) * SUB]
            xio[p0 + i] = x.astype(BF16)
        return carry

    jax.lax.fori_loop(0, NCH + 1, segment, 0)
    jax.lax.fori_loop(n_main, n_mid, mid_step, 0)
    jax.lax.fori_loop(0, NCH // LW, last_step, 0)
    for p in range(NS - LW, NS):
        out_copy(p).start()
    for p in range(NS):
        out_copy(p).wait()


@jax.jit
def pallas_interleave_layers__sliding_local_dilated__glu_gated_bilinear__prompt_kernel(
    A_x: jax.Array,
    A_wqkv: jax.Array,
    A_wo: jax.Array,
    B_x: jax.Array,
    B_w_gate: jax.Array,
    B_w_up: jax.Array,
    B_w_down: jax.Array,
):
    del B_x
    xT = A_x.reshape(S, D).T
    wdT = B_w_down.T
    any_spec = pl.BlockSpec(memory_space=pl.ANY)
    outT = pl.pallas_call(
        _kernel,
        in_specs=[any_spec] * 6,
        out_specs=any_spec,
        out_shape=jax.ShapeDtypeStruct((D, S), BF16),
        scratch_shapes=[
            pltpu.VMEM((NS, D, SUB), F32),
            pltpu.VMEM((NS, D, SUB), BF16),
            pltpu.VMEM((D, 3 * D), BF16),
            pltpu.VMEM((D, D), BF16),
            pltpu.VMEM((NCH, D, FC), BF16),
            pltpu.VMEM((NCH, D, FC), BF16),
            pltpu.VMEM((NCH, D, FC), BF16),
            pltpu.VMEM((3 * D // 2, D), U32),
            pltpu.VMEM((D // 2, D), U32),
            pltpu.VMEM((NCH + 1, 3 * D, LANES), F32),
            pltpu.VMEM((RING, 3 * D, LANES), F32),
            pltpu.VMEM((D // 2, NPRO * SUB), U32),
            pltpu.VMEM((2, TM // 2, D), U32),
            pltpu.SMEM((NG,), jnp.int32),
            pltpu.SMEM((2,), jnp.int32),
            pltpu.SemaphoreType.DMA((NS + NP + 1 + 3 * NCH,)),
            pltpu.SemaphoreType.DMA((NS,)),
        ],
        compiler_params=pltpu.CompilerParams(
            vmem_limit_bytes=100 * 1024 * 1024,
            disable_semaphore_checks=True),
    )(xT, A_wqkv, A_wo, B_w_gate, B_w_up, wdT)
    return outT.T.reshape(1, S, D)
```

```python
import jax
import jax.numpy as jnp
import jax.experimental.pallas as pl
import jax.experimental.pallas.tpu as pltpu

S = 2048
D = 576
F = 4608
H = 32
DH = 18
W = 8
DIL = 2
EPS = 1e-5
LANES = 128

TM = 512
NT = S // TM
FC = 1152
NCH = F // FC
SUB = TM // NCH
NS = S // SUB
HG = 8
NG = H // HG
SB = 5
RING = 16
PIECES = (0, 256, 640, 1152, 1728)
NP = len(PIECES) - 1
LAG = 128
MC = 256
MC2 = 288
NPRO = 12
XE = 2
CUTS = (0, 448, 576)
NOBND = False
LW = 2

PLAN = {
    0: [("N", 10), ("N", 11), ("P", (4, 6, 0, 1728))],
    1: [("L", 6)],
    2: [("L", 7)],
    3: [("L", 8)],
    4: [("L", 9), ("P", (6, 10, 0, 1728))],
    16: [("T", 0), ("O", 0), ("O", 1), ("P", (10, 12, 0, 576)),
         ("O", 2), ("P", (10, 12, 576, 1152)),
         ("O", 3), ("P", (10, 12, 1152, 1728))],
}

SCALE = DH ** -0.5
EXP2_SCALE = SCALE * 1.4426950408889634
MASKED_LOGIT = -1e9 / SCALE

NT_DIMS = (((1,), (1,)), ((), ()))
F32 = jnp.float32
BF16 = jnp.bfloat16
U32 = jnp.uint32


def _mod(a, n):
    assert n & (n - 1) == 0
    return jax.lax.bitwise_and(a, n - 1)


def _div(a, n):
    assert n & (n - 1) == 0
    return jax.lax.shift_right_logical(a, n.bit_length() - 1)


def _pack(x):
    return pltpu.bitcast(x, U32)


def _unpack(x):
    return pltpu.bitcast(x, BF16)


def _mean_rows(x, chains):
    part = jnp.sum(x.reshape(D // (8 * chains), 8 * chains, x.shape[1]), axis=0)
    return jnp.sum(part, axis=0, keepdims=True) * (1.0 / D)


def _layernorm(x, chains=1, reread=None):
    m = _mean_rows(x, chains)
    c = (x if reread is None else reread(0)) - m
    v = _mean_rows(c * c, chains)
    if reread is not None:
        c = reread(1) - m
    y = c * jax.lax.rsqrt(v + EPS)
    return y.astype(BF16)


def _kernel(xT_hbm, wqkv_hbm, wo_hbm, wg_hbm, wu_hbm, wdT_hbm, out_hbm,
            xres, xio, wqkv_raw, wo_raw, wg, wu, wd,
            wqT, woT, first, ring, xn1, xn2, row_s, zero_s, sem_in, sem_o):

    def x_copy(p):
        return pltpu.make_async_copy(
            xT_hbm.at[:, pl.ds(p * SUB, SUB)], xio.at[p], sem_in.at[p])

    def f_copy(which, c):
        src = (wg_hbm, wu_hbm, wdT_hbm)[which]
        dst = (wg, wu, wd)[which]
        start = c * FC
        if not isinstance(c, int):
            start = pl.multiple_of(start, LANES)
        return pltpu.make_async_copy(
            src.at[:, pl.ds(start, FC)], dst.at[c],
            sem_in.at[NS + NP + 1 + which * NCH + c])

    def out_copy(p):
        start = p * SUB
        if not isinstance(p, int):
            start = pl.multiple_of(start, LANES)
        return pltpu.make_async_copy(
            xio.at[p], out_hbm.at[:, pl.ds(start, SUB)], sem_o.at[p])

    def out_part_copy(p, j):
        start = p * SUB
        if not isinstance(p, int):
            start = pl.multiple_of(start, LANES)
        r = pl.ds(CUTS[j], CUTS[j + 1] - CUTS[j])
        return pltpu.make_async_copy(
            xio.at[p, r], out_hbm.at[r, pl.ds(start, SUB)],
            sem_o.at[p + j * NCH])

    def wqkv_copy(j):
        cols = pl.ds(PIECES[j], PIECES[j + 1] - PIECES[j])
        return pltpu.make_async_copy(
            wqkv_hbm.at[:, cols], wqkv_raw.at[:, cols], sem_in.at[NS + j])

    wo_copy = pltpu.make_async_copy(wo_hbm, wo_raw, sem_in.at[NS + NP])

    def transpose_cols(src, dst, lo, hi):
        for c0 in range(lo, hi, LANES):
            c1 = min(c0 + LANES, hi)
            dst[c0 // 2:c1 // 2, :] = _pack(src[:, c0:c1].T)

    lane = jax.lax.broadcasted_iota(jnp.int32, (HG, LANES), 1)

    def shifted(cur, prev, w):
        if w == 0:
            return cur
        both = jnp.where(lane < LANES - DIL * w, cur, prev)
        return pltpu.roll(both, DIL * w, 1)

    def rows(base, part, d):
        return pl.ds(base + part * D + d, HG, stride=DH)

    def attn_scores(cur, prev, p, base):
        at_start = isinstance(p, int) and p == 0
        logits = [None] * W
        for d in range(DH):
            q = cur[rows(base, 0, d), :]
            kc = cur[rows(base, 1, d), :]
            kp = kc if at_start else prev[rows(base, 1, d), :]
            for w in range(W):
                t = q * shifted(kc, kp, w)
                logits[w] = t if d == 0 else logits[w] + t
        if p is not None:
            pos = p * SUB + lane
            for w in range(1, W):
                logits[w] = jnp.where(pos >= DIL * w, logits[w], MASKED_LOGIT)
        m = logits[0]
        for w in range(1, W):
            m = jnp.maximum(m, logits[w])
        es = [jnp.exp2((lg - m) * EXP2_SCALE) for lg in logits]
        s = es[0]
        for w in range(1, W):
            s = s + es[w]
        r = 1.0 / s
        return [e * r for e in es]

    def attn_values(cur, prev, base, a, sb):
        done = []
        for d in range(DH):
            vc = cur[rows(base, 2, d), :]
            vp = prev[rows(base, 2, d), :]
            o = a[0] * vc
            for w in range(1, W):
                o = o + a[w] * shifted(vc, vp, w)
            done.append((d, o))
            if len(done) == sb or d == DH - 1:
                for dd, oo in done:
                    cur[rows(base, 0, dd), :] = oo
                done = []

    def fill_clamped(buf, dst, src):
        buf[dst, 2 * D:3 * D, :] = jnp.broadcast_to(
            buf[src, 2 * D:3 * D, 0:1], (D, LANES))

    def residual(p, from_input):
        if from_input is True:
            return xio[p].astype(F32)
        if from_input is False:
            return xres[p]
        return jnp.where(from_input, xio[p].astype(F32), xres[p])

    def out_proj(qkv, p, from_input, slot, row0, reread):
        upd = jnp.dot(_unpack(woT[...]), qkv[0:D, :].astype(BF16),
                      preferred_element_type=F32)
        x = residual(p, from_input) + upd
        xres[p] = x
        again = (lambda i: xres[p + zero_s[i]]) if reread else None
        xn2[slot, pl.ds(row0, SUB // 2), :] = _pack(
            _layernorm(x, reread=again).T)

    def ffn_up(xn, c):
        g = jnp.dot(xn, wg[c], preferred_element_type=F32)
        u = jnp.dot(xn, wu[c], preferred_element_type=F32)
        return (g * u).astype(BF16)

    def ffn_down(h, c):
        return jax.lax.dot_general(wd[c], h, NT_DIMS,
                                   preferred_element_type=F32)

    def ln1_pro(p):
        y = _layernorm(residual(p, True), chains=4 if p < NCH else 1)
        xn1[:, p * SUB:(p + 1) * SUB] = _pack(y)
        return y

    def project_pro(p0, p1, lo, hi, mc):
        for m0 in range(lo, hi, mc):
            m1 = min(m0 + mc, hi)
            res = jnp.dot(_unpack(wqT[m0 // 2:m1 // 2, :]),
                          _unpack(xn1[:, p0 * SUB:p1 * SUB]),
                          preferred_element_type=F32)
            for p in range(p0, p1):
                part = res[:, (p - p0) * SUB:(p - p0 + 1) * SUB]
                if p < NCH:
                    first[p, m0:m1, :] = part
                if p >= NCH or (p == NCH - 1 and m1 > D):
                    ring[p, m0:m1, :] = part

    for p in range(NCH):
        x_copy(p).start()
    for j in range(NP):
        wqkv_copy(j).start()
    for p in range(NCH, NCH + XE):
        x_copy(p).start()
    wo_copy.start()
    for p in range(NCH + XE, NPRO):
        x_copy(p).start()
    for c in range(NCH):
        for which in range(3):
            f_copy(which, c).start()
        if c == 0:
            for p in range(NPRO, NS):
                x_copy(p).start()
    for g in range(NG):
        row_s[g] = g * HG * DH
    zero_s[0] = 0
    zero_s[1] = 0

    for p in range(NCH):
        x_copy(p).wait()
        ln1_pro(p)
    done = 0
    for j in range(NP):
        last = j == NP - 1
        wqkv_copy(j).wait()
        if last:
            for p in range(NCH, NCH + XE):
                x_copy(p).wait()
        project_pro(0, NCH, done, PIECES[j], MC)
        transpose_cols(wqkv_raw, wqT, PIECES[j], PIECES[j + 1])
        done = PIECES[j + 1] - (0 if last else LAG)
        project_pro(0, NCH, PIECES[j], done, MC)
        if last:
            for p in range(NCH, NCH + XE):
                ln1_pro(p)
    wo_copy.wait()
    for p in range(NCH + XE, NPRO):
        x_copy(p).wait()

    def unit(u):
        i, g = divmod(u, NG)
        return first.at[i], first.at[i - 1 if i else NCH], row_s[g]

    def unit_scores(u):
        cur, prev, base = unit(u)
        return attn_scores(cur, prev, 0 if u < NG else None, base)

    fill_clamped(first, NCH, 0)
    n_units = NCH * NG
    scores = [unit_scores(0)]
    for u in range(n_units + 1):
        for kind, arg in PLAN.get(u, ()):
            if kind == "P":
                project_pro(*arg, MC2)
            elif kind == "O":
                out_proj(first.at[arg], arg, True, 0, arg * SUB // 2, False)
            elif kind == "T":
                transpose_cols(wo_raw, woT, 0, D)
            else:
                y = ln1_pro(arg)
                if kind == "L":
                    first[NCH, 0:16, :] = y[D - 16:D, :].astype(F32)
        if u + 1 < n_units:
            scores.append(unit_scores(u + 1))
        if u < n_units:
            attn_values(*unit(u), scores[u], DH)
    for which in range(3):
        f_copy(which, 0).wait()
    for p in range(NPRO, NS):
        x_copy(p).wait()

    def body(k, do_proj):
        n = _div(k, NCH)
        c = _mod(k, NCH)
        if do_proj:
            xn1[:, 0:SUB] = _pack(_layernorm(
                residual(_mod(k + NPRO, NS), k + NPRO < NS)))
        h = ffn_up(_unpack(xn2[_mod(n, 2)]), c)
        p = _mod(k + NCH, NS)
        cur = ring.at[_mod(k + NCH, RING)]
        prev = ring.at[_mod(k + NCH - 1, RING)]
        for g in range(NG):
            a = attn_scores(cur, prev, p if do_proj else None, row_s[g])
            attn_values(cur, prev, row_s[g], a, SB)
        out_proj(cur, p, do_proj and k + NCH < NS, _mod(n + 1, 2),
                 pl.multiple_of(c * (SUB // 2), SUB // 2), True)
        if do_proj:
            ring[_mod(k + NPRO, RING)] = jnp.dot(
                _unpack(wqT[...]), _unpack(xn1[:, 0:SUB]),
                preferred_element_type=F32)
        res = ffn_down(h, c)
        p0 = _mod(n, NT) * NCH
        for i in range(NCH):
            x = xres[p0 + i] + res[:, i * SUB:(i + 1) * SUB]
            xres[p0 + i] = x
            xio[p0 + i] = x.astype(BF16)

    n_main = 2 * NS - NPRO
    n_mid = 2 * NS - NCH
    assert n_main >= NS + NCH

    def main_step(k, carry):
        body(k, True)
        return carry

    def segment(i, lo):
        hi = jnp.where(i < NCH - 1, i + 1,
                       jnp.where(i == NCH - 1, NS - NCH, n_main))
        jax.lax.fori_loop(lo, hi, main_step, 0)

        @pl.when(i < NCH - 1)
        def _():
            for which in range(3):
                f_copy(which, i + 1).wait()

        @pl.when(i == NCH - 1)
        def _():
            fill_clamped(ring, (NS - 1) % RING, NS % RING)

        return hi

    def mid_step(k, carry):
        out_copy(k - n_main).start()
        body(k, False)
        return carry

    def last_step(m, carry):
        @pl.when(m == 0)
        def _():
            for p in range(n_mid - n_main, NS - NCH):
                out_copy(p).start()

        p0 = NS - NCH + m * LW
        half = LW * SUB // 2
        xn = _unpack(xn2[(2 * NT - 1) % 2,
                         pl.ds(pl.multiple_of(m * half, half), half), :])
        res = None
        for c in range(NCH - 1):
            part = ffn_down(ffn_up(xn, c), c)
            res = part if res is None else res + part
        h = ffn_up(xn, NCH - 1)
        for j in range(len(CUTS) - 1):
            r0, r1 = CUTS[j], CUTS[j + 1]
            part = res[r0:r1] + jax.lax.dot_general(
                wd[NCH - 1, r0:r1, :], h, NT_DIMS, preferred_element_type=F32)
            for i in range(LW):
                x = xres[p0 + i, r0:r1, :] + part[:, i * SUB:(i + 1) * SUB]
                xio[p0 + i, r0:r1, :] = x.astype(BF16)
            for i in range(LW):
                out_part_copy(p0 + i, j).start()
        return carry

    jax.lax.fori_loop(0, NCH + 1, segment, 0)
    jax.lax.fori_loop(n_main, n_mid, mid_step, 0)
    jax.lax.fori_loop(0, NCH // LW, last_step, 0)
    for p in range(NS - NCH):
        out_copy(p).wait()
    for j in range(len(CUTS) - 1):
        for p in range(NS - NCH, NS):
            out_part_copy(p, j).wait()


@jax.jit
def pallas_interleave_layers__sliding_local_dilated__glu_gated_bilinear__prompt_kernel(
    A_x: jax.Array,
    A_wqkv: jax.Array,
    A_wo: jax.Array,
    B_x: jax.Array,
    B_w_gate: jax.Array,
    B_w_up: jax.Array,
    B_w_down: jax.Array,
):
    del B_x
    xT = A_x.reshape(S, D).T
    wdT = B_w_down.T
    any_spec = pl.BlockSpec(memory_space=pl.ANY)
    outT = pl.pallas_call(
        _kernel,
        in_specs=[any_spec] * 6,
        out_specs=any_spec,
        out_shape=jax.ShapeDtypeStruct((D, S), BF16),
        scratch_shapes=[
            pltpu.VMEM((NS, D, SUB), F32),
            pltpu.VMEM((NS, D, SUB), BF16),
            pltpu.VMEM((D, 3 * D), BF16),
            pltpu.VMEM((D, D), BF16),
            pltpu.VMEM((NCH, D, FC), BF16),
            pltpu.VMEM((NCH, D, FC), BF16),
            pltpu.VMEM((NCH, D, FC), BF16),
            pltpu.VMEM((3 * D // 2, D), U32),
            pltpu.VMEM((D // 2, D), U32),
            pltpu.VMEM((NCH + 1, 3 * D, LANES), F32),
            pltpu.VMEM((RING, 3 * D, LANES), F32),
            pltpu.VMEM((D // 2, NPRO * SUB), U32),
            pltpu.VMEM((2, TM // 2, D), U32),
            pltpu.SMEM((NG,), jnp.int32),
            pltpu.SMEM((2,), jnp.int32),
            pltpu.SemaphoreType.DMA((NS + NP + 1 + 3 * NCH,)),
            pltpu.SemaphoreType.DMA((NS + (len(CUTS) - 2) * NCH,)),
        ],
        compiler_params=pltpu.CompilerParams(
            vmem_limit_bytes=100 * 1024 * 1024,
            disable_semaphore_checks=True,
            disable_bounds_checks=NOBND),
    )(xT, A_wqkv, A_wo, B_w_gate, B_w_up, wdT)
    return outT.T.reshape(1, S, D)
```

```python
import jax
import jax.numpy as jnp
import jax.experimental.pallas as pl
import jax.experimental.pallas.tpu as pltpu

S = 2048
D = 576
F = 4608
H = 32
DH = 18
W = 8
DIL = 2
EPS = 1e-5
LANES = 128

TM = 256
NT = S // TM
FC = 2304
NCH = F // FC
SUB = TM // NCH
NS = S // SUB
HG = 8
NG = H // HG
SB = 4
RING = 16
PIECES = (0, 256, 640, 1152, 1728)
NP = len(PIECES) - 1
LAG = 128
MC = 256
MC2 = 288
NPRO = 12
XE = 2
CUTS = (0, 448, 576)
NOBND = False
N0 = 4
SB0 = 5
SBM = 4
OS = 1
RLA = 0
RLB = 1
AHEAD = 0
LW = 2

PLAN = {
    0: [("P", (4, 6, 0, 1728))],
    1: [("L", 6), ("L", 7), ("P", (6, 8, 0, 1728))],
    3: [("L", 8), ("L", 9), ("P", (8, 10, 0, 1728))],
    5: [("L", 10), ("L", 11)],
    8: [("T", 0), ("P", (10, 12, 0, 576)), ("O", 0), ("P", (10, 12, 576, 1152)),
        ("O", 1), ("P", (10, 12, 1152, 1728))],
}

SCALE = DH ** -0.5
EXP2_SCALE = SCALE * 1.4426950408889634
MASKED_LOGIT = -1e9 / SCALE

NT_DIMS = (((1,), (1,)), ((), ()))
F32 = jnp.float32
BF16 = jnp.bfloat16
U32 = jnp.uint32


def _mod(a, n):
    assert n & (n - 1) == 0
    return jax.lax.bitwise_and(a, n - 1)


def _div(a, n):
    assert n & (n - 1) == 0
    return jax.lax.shift_right_logical(a, n.bit_length() - 1)


def _pack(x):
    return pltpu.bitcast(x, U32)


def _unpack(x):
    return pltpu.bitcast(x, BF16)


def _mean_rows(x, chains):
    part = jnp.sum(x.reshape(D // (8 * chains), 8 * chains, x.shape[1]), axis=0)
    return jnp.sum(part, axis=0, keepdims=True) * (1.0 / D)


def _layernorm(x, chains=1, reread=None):
    m = _mean_rows(x, chains)
    c = (x if reread is None else reread(0)) - m
    v = _mean_rows(c * c, chains)
    if reread is not None:
        c = reread(1) - m
    y = c * jax.lax.rsqrt(v + EPS)
    return y.astype(BF16)


def _kernel(xT_hbm, wqkv_hbm, wo_hbm, wg_hbm, wu_hbm, wdT_hbm, out_hbm,
            xres, xio, wqkv_raw, wo_raw, wg, wu, wd,
            wqT, woT, first, ring, xn1, xn2, row_s, zero_s, sem_in, sem_o):

    def x_copy(p):
        return pltpu.make_async_copy(
            xT_hbm.at[:, pl.ds(p * SUB, SUB)], xio.at[p], sem_in.at[p])

    def f_copy(which, c):
        src = (wg_hbm, wu_hbm, wdT_hbm)[which]
        dst = (wg, wu, wd)[which]
        start = c * FC
        if not isinstance(c, int):
            start = pl.multiple_of(start, LANES)
        return pltpu.make_async_copy(
            src.at[:, pl.ds(start, FC)], dst.at[c],
            sem_in.at[NS + NP + 1 + which * NCH + c])

    def out_copy(p):
        start = p * SUB
        if not isinstance(p, int):
            start = pl.multiple_of(start, LANES)
        return pltpu.make_async_copy(
            xio.at[p], out_hbm.at[:, pl.ds(start, SUB)], sem_o.at[p])

    def out_part_copy(p, j):
        start = p * SUB
        if not isinstance(p, int):
            start = pl.multiple_of(start, LANES)
        r = pl.ds(CUTS[j], CUTS[j + 1] - CUTS[j])
        return pltpu.make_async_copy(
            xio.at[p, r], out_hbm.at[r, pl.ds(start, SUB)],
            sem_o.at[p + j * NCH])

    def wqkv_copy(j):
        cols = pl.ds(PIECES[j], PIECES[j + 1] - PIECES[j])
        return pltpu.make_async_copy(
            wqkv_hbm.at[:, cols], wqkv_raw.at[:, cols], sem_in.at[NS + j])

    wo_copy = pltpu.make_async_copy(wo_hbm, wo_raw, sem_in.at[NS + NP])

    def transpose_cols(src, dst, lo, hi):
        for c0 in range(lo, hi, LANES):
            c1 = min(c0 + LANES, hi)
            dst[c0 // 2:c1 // 2, :] = _pack(src[:, c0:c1].T)

    lane = jax.lax.broadcasted_iota(jnp.int32, (HG, LANES), 1)

    def shifted(cur, prev, w):
        if w == 0:
            return cur
        both = jnp.where(lane < LANES - DIL * w, cur, prev)
        return pltpu.roll(both, DIL * w, 1)

    def rows(base, part, d):
        return pl.ds(base + part * D + d, HG, stride=DH)

    def attn_scores(cur, prev, p, base):
        at_start = isinstance(p, int) and p == 0
        logits = [None] * W
        for d in range(DH):
            q = cur[rows(base, 0, d), :]
            kc = cur[rows(base, 1, d), :]
            kp = kc if at_start else prev[rows(base, 1, d), :]
            for w in range(W):
                t = q * shifted(kc, kp, w)
                logits[w] = t if d == 0 else logits[w] + t
        if p is not None:
            pos = p * SUB + lane
            for w in range(1, W):
                logits[w] = jnp.where(pos >= DIL * w, logits[w], MASKED_LOGIT)
        m = logits[0]
        for w in range(1, W):
            m = jnp.maximum(m, logits[w])
        es = [jnp.exp2((lg - m) * EXP2_SCALE) for lg in logits]
        s = es[0]
        for w in range(1, W):
            s = s + es[w]
        r = 1.0 / s
        return [e * r for e in es]

    def attn_values(cur, prev, base, a, sb):
        done = []
        for d in range(DH):
            vc = cur[rows(base, 2, d), :]
            vp = prev[rows(base, 2, d), :]
            o = a[0] * vc
            for w in range(1, W):
                o = o + a[w] * shifted(vc, vp, w)
            done.append((d, o))
            if len(done) == sb or d == DH - 1:
                for dd, oo in done:
                    cur[rows(base, 0, dd), :] = oo
                done = []

    def fill_clamped(buf, dst, src):
        buf[dst, 2 * D:3 * D, :] = jnp.broadcast_to(
            buf[src, 2 * D:3 * D, 0:1], (D, LANES))

    def residual(p, from_input):
        if from_input is True:
            return xio[p].astype(F32)
        if from_input is False:
            return xres[p]
        return jnp.where(from_input, xio[p].astype(F32), xres[p])

    def out_proj(qkv, p, from_input, slot, row0, reread, split=1):
        o = qkv[0:D, :].astype(BF16)
        step = D // 2 // split
        upd = jnp.concatenate(
            [jnp.dot(_unpack(woT[i * step:(i + 1) * step, :]), o,
                     preferred_element_type=F32) for i in range(split)], axis=0)
        x = residual(p, from_input) + upd
        xres[p] = x
        again = (lambda i: xres[p + zero_s[i]]) if reread else None
        xn2[slot, pl.ds(row0, SUB // 2), :] = _pack(
            _layernorm(x, reread=again).T)

    def ffn_up(xn, c):
        g = jnp.dot(xn, wg[c], preferred_element_type=F32)
        u = jnp.dot(xn, wu[c], preferred_element_type=F32)
        return (g * u).astype(BF16)

    def ffn_down(h, c):
        return jax.lax.dot_general(wd[c], h, NT_DIMS,
                                   preferred_element_type=F32)

    def ln1_pro(p):
        y = _layernorm(residual(p, True), chains=4 if p < N0 else 1)
        xn1[:, p * SUB:(p + 1) * SUB] = _pack(y)
        return y

    def project_pro(p0, p1, lo, hi, mc):
        for m0 in range(lo, hi, mc):
            m1 = min(m0 + mc, hi)
            res = jnp.dot(_unpack(wqT[m0 // 2:m1 // 2, :]),
                          _unpack(xn1[:, p0 * SUB:p1 * SUB]),
                          preferred_element_type=F32)
            for p in range(p0, p1):
                part = res[:, (p - p0) * SUB:(p - p0 + 1) * SUB]
                if p < NCH:
                    first[p, m0:m1, :] = part
                if p >= NCH or (p == NCH - 1 and m1 > D):
                    ring[p, m0:m1, :] = part

    for p in range(N0):
        x_copy(p).start()
    for j in range(NP):
        wqkv_copy(j).start()
    for p in range(N0, N0 + XE):
        x_copy(p).start()
    wo_copy.start()
    for p in range(N0 + XE, NPRO):
        x_copy(p).start()
    for c in range(NCH):
        for which in range(3):
            f_copy(which, c).start()
        if c == 0:
            for p in range(NPRO, NS):
                x_copy(p).start()
    for g in range(NG):
        row_s[g] = g * HG * DH
    zero_s[0] = 0
    zero_s[1] = 0

    for p in range(N0):
        x_copy(p).wait()
        ln1_pro(p)
    done = 0
    for j in range(NP):
        last = j == NP - 1
        wqkv_copy(j).wait()
        if last:
            for p in range(N0, N0 + XE):
                x_copy(p).wait()
        project_pro(0, N0, done, PIECES[j], MC)
        transpose_cols(wqkv_raw, wqT, PIECES[j], PIECES[j + 1])
        done = PIECES[j + 1] - (0 if last else LAG)
        project_pro(0, N0, PIECES[j], done, MC)
        if last:
            for p in range(N0, N0 + XE):
                ln1_pro(p)
    wo_copy.wait()
    for p in range(N0 + XE, NPRO):
        x_copy(p).wait()

    def unit(u):
        i, g = divmod(u, NG)
        prev = (i - 1 if i else NCH) + zero_s[0]
        return first.at[i], first.at[prev], row_s[g]

    def unit_scores(u):
        cur, prev, base = unit(u)
        return attn_scores(cur, prev, 0 if u < NG else None, base)

    fill_clamped(first, NCH, 0)
    n_units = NCH * NG
    scores = [unit_scores(u) for u in range(AHEAD)]
    for u in range(n_units + 1):
        for kind, arg in PLAN.get(u, ()):
            if kind == "P":
                project_pro(*arg, MC2)
            elif kind == "O":
                out_proj(first.at[arg], arg, True, 0, arg * SUB // 2, False)
            elif kind == "T":
                transpose_cols(wo_raw, woT, 0, D)
            else:
                y = ln1_pro(arg)
                if kind == "L":
                    first[NCH, 0:16, :] = y[D - 16:D, :].astype(F32)
        if u + AHEAD < n_units:
            scores.append(unit_scores(u + AHEAD))
        if u < n_units:
            attn_values(*unit(u), scores[u], SB0)
    for which in range(3):
        f_copy(which, 0).wait()
    for p in range(NPRO, NS):
        x_copy(p).wait()

    def body(k, do_proj):
        n = _div(k, NCH)
        c = _mod(k, NCH)
        if do_proj:
            xn1[:, 0:SUB] = _pack(_layernorm(
                residual(_mod(k + NPRO, NS), k + NPRO < NS)))
        h = ffn_up(_unpack(xn2[_mod(n, 2)]), c)
        p = _mod(k + NCH, NS)
        cur = ring.at[_mod(k + NCH, RING)]
        prev = ring.at[_mod(k + NCH - 1, RING)]
        for g in range(NG):
            a = attn_scores(cur, prev, p if do_proj else None, row_s[g])
            attn_values(cur, prev, row_s[g], a, SB if do_proj else SBM)
        out_proj(cur, p, do_proj and k + NCH < NS, _mod(n + 1, 2),
                 pl.multiple_of(c * (SUB // 2), SUB // 2),
                 RLA if do_proj else RLB, 1 if do_proj else OS)
        if do_proj:
            ring[_mod(k + NPRO, RING)] = jnp.dot(
                _unpack(wqT[...]), _unpack(xn1[:, 0:SUB]),
                preferred_element_type=F32)
        res = ffn_down(h, c)
        p0 = _mod(n, NT) * NCH
        for i in range(NCH):
            x = xres[p0 + i] + res[:, i * SUB:(i + 1) * SUB]
            xres[p0 + i] = x
            xio[p0 + i] = x.astype(BF16)

    n_main = 2 * NS - NPRO
    n_mid = 2 * NS - NCH
    assert n_main >= NS + NCH

    def main_step(k, carry):
        body(k, True)
        return carry

    def segment(i, lo):
        hi = jnp.where(i < NCH - 1, i + 1,
                       jnp.where(i == NCH - 1, NS - NCH, n_main))
        jax.lax.fori_loop(lo, hi, main_step, 0)

        @pl.when(i < NCH - 1)
        def _():
            for which in range(3):
                f_copy(which, i + 1).wait()

        @pl.when(i == NCH - 1)
        def _():
            fill_clamped(ring, (NS - 1) % RING, NS % RING)

        return hi

    def mid_step(k, carry):
        out_copy(k - n_main).start()
        body(k, False)
        return carry

    def last_step(m, carry):
        @pl.when(m == 0)
        def _():
            for p in range(n_mid - n_main, NS - NCH):
                out_copy(p).start()

        p0 = NS - NCH + m * LW
        half = LW * SUB // 2
        xn = _unpack(xn2[(2 * NT - 1) % 2,
                         pl.ds(pl.multiple_of(m * half, half), half), :])
        res = None
        for c in range(NCH - 1):
            part = ffn_down(ffn_up(xn, c), c)
            res = part if res is None else res + part
        h = ffn_up(xn, NCH - 1)
        for j in range(len(CUTS) - 1):
            r0, r1 = CUTS[j], CUTS[j + 1]
            part = res[r0:r1] + jax.lax.dot_general(
                wd[NCH - 1, r0:r1, :], h, NT_DIMS, preferred_element_type=F32)
            for i in range(LW):
                x = xres[p0 + i, r0:r1, :] + part[:, i * SUB:(i + 1) * SUB]
                xio[p0 + i, r0:r1, :] = x.astype(BF16)
            for i in range(LW):
                out_part_copy(p0 + i, j).start()
        return carry

    jax.lax.fori_loop(0, NCH + 1, segment, 0)
    jax.lax.fori_loop(n_main, n_mid, mid_step, 0)
    jax.lax.fori_loop(0, NCH // LW, last_step, 0)
    for p in range(NS - NCH):
        out_copy(p).wait()
    for j in range(len(CUTS) - 1):
        for p in range(NS - NCH, NS):
            out_part_copy(p, j).wait()


@jax.jit
def pallas_interleave_layers__sliding_local_dilated__glu_gated_bilinear__prompt_kernel(
    A_x: jax.Array,
    A_wqkv: jax.Array,
    A_wo: jax.Array,
    B_x: jax.Array,
    B_w_gate: jax.Array,
    B_w_up: jax.Array,
    B_w_down: jax.Array,
):
    del B_x
    xT = A_x.reshape(S, D).T
    wdT = B_w_down.T
    any_spec = pl.BlockSpec(memory_space=pl.ANY)
    outT = pl.pallas_call(
        _kernel,
        in_specs=[any_spec] * 6,
        out_specs=any_spec,
        out_shape=jax.ShapeDtypeStruct((D, S), BF16),
        scratch_shapes=[
            pltpu.VMEM((NS, D, SUB), F32),
            pltpu.VMEM((NS, D, SUB), BF16),
            pltpu.VMEM((D, 3 * D), BF16),
            pltpu.VMEM((D, D), BF16),
            pltpu.VMEM((NCH, D, FC), BF16),
            pltpu.VMEM((NCH, D, FC), BF16),
            pltpu.VMEM((NCH, D, FC), BF16),
            pltpu.VMEM((3 * D // 2, D), U32),
            pltpu.VMEM((D // 2, D), U32),
            pltpu.VMEM((NCH + 1, 3 * D, LANES), F32),
            pltpu.VMEM((RING, 3 * D, LANES), F32),
            pltpu.VMEM((D // 2, NPRO * SUB), U32),
            pltpu.VMEM((2, TM // 2, D), U32),
            pltpu.SMEM((NG,), jnp.int32),
            pltpu.SMEM((2,), jnp.int32),
            pltpu.SemaphoreType.DMA((NS + NP + 1 + 3 * NCH,)),
            pltpu.SemaphoreType.DMA((NS + (len(CUTS) - 2) * NCH,)),
        ],
        compiler_params=pltpu.CompilerParams(
            vmem_limit_bytes=100 * 1024 * 1024,
            disable_semaphore_checks=True,
            disable_bounds_checks=NOBND),
    )(xT, A_wqkv, A_wo, B_w_gate, B_w_up, wdT)
    return outT.T.reshape(1, S, D)
```

```python
import jax
import jax.numpy as jnp
import jax.experimental.pallas as pl
import jax.experimental.pallas.tpu as pltpu

S = 2048
D = 576
F = 4608
H = 32
DH = 18
W = 8
DIL = 2
EPS = 1e-5
LANES = 128

TM = 256
NT = S // TM
FC = 2304
NCH = F // FC
SUB = TM // NCH
NS = S // SUB
HG = 8
NG = H // HG
SB = 4
RING = 16
PIECES = (0, 256, 640, 1152, 1728)
NP = len(PIECES) - 1
LAG = 128
MC = 256
MC2 = 288
NPRO = 12
XE = 2
CUTS = (0, 448, 576)
NOBND = False
N0 = 4
SB0 = 5
SBM = 4
OS = 1
RLA = 0
RLB = 1
AHEAD = 0
LW = 2

PLAN = {
    0: [("P", (4, 6, 0, 1728))],
    1: [("L", 6), ("L", 7), ("P", (6, 8, 0, 1728))],
    3: [("L", 8), ("L", 9), ("P", (8, 10, 0, 1728))],
    5: [("L", 10), ("L", 11)],
    8: [("T", 0), ("P", (10, 12, 0, 576)), ("O", 0), ("P", (10, 12, 576, 1152)),
        ("O", 1), ("P", (10, 12, 1152, 1728))],
}

SCALE = DH ** -0.5
EXP2_SCALE = SCALE * 1.4426950408889634
MASKED_LOGIT = -1e9 / SCALE

NT_DIMS = (((1,), (1,)), ((), ()))
F32 = jnp.float32
BF16 = jnp.bfloat16
U32 = jnp.uint32


def _mod(a, n):
    assert n & (n - 1) == 0
    return jax.lax.bitwise_and(a, n - 1)


def _div(a, n):
    assert n & (n - 1) == 0
    return jax.lax.shift_right_logical(a, n.bit_length() - 1)


def _pack(x):
    return pltpu.bitcast(x, U32)


def _unpack(x):
    return pltpu.bitcast(x, BF16)


def _mean_rows(x, chains):
    part = jnp.sum(x.reshape(D // (8 * chains), 8 * chains, x.shape[1]), axis=0)
    return jnp.sum(part, axis=0, keepdims=True) * (1.0 / D)


def _layernorm(x, chains=1, reread=None):
    m = _mean_rows(x, chains)
    c = (x if reread is None else reread(0)) - m
    v = _mean_rows(c * c, chains)
    if reread is not None:
        c = reread(1) - m
    y = c * jax.lax.rsqrt(v + EPS)
    return y.astype(BF16)


def _kernel(xT_hbm, wqkv_hbm, wo_hbm, wg_hbm, wu_hbm, wdT_hbm, out_hbm,
            xres, xio, wqkv_raw, wo_raw, wg, wu, wd,
            wqT, woT, first, ring, xn1, xn2, row_s, zero_s, sem_in, sem_o):

    def x_copy(p):
        return pltpu.make_async_copy(
            xT_hbm.at[:, pl.ds(p * SUB, SUB)], xio.at[p], sem_in.at[p])

    def f_copy(which, c):
        src = (wg_hbm, wu_hbm, wdT_hbm)[which]
        dst = (wg, wu, wd)[which]
        start = c * FC
        if not isinstance(c, int):
            start = pl.multiple_of(start, LANES)
        return pltpu.make_async_copy(
            src.at[:, pl.ds(start, FC)], dst.at[c],
            sem_in.at[NS + NP + 1 + which * NCH + c])

    def out_copy(p):
        start = p * SUB
        if not isinstance(p, int):
            start = pl.multiple_of(start, LANES)
        return pltpu.make_async_copy(
            xio.at[p], out_hbm.at[:, pl.ds(start, SUB)], sem_o.at[p])

    def out_part_copy(p, j):
        start = p * SUB
        if not isinstance(p, int):
            start = pl.multiple_of(start, LANES)
        r = pl.ds(CUTS[j], CUTS[j + 1] - CUTS[j])
        return pltpu.make_async_copy(
            xio.at[p, r], out_hbm.at[r, pl.ds(start, SUB)],
            sem_o.at[p + j * NCH])

    def wqkv_copy(j):
        cols = pl.ds(PIECES[j], PIECES[j + 1] - PIECES[j])
        return pltpu.make_async_copy(
            wqkv_hbm.at[:, cols], wqkv_raw.at[:, cols], sem_in.at[NS + j])

    wo_copy = pltpu.make_async_copy(wo_hbm, wo_raw, sem_in.at[NS + NP])

    def transpose_cols(src, dst, lo, hi):
        for c0 in range(lo, hi, LANES):
            c1 = min(c0 + LANES, hi)
            dst[c0 // 2:c1 // 2, :] = _pack(src[:, c0:c1].T)

    lane = jax.lax.broadcasted_iota(jnp.int32, (HG, LANES), 1)

    def shifted(cur, prev, w):
        if w == 0:
            return cur
        both = jnp.where(lane < LANES - DIL * w, cur, prev)
        return pltpu.roll(both, DIL * w, 1)

    def rows(base, part, d):
        return pl.ds(base + part * D + d, HG, stride=DH)

    def attn_scores(cur, prev, p, base):
        at_start = isinstance(p, int) and p == 0
        logits = [None] * W
        for d in range(DH):
            q = cur[rows(base, 0, d), :]
            kc = cur[rows(base, 1, d), :]
            kp = kc if at_start else prev[rows(base, 1, d), :]
            for w in range(W):
                t = q * shifted(kc, kp, w)
                logits[w] = t if d == 0 else logits[w] + t
        if p is not None:
            pos = p * SUB + lane
            for w in range(1, W):
                logits[w] = jnp.where(pos >= DIL * w, logits[w], MASKED_LOGIT)
        m = logits[0]
        for w in range(1, W):
            m = jnp.maximum(m, logits[w])
        es = [jnp.exp2((lg - m) * EXP2_SCALE) for lg in logits]
        s = es[0]
        for w in range(1, W):
            s = s + es[w]
        r = 1.0 / s
        return [e * r for e in es]

    def attn_values(cur, prev, base, a, sb):
        done = []
        for d in range(DH):
            vc = cur[rows(base, 2, d), :]
            vp = prev[rows(base, 2, d), :]
            o = a[0] * vc
            for w in range(1, W):
                o = o + a[w] * shifted(vc, vp, w)
            done.append((d, o))
            if len(done) == sb or d == DH - 1:
                for dd, oo in done:
                    cur[rows(base, 0, dd), :] = oo
                done = []

    def fill_clamped(buf, dst, src):
        buf[dst, 2 * D:3 * D, :] = jnp.broadcast_to(
            buf[src, 2 * D:3 * D, 0:1], (D, LANES))

    def residual(p, from_input):
        if from_input is True:
            return xio[p].astype(F32)
        if from_input is False:
            return xres[p]
        return jnp.where(from_input, xio[p].astype(F32), xres[p])

    def out_proj(qkv, p, from_input, slot, row0, reread, split=1):
        o = qkv[0:D, :].astype(BF16)
        step = D // 2 // split
        upd = jnp.concatenate(
            [jnp.dot(_unpack(woT[i * step:(i + 1) * step, :]), o,
                     preferred_element_type=F32) for i in range(split)], axis=0)
        x = residual(p, from_input) + upd
        xres[p] = x
        again = (lambda i: xres[p + zero_s[i]]) if reread else None
        xn2[slot, pl.ds(row0, SUB // 2), :] = _pack(
            _layernorm(x, reread=again).T)

    def ffn_up(xn, c):
        g = jnp.dot(xn, wg[c], preferred_element_type=F32)
        u = jnp.dot(xn, wu[c], preferred_element_type=F32)
        return (g * u).astype(BF16)

    def ffn_down(h, c):
        return jax.lax.dot_general(wd[c], h, NT_DIMS,
                                   preferred_element_type=F32)

    def ln1_pro(p):
        y = _layernorm(residual(p, True), chains=4 if p < N0 else 1)
        xn1[:, p * SUB:(p + 1) * SUB] = _pack(y)
        return y

    def project_pro(p0, p1, lo, hi, mc):
        for m0 in range(lo, hi, mc):
            m1 = min(m0 + mc, hi)
            res = jnp.dot(_unpack(wqT[m0 // 2:m1 // 2, :]),
                          _unpack(xn1[:, p0 * SUB:p1 * SUB]),
                          preferred_element_type=F32)
            for p in range(p0, p1):
                part = res[:, (p - p0) * SUB:(p - p0 + 1) * SUB]
                if p < NCH:
                    first[p, m0:m1, :] = part
                if p >= NCH or (p == NCH - 1 and m1 > D):
                    ring[p, m0:m1, :] = part

    for p in range(N0):
        x_copy(p).start()
    for j in range(NP):
        wqkv_copy(j).start()
    for p in range(N0, N0 + XE):
        x_copy(p).start()
    wo_copy.start()
    for p in range(N0 + XE, NPRO):
        x_copy(p).start()
    for c in range(NCH):
        for which in range(3):
            f_copy(which, c).start()
        if c == 0:
            for p in range(NPRO, NS):
                x_copy(p).start()
    for g in range(NG):
        row_s[g] = g * HG * DH
    zero_s[0] = 0
    zero_s[1] = 0

    for p in range(N0):
        x_copy(p).wait()
        ln1_pro(p)
    done = 0
    for j in range(NP):
        last = j == NP - 1
        wqkv_copy(j).wait()
        if last:
            for p in range(N0, N0 + XE):
                x_copy(p).wait()
        project_pro(0, N0, done, PIECES[j], MC)
        transpose_cols(wqkv_raw, wqT, PIECES[j], PIECES[j + 1])
        done = PIECES[j + 1] - (0 if last else LAG)
        project_pro(0, N0, PIECES[j], done, MC)
        if last:
            for p in range(N0, N0 + XE):
                ln1_pro(p)
    wo_copy.wait()
    for p in range(N0 + XE, NPRO):
        x_copy(p).wait()

    def unit(u):
        i, g = divmod(u, NG)
        prev = (i - 1 if i else NCH) + zero_s[0]
        return first.at[i], first.at[prev], row_s[g]

    def unit_scores(u):
        cur, prev, base = unit(u)
        return attn_scores(cur, prev, 0 if u < NG else None, base)

    fill_clamped(first, NCH, 0)
    n_units = NCH * NG
    scores = [unit_scores(u) for u in range(AHEAD)]
    for u in range(n_units + 1):
        for kind, arg in PLAN.get(u, ()):
            if kind == "P":
                project_pro(*arg, MC2)
            elif kind == "O":
                out_proj(first.at[arg], arg, True, 0, arg * SUB // 2, False)
            elif kind == "T":
                transpose_cols(wo_raw, woT, 0, D)
            else:
                y = ln1_pro(arg)
                if kind == "L":
                    first[NCH, 0:16, :] = y[D - 16:D, :].astype(F32)
        if u + AHEAD < n_units:
            scores.append(unit_scores(u + AHEAD))
        if u < n_units:
            attn_values(*unit(u), scores[u], SB0)
    for which in range(3):
        f_copy(which, 0).wait()
    for p in range(NPRO, NS):
        x_copy(p).wait()

    def body(k, do_proj):
        n = _div(k, NCH)
        c = _mod(k, NCH)
        if do_proj:
            xn1[:, 0:SUB] = _pack(_layernorm(
                residual(_mod(k + NPRO, NS), k + NPRO < NS)))
        h = ffn_up(_unpack(xn2[_mod(n, 2)]), c)
        p = _mod(k + NCH, NS)
        cur = ring.at[_mod(k + NCH, RING)]
        prev = ring.at[_mod(k + NCH - 1, RING)]
        for g in range(NG):
            a = attn_scores(cur, prev, p if do_proj else None, row_s[g])
            attn_values(cur, prev, row_s[g], a, SB if do_proj else SBM)
        out_proj(cur, p, do_proj and k + NCH < NS, _mod(n + 1, 2),
                 pl.multiple_of(c * (SUB // 2), SUB // 2),
                 RLA if do_proj else RLB, 1 if do_proj else OS)
        if do_proj:
            ring[_mod(k + NPRO, RING)] = jnp.dot(
                _unpack(wqT[...]), _unpack(xn1[:, 0:SUB]),
                preferred_element_type=F32)
        res = ffn_down(h, c)
        p0 = _mod(n, NT) * NCH
        for i in range(NCH):
            x = xres[p0 + i] + res[:, i * SUB:(i + 1) * SUB]
            xres[p0 + i] = x
            xio[p0 + i] = x.astype(BF16)

    n_main = 2 * NS - NPRO
    n_mid = 2 * NS - NCH
    assert n_main >= NS + NCH

    def main_step(k, carry):
        body(k, True)
        return carry

    def segment(i, lo):
        hi = jnp.where(i < NCH - 1, i + 1,
                       jnp.where(i == NCH - 1, NS - NCH, n_main))
        jax.lax.fori_loop(lo, hi, main_step, 0)

        @pl.when(i < NCH - 1)
        def _():
            for which in range(3):
                f_copy(which, i + 1).wait()

        @pl.when(i == NCH - 1)
        def _():
            fill_clamped(ring, (NS - 1) % RING, NS % RING)

        return hi

    def mid_step(k, carry):
        out_copy(k - n_main).start()
        body(k, False)
        return carry

    def last_step(c, carry):
        p0 = NS - NCH
        h = ffn_up(_unpack(xn2[(2 * NT - 1) % 2]), c)
        for j in range(len(CUTS) - 1):
            r0, r1 = CUTS[j], CUTS[j + 1]
            part = jax.lax.dot_general(
                wd[c, r0:r1, :], h, NT_DIMS, preferred_element_type=F32)
            for i in range(NCH):
                x = xres[p0 + i, r0:r1, :] + part[:, i * SUB:(i + 1) * SUB]
                xres[p0 + i, r0:r1, :] = x
                xio[p0 + i, r0:r1, :] = x.astype(BF16)

            @pl.when(c == NCH - 1)
            def _():
                for i in range(NCH):
                    out_part_copy(p0 + i, j).start()
        return carry

    jax.lax.fori_loop(0, NCH + 1, segment, 0)
    jax.lax.fori_loop(n_main, n_mid, mid_step, 0)
    for p in range(n_mid - n_main, NS - NCH):
        out_copy(p).start()
    jax.lax.fori_loop(0, NCH, last_step, 0)
    for p in range(NS - NCH):
        out_copy(p).wait()
    for j in range(len(CUTS) - 1):
        for p in range(NS - NCH, NS):
            out_part_copy(p, j).wait()


@jax.jit
def pallas_interleave_layers__sliding_local_dilated__glu_gated_bilinear__prompt_kernel(
    A_x: jax.Array,
    A_wqkv: jax.Array,
    A_wo: jax.Array,
    B_x: jax.Array,
    B_w_gate: jax.Array,
    B_w_up: jax.Array,
    B_w_down: jax.Array,
):
    del B_x
    xT = A_x.reshape(S, D).T
    wdT = B_w_down.T
    any_spec = pl.BlockSpec(memory_space=pl.ANY)
    outT = pl.pallas_call(
        _kernel,
        in_specs=[any_spec] * 6,
        out_specs=any_spec,
        out_shape=jax.ShapeDtypeStruct((D, S), BF16),
        scratch_shapes=[
            pltpu.VMEM((NS, D, SUB), F32),
            pltpu.VMEM((NS, D, SUB), BF16),
            pltpu.VMEM((D, 3 * D), BF16),
            pltpu.VMEM((D, D), BF16),
            pltpu.VMEM((NCH, D, FC), BF16),
            pltpu.VMEM((NCH, D, FC), BF16),
            pltpu.VMEM((NCH, D, FC), BF16),
            pltpu.VMEM((3 * D // 2, D), U32),
            pltpu.VMEM((D // 2, D), U32),
            pltpu.VMEM((NCH + 1, 3 * D, LANES), F32),
            pltpu.VMEM((RING, 3 * D, LANES), F32),
            pltpu.VMEM((D // 2, NPRO * SUB), U32),
            pltpu.VMEM((2, TM // 2, D), U32),
            pltpu.SMEM((NG,), jnp.int32),
            pltpu.SMEM((2,), jnp.int32),
            pltpu.SemaphoreType.DMA((NS + NP + 1 + 3 * NCH,)),
            pltpu.SemaphoreType.DMA((NS + (len(CUTS) - 2) * NCH,)),
        ],
        compiler_params=pltpu.CompilerParams(
            vmem_limit_bytes=100 * 1024 * 1024,
            disable_semaphore_checks=True,
            disable_bounds_checks=NOBND),
    )(xT, A_wqkv, A_wo, B_w_gate, B_w_up, wdT)
    return outT.T.reshape(1, S, D)
```

```python
import jax
import jax.numpy as jnp
import jax.experimental.pallas as pl
import jax.experimental.pallas.tpu as pltpu

S = 2048
D = 576
F = 4608
H = 32
DH = 18
W = 8
DIL = 2
EPS = 1e-5
LANES = 128

TM = 256
NT = S // TM
FC = 2304
NCH = F // FC
SUB = TM // NCH
NS = S // SUB
HG = 8
NG = H // HG
SB = 4
SB0 = 5
RING = 16
PIECES = (0, 256, 640, 1152, 1728)
NP = len(PIECES) - 1
LAG = 128
MC = 256
MC2 = 288
NPRO = 12
XE = 2
CUTS = (0, 448, 576)
N0 = 4

PLAN = {
    0: [("P", (4, 6, 0, 1728))],
    1: [("L", 6)],
    2: [("L", 7), ("P", (6, 8, 0, 1728))],
    3: [("L", 8)],
    4: [("L", 9), ("P", (8, 10, 0, 1728))],
    5: [("L", 10)],
    6: [("L", 11)],
    8: [("T", 0), ("P", (10, 12, 0, 576)), ("O", 0),
        ("P", (10, 12, 576, 1152)), ("O", 1), ("P", (10, 12, 1152, 1728))],
}

SCALE = DH ** -0.5
EXP2_SCALE = SCALE * 1.4426950408889634
MASKED_LOGIT = -1e9 / SCALE

NT_DIMS = (((1,), (1,)), ((), ()))
F32 = jnp.float32
BF16 = jnp.bfloat16
U32 = jnp.uint32


def _mod(a, n):
    assert n & (n - 1) == 0
    return jax.lax.bitwise_and(a, n - 1)


def _div(a, n):
    assert n & (n - 1) == 0
    return jax.lax.shift_right_logical(a, n.bit_length() - 1)


def _pack(x):
    return pltpu.bitcast(x, U32)


def _unpack(x):
    return pltpu.bitcast(x, BF16)


def _mean_rows(x, chains):
    part = jnp.sum(x.reshape(D // (8 * chains), 8 * chains, x.shape[1]), axis=0)
    return jnp.sum(part, axis=0, keepdims=True) * (1.0 / D)


def _layernorm(x, chains=1, reread=None):
    m = _mean_rows(x, chains)
    c = (x if reread is None else reread(0)) - m
    v = _mean_rows(c * c, chains)
    if reread is not None:
        c = reread(1) - m
    y = c * jax.lax.rsqrt(v + EPS)
    return y.astype(BF16)


def _kernel(xT_hbm, wqkv_hbm, wo_hbm, wg_hbm, wu_hbm, wdT_hbm, out_hbm,
            xres, xio, wqkv_raw, wo_raw, wg, wu, wd,
            wqT, woT, first, ring, xn1, xn2, row_s, zero_s, sem_in, sem_o):

    def x_copy(p):
        return pltpu.make_async_copy(
            xT_hbm.at[:, pl.ds(p * SUB, SUB)], xio.at[p], sem_in.at[p])

    def f_copy(which, c):
        src = (wg_hbm, wu_hbm, wdT_hbm)[which]
        dst = (wg, wu, wd)[which]
        start = c * FC
        if not isinstance(c, int):
            start = pl.multiple_of(start, LANES)
        return pltpu.make_async_copy(
            src.at[:, pl.ds(start, FC)], dst.at[c],
            sem_in.at[NS + NP + 1 + which * NCH + c])

    def out_copy(p):
        start = p * SUB
        if not isinstance(p, int):
            start = pl.multiple_of(start, LANES)
        return pltpu.make_async_copy(
            xio.at[p], out_hbm.at[:, pl.ds(start, SUB)], sem_o.at[p])

    def out_part_copy(p, j):
        r = pl.ds(CUTS[j], CUTS[j + 1] - CUTS[j])
        return pltpu.make_async_copy(
            xio.at[p, r], out_hbm.at[r, pl.ds(p * SUB, SUB)],
            sem_o.at[p + j * NCH])

    def wqkv_copy(j):
        cols = pl.ds(PIECES[j], PIECES[j + 1] - PIECES[j])
        return pltpu.make_async_copy(
            wqkv_hbm.at[:, cols], wqkv_raw.at[:, cols], sem_in.at[NS + j])

    wo_copy = pltpu.make_async_copy(wo_hbm, wo_raw, sem_in.at[NS + NP])

    def transpose_cols(src, dst, lo, hi):
        for c0 in range(lo, hi, LANES):
            c1 = min(c0 + LANES, hi)
            dst[c0 // 2:c1 // 2, :] = _pack(src[:, c0:c1].T)

    lane = jax.lax.broadcasted_iota(jnp.int32, (HG, LANES), 1)

    def shifted(cur, prev, w):
        if w == 0:
            return cur
        both = jnp.where(lane < LANES - DIL * w, cur, prev)
        return pltpu.roll(both, DIL * w, 1)

    def rows(base, part, d):
        return pl.ds(base + part * D + d, HG, stride=DH)

    def attn_scores(cur, prev, p, base):
        at_start = isinstance(p, int) and p == 0
        logits = [None] * W
        for d in range(DH):
            q = cur[rows(base, 0, d), :]
            kc = cur[rows(base, 1, d), :]
            kp = kc if at_start else prev[rows(base, 1, d), :]
            for w in range(W):
                t = q * shifted(kc, kp, w)
                logits[w] = t if d == 0 else logits[w] + t
        if p is not None:
            pos = p * SUB + lane
            for w in range(1, W):
                logits[w] = jnp.where(pos >= DIL * w, logits[w], MASKED_LOGIT)
        m = logits[0]
        for w in range(1, W):
            m = jnp.maximum(m, logits[w])
        es = [jnp.exp2((lg - m) * EXP2_SCALE) for lg in logits]
        s = es[0]
        for w in range(1, W):
            s = s + es[w]
        r = 1.0 / s
        return [e * r for e in es]

    def attn_values(cur, prev, base, a, sb):
        done = []
        for d in range(DH):
            vc = cur[rows(base, 2, d), :]
            vp = prev[rows(base, 2, d), :]
            o = a[0] * vc
            for w in range(1, W):
                o = o + a[w] * shifted(vc, vp, w)
            done.append((d, o))
            if len(done) == sb or d == DH - 1:
                for dd, oo in done:
                    cur[rows(base, 0, dd), :] = oo
                done = []

    def fill_clamped(buf, dst, src):
        buf[dst, 2 * D:3 * D, :] = jnp.broadcast_to(
            buf[src, 2 * D:3 * D, 0:1], (D, LANES))

    def residual(p, from_input):
        if from_input is True:
            return xio[p].astype(F32)
        if from_input is False:
            return xres[p]
        return jnp.where(from_input, xio[p].astype(F32), xres[p])

    def out_proj(qkv, p, from_input, slot, row0, reread):
        upd = jnp.dot(_unpack(woT[...]), qkv[0:D, :].astype(BF16),
                      preferred_element_type=F32)
        x = residual(p, from_input) + upd
        xres[p] = x
        again = (lambda i: xres[p + zero_s[i]]) if reread else None
        xn2[slot, pl.ds(row0, SUB // 2), :] = _pack(
            _layernorm(x, reread=again).T)

    def ffn_up(xn, c):
        g = jnp.dot(xn, wg[c], preferred_element_type=F32)
        u = jnp.dot(xn, wu[c], preferred_element_type=F32)
        return (g * u).astype(BF16)

    def ffn_down(h, c):
        return jax.lax.dot_general(wd[c], h, NT_DIMS,
                                   preferred_element_type=F32)

    def ln1_pro(p):
        y = _layernorm(residual(p, True), chains=4 if p < N0 else 1)
        xn1[:, p * SUB:(p + 1) * SUB] = _pack(y)
        return y

    def project_pro(p0, p1, lo, hi, mc):
        for m0 in range(lo, hi, mc):
            m1 = min(m0 + mc, hi)
            res = jnp.dot(_unpack(wqT[m0 // 2:m1 // 2, :]),
                          _unpack(xn1[:, p0 * SUB:p1 * SUB]),
                          preferred_element_type=F32)
            for p in range(p0, p1):
                part = res[:, (p - p0) * SUB:(p - p0 + 1) * SUB]
                if p < NCH:
                    first[p, m0:m1, :] = part
                if p >= NCH or (p == NCH - 1 and m1 > D):
                    ring[p, m0:m1, :] = part

    for p in range(N0):
        x_copy(p).start()
    for j in range(NP):
        wqkv_copy(j).start()
    for p in range(N0, N0 + XE):
        x_copy(p).start()
    wo_copy.start()
    for p in range(N0 + XE, NPRO):
        x_copy(p).start()
    for c in range(NCH):
        for which in range(3):
            f_copy(which, c).start()
        if c == 0:
            for p in range(NPRO, NS):
                x_copy(p).start()
    for g in range(NG):
        row_s[g] = g * HG * DH
    zero_s[0] = 0
    zero_s[1] = 0

    for p in range(N0):
        x_copy(p).wait()
        ln1_pro(p)
    done = 0
    for j in range(NP):
        last = j == NP - 1
        wqkv_copy(j).wait()
        if last:
            for p in range(N0, N0 + XE):
                x_copy(p).wait()
        project_pro(0, N0, done, PIECES[j], MC)
        transpose_cols(wqkv_raw, wqT, PIECES[j], PIECES[j + 1])
        done = PIECES[j + 1] - (0 if last else LAG)
        project_pro(0, N0, PIECES[j], done, MC)
        if last:
            for p in range(N0, N0 + XE):
                ln1_pro(p)
    wo_copy.wait()
    for p in range(N0 + XE, NPRO):
        x_copy(p).wait()

    fill_clamped(first, NCH, 0)
    for u in range(NCH * NG + 1):
        for kind, arg in PLAN.get(u, ()):
            if kind == "P":
                project_pro(*arg, MC2)
            elif kind == "O":
                out_proj(first.at[arg], arg, True, 0, arg * SUB // 2, False)
            elif kind == "T":
                transpose_cols(wo_raw, woT, 0, D)
            else:
                first[NCH, 0:16, :] = ln1_pro(arg)[D - 16:D, :].astype(F32)
        if u < NCH * NG:
            i, g = divmod(u, NG)
            cur = first.at[i]
            prev = first.at[(i - 1 if i else NCH) + zero_s[0]]
            a = attn_scores(cur, prev, None if i else 0, row_s[g])
            attn_values(cur, prev, row_s[g], a, SB0)
    for which in range(3):
        f_copy(which, 0).wait()
    for p in range(NPRO, NS):
        x_copy(p).wait()

    def body(k, do_proj):
        n = _div(k, NCH)
        c = _mod(k, NCH)
        if do_proj:
            xn1[:, 0:SUB] = _pack(_layernorm(
                residual(_mod(k + NPRO, NS), k + NPRO < NS)))
        h = ffn_up(_unpack(xn2[_mod(n, 2)]), c)
        p = _mod(k + NCH, NS)
        cur = ring.at[_mod(k + NCH, RING)]
        prev = ring.at[_mod(k + NCH - 1, RING)]
        for g in range(NG):
            a = attn_scores(cur, prev, p if do_proj else None, row_s[g])
            attn_values(cur, prev, row_s[g], a, SB)
        out_proj(cur, p, do_proj and k + NCH < NS, _mod(n + 1, 2),
                 pl.multiple_of(c * (SUB // 2), SUB // 2), not do_proj)
        if do_proj:
            ring[_mod(k + NPRO, RING)] = jnp.dot(
                _unpack(wqT[...]), _unpack(xn1[:, 0:SUB]),
                preferred_element_type=F32)
        res = ffn_down(h, c)
        p0 = _mod(n, NT) * NCH
        for i in range(NCH):
            x = xres[p0 + i] + res[:, i * SUB:(i + 1) * SUB]
            xres[p0 + i] = x
            xio[p0 + i] = x.astype(BF16)

    n_main = 2 * NS - NPRO
    n_mid = 2 * NS - NCH
    assert n_main >= NS + NCH

    def main_step(k, carry):
        body(k, True)
        return carry

    def segment(i, lo):
        hi = jnp.where(i < NCH - 1, i + 1,
                       jnp.where(i == NCH - 1, NS - NCH, n_main))
        jax.lax.fori_loop(lo, hi, main_step, 0)

        @pl.when(i < NCH - 1)
        def _():
            for which in range(3):
                f_copy(which, i + 1).wait()

        @pl.when(i == NCH - 1)
        def _():
            fill_clamped(ring, (NS - 1) % RING, NS % RING)

        return hi

    def mid_step(k, carry):
        out_copy(k - n_main).start()
        body(k, False)
        return carry

    def last_step(c, carry):
        p0 = NS - NCH
        h = ffn_up(_unpack(xn2[(2 * NT - 1) % 2]), c)
        for j in range(len(CUTS) - 1):
            r0, r1 = CUTS[j], CUTS[j + 1]
            part = jax.lax.dot_general(
                wd[c, r0:r1, :], h, NT_DIMS, preferred_element_type=F32)
            for i in range(NCH):
                x = xres[p0 + i, r0:r1, :] + part[:, i * SUB:(i + 1) * SUB]
                xres[p0 + i, r0:r1, :] = x
                xio[p0 + i, r0:r1, :] = x.astype(BF16)

            @pl.when(c == NCH - 1)
            def _():
                for i in range(NCH):
                    out_part_copy(p0 + i, j).start()
        return carry

    jax.lax.fori_loop(0, NCH + 1, segment, 0)
    jax.lax.fori_loop(n_main, n_mid, mid_step, 0)
    for p in range(n_mid - n_main, NS - NCH):
        out_copy(p).start()
    jax.lax.fori_loop(0, NCH, last_step, 0)
    for p in range(NS - NCH):
        out_copy(p).wait()
    for j in range(len(CUTS) - 1):
        for p in range(NS - NCH, NS):
            out_part_copy(p, j).wait()


@jax.jit
def pallas_interleave_layers__sliding_local_dilated__glu_gated_bilinear__prompt_kernel(
    A_x: jax.Array,
    A_wqkv: jax.Array,
    A_wo: jax.Array,
    B_x: jax.Array,
    B_w_gate: jax.Array,
    B_w_up: jax.Array,
    B_w_down: jax.Array,
):
    del B_x
    xT = A_x.reshape(S, D).T
    wdT = B_w_down.T
    any_spec = pl.BlockSpec(memory_space=pl.ANY)
    outT = pl.pallas_call(
        _kernel,
        in_specs=[any_spec] * 6,
        out_specs=any_spec,
        out_shape=jax.ShapeDtypeStruct((D, S), BF16),
        scratch_shapes=[
            pltpu.VMEM((NS, D, SUB), F32),
            pltpu.VMEM((NS, D, SUB), BF16),
            pltpu.VMEM((D, 3 * D), BF16),
            pltpu.VMEM((D, D), BF16),
            pltpu.VMEM((NCH, D, FC), BF16),
            pltpu.VMEM((NCH, D, FC), BF16),
            pltpu.VMEM((NCH, D, FC), BF16),
            pltpu.VMEM((3 * D // 2, D), U32),
            pltpu.VMEM((D // 2, D), U32),
            pltpu.VMEM((NCH + 1, 3 * D, LANES), F32),
            pltpu.VMEM((RING, 3 * D, LANES), F32),
            pltpu.VMEM((D // 2, NPRO * SUB), U32),
            pltpu.VMEM((2, TM // 2, D), U32),
            pltpu.SMEM((NG,), jnp.int32),
            pltpu.SMEM((2,), jnp.int32),
            pltpu.SemaphoreType.DMA((NS + NP + 1 + 3 * NCH,)),
            pltpu.SemaphoreType.DMA((NS + (len(CUTS) - 2) * NCH,)),
        ],
        compiler_params=pltpu.CompilerParams(
            vmem_limit_bytes=100 * 1024 * 1024,
            disable_semaphore_checks=True),
    )(xT, A_wqkv, A_wo, B_w_gate, B_w_up, wdT)
    return outT.T.reshape(1, S, D)
```

```python
import jax
import jax.numpy as jnp
import jax.experimental.pallas as pl
import jax.experimental.pallas.tpu as pltpu

S = 2048
D = 576
F = 4608
H = 32
DH = 18
W = 8
DIL = 2
EPS = 1e-5
LANES = 128

TM = 256
NT = S // TM
FC = 2304
NCH = F // FC
SUB = TM // NCH
NS = S // SUB
HG = 8
NG = H // HG
SB = 4
SB0 = 5
RING = 16
PIECES = (0, 256, 640, 1152, 1728)
NP = len(PIECES) - 1
MC2 = 288
NPRO = 12
CUTS = (0, 448, 576)
N0 = 4

START = [
    ("x", 0), ("L", 0), ("x", 1), ("L", 1),
    ("w", 0), ("T", 0), ("P", (0, 2, 0, 256, 128)),
    ("x", 2), ("x", 3), ("L", 2), ("L", 3), ("P", (2, 4, 0, 256, 128)),
    ("w", 1), ("T", 1), ("P", (0, 4, 256, 512, 128)),
    ("w", 2), ("P", (0, 4, 512, 640, 256)), ("T", 2),
    ("P", (0, 4, 640, 1024, 256)),
    ("w", 3), ("x", 4), ("x", 5), ("P", (0, 4, 1024, 1152, 256)), ("T", 3),
    ("P", (0, 4, 1152, 1728, 256)), ("L", 4), ("L", 5),
]

PLAN = {
    0: [("P", (4, 6, 0, 1728))],
    1: [("L", 6)],
    2: [("L", 7), ("P", (6, 8, 0, 1728))],
    3: [("L", 8)],
    4: [("L", 9), ("P", (8, 10, 0, 1728))],
    5: [("L", 10)],
    6: [("L", 11)],
    8: [("T", 0), ("P", (10, 12, 0, 576)), ("O", 0),
        ("P", (10, 12, 576, 1152)), ("O", 1), ("P", (10, 12, 1152, 1728))],
}

SCALE = DH ** -0.5
EXP2_SCALE = SCALE * 1.4426950408889634
MASKED_LOGIT = -1e9 / SCALE

NT_DIMS = (((1,), (1,)), ((), ()))
F32 = jnp.float32
BF16 = jnp.bfloat16
U32 = jnp.uint32


def _mod(a, n):
    assert n & (n - 1) == 0
    return jax.lax.bitwise_and(a, n - 1)


def _div(a, n):
    assert n & (n - 1) == 0
    return jax.lax.shift_right_logical(a, n.bit_length() - 1)


def _pack(x):
    return pltpu.bitcast(x, U32)


def _unpack(x):
    return pltpu.bitcast(x, BF16)


def _mean_rows(x, chains):
    part = jnp.sum(x.reshape(D // (8 * chains), 8 * chains, x.shape[1]), axis=0)
    return jnp.sum(part, axis=0, keepdims=True) * (1.0 / D)


def _layernorm(x, chains=1, reread=None):
    m = _mean_rows(x, chains)
    c = (x if reread is None else reread(0)) - m
    v = _mean_rows(c * c, chains)
    if reread is not None:
        c = reread(1) - m
    y = c * jax.lax.rsqrt(v + EPS)
    return y.astype(BF16)


def _kernel(xT_hbm, wqkv_hbm, wo_hbm, wg_hbm, wu_hbm, wdT_hbm, out_hbm,
            xres, xio, wqkv_raw, wo_raw, wg, wu, wd,
            wqT, woT, first, ring, xn1, xn2, row_s, zero_s, sem_in, sem_o):

    def x_copy(p):
        return pltpu.make_async_copy(
            xT_hbm.at[:, pl.ds(p * SUB, SUB)], xio.at[p], sem_in.at[p])

    def f_copy(which, c):
        src = (wg_hbm, wu_hbm, wdT_hbm)[which]
        dst = (wg, wu, wd)[which]
        start = c * FC
        if not isinstance(c, int):
            start = pl.multiple_of(start, LANES)
        return pltpu.make_async_copy(
            src.at[:, pl.ds(start, FC)], dst.at[c],
            sem_in.at[NS + NP + 1 + which * NCH + c])

    def out_copy(p):
        start = p * SUB
        if not isinstance(p, int):
            start = pl.multiple_of(start, LANES)
        return pltpu.make_async_copy(
            xio.at[p], out_hbm.at[:, pl.ds(start, SUB)], sem_o.at[p])

    def out_part_copy(p, j):
        r = pl.ds(CUTS[j], CUTS[j + 1] - CUTS[j])
        return pltpu.make_async_copy(
            xio.at[p, r], out_hbm.at[r, pl.ds(p * SUB, SUB)],
            sem_o.at[p + j * NCH])

    def wqkv_copy(j):
        cols = pl.ds(PIECES[j], PIECES[j + 1] - PIECES[j])
        return pltpu.make_async_copy(
            wqkv_hbm.at[:, cols], wqkv_raw.at[:, cols], sem_in.at[NS + j])

    wo_copy = pltpu.make_async_copy(wo_hbm, wo_raw, sem_in.at[NS + NP])

    def transpose_cols(src, dst, lo, hi):
        for c0 in range(lo, hi, LANES):
            c1 = min(c0 + LANES, hi)
            dst[c0 // 2:c1 // 2, :] = _pack(src[:, c0:c1].T)

    lane = jax.lax.broadcasted_iota(jnp.int32, (HG, LANES), 1)

    def shifted(cur, prev, w):
        if w == 0:
            return cur
        both = jnp.where(lane < LANES - DIL * w, cur, prev)
        return pltpu.roll(both, DIL * w, 1)

    def rows(base, part, d):
        return pl.ds(base + part * D + d, HG, stride=DH)

    def attn_scores(cur, prev, p, base):
        at_start = isinstance(p, int) and p == 0
        logits = [None] * W
        for d in range(DH):
            q = cur[rows(base, 0, d), :]
            kc = cur[rows(base, 1, d), :]
            kp = kc if at_start else prev[rows(base, 1, d), :]
            for w in range(W):
                t = q * shifted(kc, kp, w)
                logits[w] = t if d == 0 else logits[w] + t
        if p is not None:
            pos = p * SUB + lane
            for w in range(1, W):
                logits[w] = jnp.where(pos >= DIL * w, logits[w], MASKED_LOGIT)
        m = logits[0]
        for w in range(1, W):
            m = jnp.maximum(m, logits[w])
        es = [jnp.exp2((lg - m) * EXP2_SCALE) for lg in logits]
        s = es[0]
        for w in range(1, W):
            s = s + es[w]
        r = 1.0 / s
        return [e * r for e in es]

    def attn_values(cur, prev, base, a, sb):
        done = []
        for d in range(DH):
            vc = cur[rows(base, 2, d), :]
            vp = prev[rows(base, 2, d), :]
            o = a[0] * vc
            for w in range(1, W):
                o = o + a[w] * shifted(vc, vp, w)
            done.append((d, o))
            if len(done) == sb or d == DH - 1:
                for dd, oo in done:
                    cur[rows(base, 0, dd), :] = oo
                done = []

    def fill_clamped(buf, dst, src):
        buf[dst, 2 * D:3 * D, :] = jnp.broadcast_to(
            buf[src, 2 * D:3 * D, 0:1], (D, LANES))

    def residual(p, from_input):
        if from_input is True:
            return xio[p].astype(F32)
        if from_input is False:
            return xres[p]
        return jnp.where(from_input, xio[p].astype(F32), xres[p])

    def out_proj(qkv, p, from_input, slot, row0, reread):
        upd = jnp.dot(_unpack(woT[...]), qkv[0:D, :].astype(BF16),
                      preferred_element_type=F32)
        x = residual(p, from_input) + upd
        xres[p] = x
        again = (lambda i: xres[p + zero_s[i]]) if reread else None
        xn2[slot, pl.ds(row0, SUB // 2), :] = _pack(
            _layernorm(x, reread=again).T)

    def ffn_up(xn, c):
        g = jnp.dot(xn, wg[c], preferred_element_type=F32)
        u = jnp.dot(xn, wu[c], preferred_element_type=F32)
        return (g * u).astype(BF16)

    def ffn_down(h, c):
        return jax.lax.dot_general(wd[c], h, NT_DIMS,
                                   preferred_element_type=F32)

    def ln1_pro(p):
        y = _layernorm(residual(p, True), chains=4 if p < N0 else 1)
        xn1[:, p * SUB:(p + 1) * SUB] = _pack(y)
        return y

    def project_pro(p0, p1, lo, hi, mc):
        for m0 in range(lo, hi, mc):
            m1 = min(m0 + mc, hi)
            res = jnp.dot(_unpack(wqT[m0 // 2:m1 // 2, :]),
                          _unpack(xn1[:, p0 * SUB:p1 * SUB]),
                          preferred_element_type=F32)
            for p in range(p0, p1):
                part = res[:, (p - p0) * SUB:(p - p0 + 1) * SUB]
                if p < NCH:
                    first[p, m0:m1, :] = part
                if p >= NCH or (p == NCH - 1 and m1 > D):
                    ring[p, m0:m1, :] = part

    def copy_of(kind, arg):
        return x_copy(arg) if kind == "x" else wqkv_copy(arg)

    for step in START:
        if step[0] in "xw":
            copy_of(*step).start()
    n_early = 1 + max(step[1] for step in START if step[0] == "x")
    wo_copy.start()
    for p in range(n_early, NPRO):
        x_copy(p).start()
    for c in range(NCH):
        for which in range(3):
            f_copy(which, c).start()
        if c == 0:
            for p in range(NPRO, NS):
                x_copy(p).start()
    for g in range(NG):
        row_s[g] = g * HG * DH
    zero_s[0] = 0
    zero_s[1] = 0

    for kind, arg in START:
        if kind in "xw":
            copy_of(kind, arg).wait()
        elif kind == "L":
            ln1_pro(arg)
        elif kind == "T":
            transpose_cols(wqkv_raw, wqT, PIECES[arg], PIECES[arg + 1])
        else:
            project_pro(*arg)
    wo_copy.wait()
    for p in range(n_early, NPRO):
        x_copy(p).wait()

    fill_clamped(first, NCH, 0)
    for u in range(NCH * NG + 1):
        for kind, arg in PLAN.get(u, ()):
            if kind == "P":
                project_pro(*arg, MC2)
            elif kind == "O":
                out_proj(first.at[arg], arg, True, 0, arg * SUB // 2, False)
            elif kind == "T":
                transpose_cols(wo_raw, woT, 0, D)
            else:
                first[NCH, 0:16, :] = ln1_pro(arg)[D - 16:D, :].astype(F32)
        if u < NCH * NG:
            i, g = divmod(u, NG)
            cur = first.at[i]
            prev = first.at[(i - 1 if i else NCH) + zero_s[0]]
            a = attn_scores(cur, prev, None if i else 0, row_s[g])
            attn_values(cur, prev, row_s[g], a, SB0)
    for which in range(3):
        f_copy(which, 0).wait()
    for p in range(NPRO, NS):
        x_copy(p).wait()

    def body(k, do_proj):
        n = _div(k, NCH)
        c = _mod(k, NCH)
        if do_proj:
            xn1[:, 0:SUB] = _pack(_layernorm(
                residual(_mod(k + NPRO, NS), k + NPRO < NS)))
        h = ffn_up(_unpack(xn2[_mod(n, 2)]), c)
        p = _mod(k + NCH, NS)
        cur = ring.at[_mod(k + NCH, RING)]
        prev = ring.at[_mod(k + NCH - 1, RING)]
        for g in range(NG):
            a = attn_scores(cur, prev, p if do_proj else None, row_s[g])
            attn_values(cur, prev, row_s[g], a, SB)
        out_proj(cur, p, do_proj and k + NCH < NS, _mod(n + 1, 2),
                 pl.multiple_of(c * (SUB // 2), SUB // 2), not do_proj)
        if do_proj:
            ring[_mod(k + NPRO, RING)] = jnp.dot(
                _unpack(wqT[...]), _unpack(xn1[:, 0:SUB]),
                preferred_element_type=F32)
        res = ffn_down(h, c)
        p0 = _mod(n, NT) * NCH
        for i in range(NCH):
            x = xres[p0 + i] + res[:, i * SUB:(i + 1) * SUB]
            xres[p0 + i] = x
            xio[p0 + i] = x.astype(BF16)

    n_main = 2 * NS - NPRO
    n_mid = 2 * NS - NCH
    assert n_main >= NS + NCH

    def main_step(k, carry):
        body(k, True)
        return carry

    def segment(i, lo):
        hi = jnp.where(i < NCH - 1, i + 1,
                       jnp.where(i == NCH - 1, NS - NCH, n_main))
        jax.lax.fori_loop(lo, hi, main_step, 0)

        @pl.when(i < NCH - 1)
        def _():
            for which in range(3):
                f_copy(which, i + 1).wait()

        @pl.when(i == NCH - 1)
        def _():
            fill_clamped(ring, (NS - 1) % RING, NS % RING)

        return hi

    def mid_step(k, carry):
        out_copy(k - n_main).start()
        body(k, False)
        return carry

    def last_step(c, carry):
        p0 = NS - NCH
        h = ffn_up(_unpack(xn2[(2 * NT - 1) % 2]), c)
        for j in range(len(CUTS) - 1):
            r0, r1 = CUTS[j], CUTS[j + 1]
            part = jax.lax.dot_general(
                wd[c, r0:r1, :], h, NT_DIMS, preferred_element_type=F32)
            for i in range(NCH):
                x = xres[p0 + i, r0:r1, :] + part[:, i * SUB:(i + 1) * SUB]
                xres[p0 + i, r0:r1, :] = x
                xio[p0 + i, r0:r1, :] = x.astype(BF16)

            @pl.when(c == NCH - 1)
            def _():
                for i in range(NCH):
                    out_part_copy(p0 + i, j).start()
        return carry

    jax.lax.fori_loop(0, NCH + 1, segment, 0)
    jax.lax.fori_loop(n_main, n_mid, mid_step, 0)
    for p in range(n_mid - n_main, NS - NCH):
        out_copy(p).start()
    jax.lax.fori_loop(0, NCH, last_step, 0)
    for p in range(NS - NCH):
        out_copy(p).wait()
    for j in range(len(CUTS) - 1):
        for p in range(NS - NCH, NS):
            out_part_copy(p, j).wait()


@jax.jit
def pallas_interleave_layers__sliding_local_dilated__glu_gated_bilinear__prompt_kernel(
    A_x: jax.Array,
    A_wqkv: jax.Array,
    A_wo: jax.Array,
    B_x: jax.Array,
    B_w_gate: jax.Array,
    B_w_up: jax.Array,
    B_w_down: jax.Array,
):
    del B_x
    xT = A_x.reshape(S, D).T
    wdT = B_w_down.T
    any_spec = pl.BlockSpec(memory_space=pl.ANY)
    outT = pl.pallas_call(
        _kernel,
        in_specs=[any_spec] * 6,
        out_specs=any_spec,
        out_shape=jax.ShapeDtypeStruct((D, S), BF16),
        scratch_shapes=[
            pltpu.VMEM((NS, D, SUB), F32),
            pltpu.VMEM((NS, D, SUB), BF16),
            pltpu.VMEM((D, 3 * D), BF16),
            pltpu.VMEM((D, D), BF16),
            pltpu.VMEM((NCH, D, FC), BF16),
            pltpu.VMEM((NCH, D, FC), BF16),
            pltpu.VMEM((NCH, D, FC), BF16),
            pltpu.VMEM((3 * D // 2, D), U32),
            pltpu.VMEM((D // 2, D), U32),
            pltpu.VMEM((NCH + 1, 3 * D, LANES), F32),
            pltpu.VMEM((RING, 3 * D, LANES), F32),
            pltpu.VMEM((D // 2, NPRO * SUB), U32),
            pltpu.VMEM((2, TM // 2, D), U32),
            pltpu.SMEM((NG,), jnp.int32),
            pltpu.SMEM((2,), jnp.int32),
            pltpu.SemaphoreType.DMA((NS + NP + 1 + 3 * NCH,)),
            pltpu.SemaphoreType.DMA((NS + (len(CUTS) - 2) * NCH,)),
        ],
        compiler_params=pltpu.CompilerParams(
            vmem_limit_bytes=100 * 1024 * 1024,
            disable_semaphore_checks=True),
    )(xT, A_wqkv, A_wo, B_w_gate, B_w_up, wdT)
    return outT.T.reshape(1, S, D)
```
